```python
import jax
import jax.numpy as jnp

def _softmax(x, axis=-1):
    return jax.nn.softmax(x, axis=axis)

def _gelu(x):
    return jax.nn.gelu(x, approximate=True)

def _silu(x):
    return jax.nn.silu(x)

def _sigmoid(x):
    return jax.nn.sigmoid(x)

def _layernorm(x, axis=-1, eps=1e-05):
    m = jnp.mean(x, axis=axis, keepdims=True)
    v = jnp.var(x, axis=axis, keepdims=True)
    return (x - m) / jnp.sqrt(v + eps)

def _scatter_add(tgt, idx, src, axis=0):
    return tgt.at[idx].add(src)

def _segment_sum(src, seg, n):
    return jax.ops.segment_sum(src, seg, n)

class _Rng:

    def __init__(self, key):
        self._k = key

    def _next(self):
        self._k, sub = jax.random.split(self._k)
        return sub

    def normal(self, shape):
        return jax.random.normal(self._next(), shape, dtype=jnp.bfloat16)

    def randint(self, lo, hi, shape):
        return jax.random.randint(self._next(), shape, lo, hi, dtype=jnp.int32)

    def uniform(self, shape, lo=0.0, hi=1.0):
        return jax.random.uniform(self._next(), shape, jnp.bfloat16, lo, hi)

    def permutation(self, n):
        return jax.random.permutation(self._next(), n)
kernel_name = 'interleave_layers__memory_aug_recurrent_mem_tr__moe_arch_mod__prompt'

def setup_inputs():
    _rng = _Rng(jax.random.key(int.from_bytes(__import__("os").urandom(4), "little")))
    _w = lambda a: (lambda t: t.astype(jnp.bfloat16) if jnp.issubdtype(t.dtype, jnp.floating) else t)(jnp.asarray(a))

    def _A_setup():
        B, S, Dm = (1, 2048, 512)
        H, Dh = (32, 128)
        M, seg = (8, 32)
        seg = min(seg, S)
        S = S // seg * seg
        return {'x': _w((lambda *s: _rng.normal(s) * 0.05)(B, S, Dm)), 'mem0': _w((lambda *s: _rng.normal(s) * 0.05)(B, M, Dm)), 'Wq': _w((lambda *s: _rng.normal(s) * 0.05)(Dm, H, Dh) * Dm ** (-0.5)), 'Wk': _w((lambda *s: _rng.normal(s) * 0.05)(Dm, H, Dh) * Dm ** (-0.5)), 'Wv': _w((lambda *s: _rng.normal(s) * 0.05)(Dm, H, Dh) * Dm ** (-0.5)), 'Wo': _w((lambda *s: _rng.normal(s) * 0.05)(H, Dh, Dm) * (H * Dh) ** (-0.5)), 'seg_len': seg}
    _A_in = _A_setup()

    def _B_setup():
        B, S, D, F, C = (1, 2048, 512, 1792, 1)
        return {'x': _w((lambda *s: _rng.normal(s) * 0.05)(B, S, D)), 'w_r': _w((lambda *s: _rng.normal(s) * 0.05)(D)), 'w_gate': _w((lambda *s: _rng.normal(s) * 0.05)(D, F)), 'w_up': _w((lambda *s: _rng.normal(s) * 0.05)(D, F)), 'w_down': _w((lambda *s: _rng.normal(s) * 0.05)(F, D))}
    _B_in = _B_setup()
    return {'A_x': _A_in['x'], 'A_mem0': _A_in['mem0'], 'A_Wq': _A_in['Wq'], 'A_Wk': _A_in['Wk'], 'A_Wv': _A_in['Wv'], 'A_Wo': _A_in['Wo'], 'A_seg_len': _A_in['seg_len'], 'B_x': _B_in['x'], 'B_w_r': _B_in['w_r'], 'B_w_gate': _B_in['w_gate'], 'B_w_up': _B_in['w_up'], 'B_w_down': _B_in['w_down']}

def reference(A_x, A_mem0, A_Wq, A_Wk, A_Wv, A_Wo, A_seg_len, B_x, B_w_r, B_w_gate, B_w_up, B_w_down):

    def _A_ref(x, mem0, Wq, Wk, Wv, Wo, seg_len):
        B, S, Dm = x.shape
        H, Dh = (Wq.shape[1], Wq.shape[2])
        M = mem0.shape[1]
        scale = Dh ** (-0.5)
        n_seg = S // seg_len
        L = M + seg_len
        idx = jnp.arange(L)
        mask = (idx[:, None] < M) | (idx[:, None] >= idx[None, :])
        mem = mem0
        outs = []
        for s in range(n_seg):
            xs = x[:, s * seg_len:(s + 1) * seg_len, :].copy()
            h = jnp.concatenate([mem, xs], axis=1)
            q = jnp.einsum('btd,dhe->bhte', h, Wq)
            k = jnp.einsum('btd,dhe->bhte', h, Wk)
            v = jnp.einsum('btd,dhe->bhte', h, Wv)
            scores = jnp.einsum('bhqe,bhke->bhqk', q, k) * scale
            scores = jnp.where(mask[None, None], scores, -1000000000.0)
            p = _softmax(scores, axis=-1)
            o = jnp.einsum('bhqk,bhke->bhqe', p, v)
            o = jnp.einsum('bhte,hed->btd', o, Wo)
            mem = o[:, :M, :].copy()
            outs.append(o[:, M:, :])
        return jnp.concatenate(outs, axis=1)

    def _B_ref(x, w_r, w_gate, w_up, w_down):
        B, S, D = x.shape
        C = 1
        r = x @ w_r
        idx = jnp.argsort(-r, axis=-1)[:, :C]
        idx_e = jnp.repeat(idx.reshape(B, C, 1), D, axis=2)
        x_sel = jnp.take_along_axis(x, idx_e, axis=1)
        g = _silu(x_sel @ w_gate)
        u = x_sel @ w_up
        y = g * u @ w_down
        r_sel = _sigmoid(jnp.take_along_axis(r, idx, axis=1))
        y = y * r_sel.reshape(B, C, 1)
        b_off = (jnp.arange(B) * S).reshape(B, 1)
        flat_idx = (idx + b_off).reshape(B * C)
        zero = (x * 0.0).reshape(B * S, D)
        upd = _scatter_add(zero, flat_idx, y.reshape(B * C, D), axis=0)
        return x + upd.reshape(B, S, D)
    x = A_x
    x = x + _A_ref(_layernorm(x, axis=-1), A_mem0, A_Wq, A_Wk, A_Wv, A_Wo, A_seg_len)
    x = x + _B_ref(_layernorm(x, axis=-1), B_w_r, B_w_gate, B_w_up, B_w_down)
    x = x + _A_ref(_layernorm(x, axis=-1), A_mem0, A_Wq, A_Wk, A_Wv, A_Wo, A_seg_len)
    x = x + _B_ref(_layernorm(x, axis=-1), B_w_r, B_w_gate, B_w_up, B_w_down)
    return x
```

```python
import functools

import jax
import jax.numpy as jnp
from jax import lax
import jax.experimental.pallas as pl
import jax.experimental.pallas.tpu as pltpu

F32 = jnp.float32
BF16 = jnp.bfloat16
U32 = jnp.uint32
LN_EPS = 1e-5
MASK_FILL = -1000000000.0
LANES = 128
GROUP = 4
UNROLL = 4
N_TAIL = 2


def _rb(v):
    return v.astype(BF16).astype(F32)


def _layernorm(x):
    inv_n = 1.0 / x.shape[-1]
    mean = jnp.sum(x, axis=-1, keepdims=True) * inv_n
    cen = x - mean
    var = jnp.sum(cen * cen, axis=-1, keepdims=True) * inv_n
    den = _rb(jnp.sqrt(_rb(_rb(var) + LN_EPS)))
    return _rb(_rb(x - _rb(mean)) / den)


def _mm(a, b):
    return lax.dot_general(a, b, (((1,), (0,)), ((), ())), preferred_element_type=F32)


def _mm_nt(a, b):
    return lax.dot_general(a, b, (((1,), (1,)), ((), ())), preferred_element_type=F32)


def _schedule(n_groups):
    last = n_groups - 1
    order = [("H", 0), ("Q", 1), ("S", 0), ("K", 1), ("V", 1), ("S", 1)]
    for g in range(2, n_groups):
        order += [("Q", g), ("P", g - 2), ("K", g), ("V", g), ("S", g)]
    order += [("O", 0), ("P", last - 1), ("O", 1), ("O", 2), ("P", last)]
    order += [("O", g) for g in range(3, n_groups - N_TAIL)]
    return order


def _kernel(x_hbm, mem0_ref, wq_hbm, wk_hbm, wv_hbm, wo_hbm, wr_ref, wg_hbm, wu_hbm, wd_hbm,
            out_hbm,
            xa, xb, xo, x1s, na, nb, stage, wqkv, wo, wg, wu, wd, mem, att, sems,
            *, S, D, H, Dh, M, T):
    n_seg = S // T
    L = T + M
    scale = Dh ** -0.5
    n_groups = H // GROUP
    gw = GROUP * Dh
    n_col = D // LANES
    n_chunk = 4
    dc = D // n_chunk

    x_cp = pltpu.make_async_copy(x_hbm, xa.at[pl.ds(T, S)], sems.at[0])
    x_cp.start()
    w_cps = []
    for i, w_hbm in enumerate((wq_hbm, wk_hbm, wv_hbm)):
        for c in range(n_chunk):
            rows = pl.ds(c * dc * H, dc * H)
            cp = pltpu.make_async_copy(w_hbm.at[rows], stage.at[i, rows], sems.at[5 + i * n_chunk + c])
            cp.start()
            w_cps.append(cp)
    wo_cp = pltpu.make_async_copy(wo_hbm, wo, sems.at[1])
    wo_cp.start()
    ffn_cps = [pltpu.make_async_copy(src, dst, sems.at[2 + i])
               for i, (src, dst) in enumerate(((wg_hbm, wg), (wu_hbm, wu), (wd_hbm, wd)))]

    xa[pl.ds(0, T), :] = jnp.zeros((T, D), BF16)
    att[...] = jnp.zeros((T, D), F32)
    x_cp.wait()

    def ln_body(i, carry):
        rows = pl.ds(pl.multiple_of(T + i * 128, T), 128)
        na[rows, :] = _layernorm(xa[rows, :].astype(F32))
        return carry

    lax.fori_loop(0, S // 128, ln_body, 0)

    for i in range(3):
        src = stage.at[i].bitcast(U32)
        for c in range(n_chunk):
            w_cps[i * n_chunk + c].wait()

            def relayout(b, carry, i=i, src=src):
                blk = src.at[pl.ds(pl.multiple_of(b * (8 * H), 8 * H), 8 * H)]
                rows = pl.ds(pl.multiple_of(b * 8, 8), 8)
                for j in range(H // 2):
                    even = blk[pl.ds(j, 8, stride=H), :]
                    odd = blk[pl.ds(j + H // 2, 8, stride=H), :]
                    wqkv[i, rows, pl.ds(2 * j * Dh, Dh)] = (even & 0xFFFF) | (odd << 16)
                    wqkv[i, rows, pl.ds((2 * j + 1) * Dh, Dh)] = (even >> 16) | ((odd >> 16) << 16)
                return carry

            lax.fori_loop(c * dc // 16, (c + 1) * dc // 16, relayout, 0)
    wo_cp.wait()
    for cp in ffn_cps:
        cp.start()

    qi = lax.broadcasted_iota(jnp.int32, (L, L), 0)
    ki = lax.broadcasted_iota(jnp.int32, (L, L), 1)
    allowed = (qi >= T) | (ki >= T) | (ki <= qi)
    w_r = wr_ref[...].astype(F32).reshape(1, D)
    row_id = lax.broadcasted_iota(jnp.int32, (T, 1), 0)

    def softmax(raw):
        sc = jnp.where(allowed, raw * scale, MASK_FILL)
        e = jnp.exp(sc - jnp.max(sc, axis=-1, keepdims=True))
        return e / jnp.sum(e, axis=-1, keepdims=True)

    def col(n):
        return pl.ds(n * LANES, LANES)

    def attend(n_in, s, mem_cols):
        rows = pl.ds(pl.multiple_of(T + s * T, T), T)
        h_col = lambda n: jnp.concatenate([n_in[rows, col(n)], mem_cols[n]], axis=0)
        h_all = lambda: jnp.concatenate([h_col(n) for n in range(n_col)], axis=1)
        proj = lambda i, g: _mm(h_all(), pltpu.bitcast(wqkv[i, :, pl.ds(g * gw, gw)], BF16))
        head = lambda t, i: t[:, i * Dh:(i + 1) * Dh]
        q, k, v, p, o = {}, {}, {}, {}, {}
        acc = None
        for op, g in _schedule(n_groups):
            if op == "H":
                part = [None] * 3
                for n in range(n_col):
                    for i in range(3):
                        w = wqkv[i, pl.ds(n * LANES // 2, LANES // 2), pl.ds(g * gw, gw)]
                        t = _mm(h_col(n), pltpu.bitcast(w, BF16))
                        part[i] = t if part[i] is None else part[i] + t
                q[g], k[g], v[g] = part[0], part[1].astype(BF16), part[2].astype(BF16)
            elif op == "Q":
                q[g] = proj(0, g)
            elif op == "K":
                k[g] = proj(1, g).astype(BF16)
            elif op == "V":
                v[g] = proj(2, g).astype(BF16)
            elif op == "S":
                raw = [_mm_nt(head(q[g], i), head(k[g], i)) for i in range(GROUP)]
                p[g] = [softmax(t) for t in raw]
            elif op == "P":
                o[g] = jnp.concatenate([_mm(p[g][i], head(v[g], i)) for i in range(GROUP)], axis=1)
            else:
                t = _mm(o[g], wo[pl.ds(g * gw, gw), :])
                acc = t if acc is None else acc + t
        first = n_groups - N_TAIL
        tail = jnp.concatenate([o[g] for g in range(first, n_groups)], axis=1)
        outs = [acc[:, n * LANES:(n + 1) * LANES] + _mm(tail, wo[pl.ds(first * gw, N_TAIL * gw), col(n)])
                for n in range(n_col)]
        return jnp.concatenate([t[:T] for t in outs], axis=1), [t[T:] for t in outs]

    def layer(x_in, n_in, x_out, n_out, first_layer):
        def epilogue(s, a, best, best_row):
            rows = pl.ds(pl.multiple_of(s * T, T), T)
            x1 = _rb(x_in[rows, :].astype(F32) + _rb(a))
            n1 = _layernorm(x1)
            r = _rb(jnp.sum(n1 * w_r, axis=-1, keepdims=True))
            better = (r > best) & (s > 0)
            best = jnp.where(better, r, best)
            best_row = jnp.where(better, row_id + s * T, best_row)
            x2 = (x1 + n1).astype(BF16)
            x1s[rows, :] = x1
            x_out[rows, :] = x2
            if n_out is not None:
                n_out[rows, :] = _layernorm(x2.astype(F32))
            return best, best_row

        def trip(t, carry):
            a = att[...]
            mem_cols = [mem[:, col(n)] for n in range(n_col)]
            for u in range(UNROLL):
                s = t * UNROLL + u
                carry = epilogue(s, a, *carry)
                a, mem_cols = attend(n_in, s, mem_cols)
            att[...] = a
            for n in range(n_col):
                mem[:, col(n)] = mem_cols[n]
            return carry

        mem[...] = mem0_ref[...].astype(F32)
        init = (jnp.full((T, 1), -jnp.inf, F32), jnp.full((T, 1), T, jnp.int32))
        best, best_row = lax.fori_loop(0, n_seg // UNROLL, trip, init)
        best, best_row = epilogue(n_seg, att[...], best, best_row)
        if first_layer:
            for cp in ffn_cps:
                cp.wait()

        top = jnp.max(best, axis=0, keepdims=True)
        sel = jnp.min(jnp.where(best == top, best_row, T + S - 1))
        start = pl.multiple_of(jnp.clip((sel // 16) * 16, T, T + S - 16), 16)
        rows = pl.ds(start, 16)
        x1 = x1s[rows, :]
        n1 = _layernorm(x1)
        r = _rb(jnp.sum(n1 * w_r, axis=-1, keepdims=True))
        g = _rb(_mm(n1, wg[...]))
        u = _rb(_mm(n1, wu[...]))
        y = _rb(_mm(_rb(g * jax.nn.sigmoid(g)) * u, wd[...]))
        y = _rb(y * _rb(jax.nn.sigmoid(r)))
        hit = lax.broadcasted_iota(jnp.int32, (16, 1), 0) + start == sel
        x2 = (x1 + _rb(n1 + jnp.where(hit, y, 0.0))).astype(BF16)
        x_out[rows, :] = x2
        if n_out is not None:
            n_out[rows, :] = _layernorm(x2.astype(F32))

    layer(xa, na, xb, nb, True)
    layer(xb, nb, xo, None, False)

    out_cp = pltpu.make_async_copy(xo.at[pl.ds(T, S)], out_hbm, sems.at[0])
    out_cp.start()
    out_cp.wait()


@functools.partial(jax.jit, static_argnames=("A_seg_len",))
def pallas_interleave_layers__memory_aug_recurrent_mem_tr__moe_arch_mod__prompt_kernel(
    A_x, A_mem0, A_Wq, A_Wk, A_Wv, A_Wo, A_seg_len, B_x, B_w_r, B_w_gate, B_w_up, B_w_down,
):
    del B_x
    B, S, D = A_x.shape
    _, H, Dh = A_Wq.shape
    M = A_mem0.shape[1]
    T = int(A_seg_len)
    F = B_w_gate.shape[1]
    assert B == 1 and S % (T * UNROLL) == 0 and T % 16 == 0 and M % 8 == 0 and H % GROUP == 0

    hbm = pl.BlockSpec(memory_space=pl.ANY)
    vmem = pl.BlockSpec(memory_space=pltpu.VMEM)
    out = pl.pallas_call(
        functools.partial(_kernel, S=S, D=D, H=H, Dh=Dh, M=M, T=T),
        out_shape=jax.ShapeDtypeStruct((S, D), BF16),
        in_specs=[hbm, vmem, hbm, hbm, hbm, hbm, vmem, hbm, hbm, hbm],
        out_specs=hbm,
        scratch_shapes=[
            pltpu.VMEM((T + S, D), BF16),
            pltpu.VMEM((T + S, D), BF16),
            pltpu.VMEM((T + S, D), BF16),
            pltpu.VMEM((T + S, D), F32),
            pltpu.VMEM((T + S, D), F32),
            pltpu.VMEM((T + S, D), F32),
            pltpu.VMEM((3, D * H, Dh), BF16),
            pltpu.VMEM((3, D // 2, H * Dh), U32),
            pltpu.VMEM((H * Dh, D), BF16),
            pltpu.VMEM((D, F), BF16),
            pltpu.VMEM((D, F), BF16),
            pltpu.VMEM((F, D), BF16),
            pltpu.VMEM((M, D), F32),
            pltpu.VMEM((T, D), F32),
            pltpu.SemaphoreType.DMA((17,)),
        ],
        compiler_params=pltpu.CompilerParams(vmem_limit_bytes=100 * 1024 * 1024),
    )(
        A_x.reshape(S, D), A_mem0.reshape(M, D),
        A_Wq.reshape(D * H, Dh), A_Wk.reshape(D * H, Dh), A_Wv.reshape(D * H, Dh),
        A_Wo.reshape(H * Dh, D), B_w_r, B_w_gate, B_w_up, B_w_down,
    )
    return out.reshape(B, S, D)
```

```python
import functools

import jax
import jax.numpy as jnp
from jax import lax
import jax.experimental.pallas as pl
import jax.experimental.pallas.tpu as pltpu

F32 = jnp.float32
BF16 = jnp.bfloat16
U32 = jnp.uint32
LN_EPS = 1e-5
MASK_FILL = -1000000000.0
LOG2E = 1.4426950408889634
LANES = 128
SUB = 8
GROUP = 4
CHUNK = 8
UNROLL = 4
N_TAIL = 2
N_EARLY = 7
EARLY_ROWS = 64


def _rb(v):
    return v.astype(BF16).astype(F32)


def _layernorm(x):
    inv_n = 1.0 / x.shape[-1]
    mean = jnp.sum(x, axis=-1, keepdims=True) * inv_n
    cen = x - mean
    var = jnp.sum(cen * cen, axis=-1, keepdims=True) * inv_n
    den = _rb(jnp.sqrt(_rb(_rb(var) + LN_EPS)))
    return _rb(_rb(x - _rb(mean)) / den)


def _mm(a, b):
    return lax.dot_general(a, b, (((1,), (0,)), ((), ())), preferred_element_type=F32)


def _mm_nt(a, b):
    return lax.dot_general(a, b, (((1,), (1,)), ((), ())), preferred_element_type=F32)


def _schedule(n_groups):
    last = n_groups - 1
    order = [("H", 0), ("Q", 1), ("S", 0), ("K", 1), ("V", 1), ("S", 1)]
    for g in range(2, n_groups):
        order += [("Q", g), ("P", g - 2), ("K", g), ("V", g), ("S", g)]
        if g == 3:
            order += [("E", 0)]
        if g == 5:
            order += [("E", 1)]
    order += [("O", 0), ("P", last - 1), ("O", 1), ("O", 2), ("P", last)]
    order += [("O", g) for g in range(3, n_groups - N_TAIL)]
    return order


def _kernel(x_hbm, mem0_hbm, wq_hbm, wk_hbm, wv_hbm, wo_hbm, wr_hbm, wg_hbm, wu_hbm, wd_hbm,
            out_hbm,
            xa, xb, xo, xn, xe, ne, early, stage, wqkv, wo, wg, wu, wd, mem, att, mem0_ref, wr_ref, sems, wsem, osem,
            *, S, D, H, Dh, M, T):
    n_seg = S // T
    L = T + M
    scale = Dh ** -0.5
    n_groups = H // GROUP
    gw = GROUP * Dh
    n_col = D // LANES
    per_w = H // CHUNK
    n_chunk = 3 * per_w

    w_cps = [pltpu.make_async_copy(w_hbm.at[:, pl.ds(j * CHUNK, CHUNK), :], stage.at[i * per_w + j],
                                   wsem.at[i * per_w + j])
             for i, w_hbm in enumerate((wq_hbm, wk_hbm, wv_hbm)) for j in range(per_w)]

    def wait_chunk(c):
        pltpu.make_async_copy(stage.at[c], stage.at[c], wsem.at[c]).wait()

    xe_cp = pltpu.make_async_copy(x_hbm.at[:, pl.ds(0, SUB), :], xe, sems.at[0])
    n_fill = n_chunk // 2 - 1
    cuts = [k * n_seg // (2 * n_fill - 2) for k in range(n_fill)] + [n_seg]
    x_cps = [pltpu.make_async_copy(x_hbm.at[pl.ds(lo, hi - lo)], xa.at[pl.ds(1 + lo, hi - lo)], sems.at[1])
             for lo, hi in zip(cuts[:-1], cuts[1:])]
    late_cps = [pltpu.make_async_copy(mem0_hbm, mem0_ref, sems.at[2]),
                pltpu.make_async_copy(wr_hbm, wr_ref, sems.at[3])]
    for j in range(per_w):
        rows = pl.ds(j * CHUNK * Dh, CHUNK * Dh)
        late_cps.append(pltpu.make_async_copy(wo_hbm.at[rows], wo.at[rows], sems.at[4]))
    ffn_cps = [pltpu.make_async_copy(src, dst, sems.at[5 + i])
               for i, (src, dst) in enumerate(((wg_hbm, wg), (wu_hbm, wu), (wd_hbm, wd)))]
    xe_cp.start()
    w_cps[0].start()

    def relayout(c, lo=0, size=D):
        flat = stage[c, pl.ds(lo, size)].reshape(size, CHUNK * Dh)
        wqkv[c, pl.ds(lo // 2, size // 2), :] = pltpu.bitcast(flat, U32)

    def weight(i, g, lo=0, size=D):
        j, r = divmod(g, CHUNK // GROUP)
        return pltpu.bitcast(wqkv[i * per_w + j, pl.ds(lo // 2, size // 2), pl.ds(r * gw, gw)], BF16)

    def project_early(c, fresh):
        n_rows = n_seg * SUB // EARLY_ROWS
        n_piece = CHUNK * n_rows
        size = 2 * D // n_piece
        for piece in range(n_piece):
            hd, r = divmod(piece, n_rows)
            rows, cols = pl.ds(r * EARLY_ROWS, EARLY_ROWS), pl.ds(hd * Dh, Dh)
            early[c, rows, cols] = _mm(ne[rows, :], pltpu.bitcast(wqkv[c, :, cols], BF16))
            if fresh:
                which, lo = divmod(piece * size, D)
                relayout(2 * c + which, lo, size)

    for buf in (xa, xb):
        buf[0] = jnp.zeros((T, D), BF16)
        buf[n_seg + 1] = jnp.zeros((T, D), BF16)
    att[...] = jnp.zeros((T, D), F32)

    xe_cp.wait()
    w_cps[1].start()
    ne[...] = _layernorm(xe[...].astype(F32).reshape(n_seg * SUB, D)).astype(BF16)
    wait_chunk(0)
    w_cps[2].start()
    relayout(0)

    @pl.loop(0, n_chunk // 2)
    def _(c):
        @pl.when(c > 0)
        def _():
            wait_chunk(2 * c)

        for k in range(n_chunk // 2):
            @pl.when(c == k)
            def _():
                for cp in w_cps[2 * k + 3:2 * k + 5] + (x_cps[k:k + 1] or late_cps):
                    cp.start()

        wait_chunk(2 * c + 1)
        project_early(c, True)

    @pl.loop(n_chunk // 2, N_EARLY)
    def _(c):
        project_early(c, False)

    for cp in x_cps + late_cps:
        cp.wait()
    for cp in ffn_cps:
        cp.start()

    qi = lax.broadcasted_iota(jnp.int32, (L, L), 0)
    ki = lax.broadcasted_iota(jnp.int32, (L, L), 1)
    allowed = (qi >= T) | (ki >= T) | (ki <= qi)
    w_r = wr_ref[...].astype(F32).reshape(1, D)
    row_id = lax.broadcasted_iota(jnp.int32, (T, LANES), 0)
    router = n_seg + 2

    def softmax(raw):
        sc = jnp.where(allowed, raw * (scale * LOG2E), MASK_FILL * LOG2E)
        e = jnp.exp2(sc - jnp.max(sc, axis=-1, keepdims=True))
        return e * pltpu.reciprocal(jnp.sum(e, axis=-1, keepdims=True), approx=True)

    def col(n):
        return pl.ds(n * LANES, LANES)

    def attend(s, mem_cols, n_early, side_work):
        def skip(i, g):
            return SUB if i * per_w + g * GROUP // CHUNK < n_early else 0

        def h_col(n, lo):
            return jnp.concatenate([xn[s + 1, pl.ds(lo, T - lo), col(n)], mem_cols[n]], axis=0)

        def complete(i, g, t):
            if not skip(i, g):
                return t
            j, r = divmod(g, CHUNK // GROUP)
            done = early[i * per_w + j, pl.ds(pl.multiple_of(s * SUB, SUB), SUB), pl.ds(r * gw, gw)]
            return jnp.concatenate([done, t], axis=0)

        def proj(i, g):
            h = jnp.concatenate([h_col(n, skip(i, g)) for n in range(n_col)], axis=1)
            return complete(i, g, _mm(h, weight(i, g)))

        head = lambda t, i: t[:, i * Dh:(i + 1) * Dh]
        q, k, v, p, o = {}, {}, {}, {}, {}
        acc = None
        for op, g in _schedule(n_groups):
            if op == "H":
                part = [None] * 3
                for n in range(n_col):
                    for i in range(3):
                        t = _mm(h_col(n, skip(i, g)), weight(i, g, n * LANES, LANES))
                        part[i] = t if part[i] is None else part[i] + t
                part = [complete(i, g, t) for i, t in enumerate(part)]
                q[g], k[g], v[g] = part[0], part[1].astype(BF16), part[2].astype(BF16)
            elif op == "E":
                side_work[g]()
            elif op == "Q":
                q[g] = proj(0, g)
            elif op == "K":
                k[g] = proj(1, g).astype(BF16)
            elif op == "V":
                v[g] = proj(2, g).astype(BF16)
            elif op == "S":
                raw = [_mm_nt(head(q[g], i), head(k[g], i)) for i in range(GROUP)]
                p[g] = [softmax(t) for t in raw]
            elif op == "P":
                o[g] = jnp.concatenate([_mm(p[g][i], head(v[g], i)) for i in range(GROUP)], axis=1)
            else:
                t = _mm(o[g], wo[pl.ds(g * gw, gw), :])
                acc = t if acc is None else acc + t
        first = n_groups - N_TAIL
        tail = jnp.concatenate([o[g] for g in range(first, n_groups)], axis=1)
        outs = [acc[:, n * LANES:(n + 1) * LANES] + _mm(tail, wo[pl.ds(first * gw, N_TAIL * gw), col(n)])
                for n in range(n_col)]
        return jnp.concatenate([t[:T] for t in outs], axis=1), [t[T:] for t in outs]

    def layer(x_in, x_out, first_layer):
        def normalize(slot):
            xn[slot] = _layernorm(x_in[slot].astype(F32))

        def epilogue(slot, a):
            x1 = (x_in[slot].astype(F32) + _rb(a)).astype(BF16)
            n1 = _layernorm(x1.astype(F32))
            r = _rb(jnp.sum(n1 * w_r, axis=-1, keepdims=True))
            best = xn[router, :, col(0)]
            better = (r > best) & (slot > 0)
            xn[router, :, col(0)] = jnp.where(better, r, best)
            xn[router, :, col(1)] = jnp.where(better, (row_id + slot * T).astype(F32), xn[router, :, col(1)])
            x_in[slot] = x1
            x_out[slot] = (x1.astype(F32) + n1).astype(BF16)
            xn[slot] = n1

        n_trip = n_seg // UNROLL
        n_sent = n_seg - UNROLL - 1
        if not first_layer:
            head_cp = pltpu.make_async_copy(x_out.at[pl.ds(1, n_sent)], out_hbm.at[pl.ds(0, n_sent)],
                                            osem.at[0])

        normalize(1)
        mem[...] = mem0_ref[...].astype(F32)
        xn[router, :, col(0)] = jnp.full((T, LANES), -jnp.inf, F32)
        xn[router, :, col(1)] = jnp.full((T, LANES), T, F32)

        @pl.loop(0, n_trip)
        def _(t):
            if not first_layer:
                pl.when(t == n_trip - 1)(head_cp.start)
            a = att[...]
            mem_cols = [mem[:, col(n)] for n in range(n_col)]
            for u in range(UNROLL):
                s = t * UNROLL + u
                side = (functools.partial(epilogue, s, a), functools.partial(normalize, s + 2))
                a, mem_cols = attend(s, mem_cols, N_EARLY if first_layer else 0, side)
            att[...] = a
            for n in range(n_col):
                mem[:, col(n)] = mem_cols[n]

        epilogue(n_seg, att[...])
        best, best_row = xn[router, :, col(0)], xn[router, :, col(1)]
        if first_layer:
            for cp in ffn_cps:
                cp.wait()
        else:
            tail_cp = pltpu.make_async_copy(x_out.at[pl.ds(1 + n_sent, n_seg - n_sent)],
                                            out_hbm.at[pl.ds(n_sent, n_seg - n_sent)], osem.at[1])
            tail_cp.start()

        top = jnp.max(best, axis=0, keepdims=True)
        sel = jnp.min(jnp.where(best == top, best_row, T + S - 1), axis=0, keepdims=True)
        sel = sel.astype(jnp.int32)[0, 0]
        slot = jnp.clip(sel // T, 1, n_seg)
        n1 = xn[slot]
        g = _rb(_mm(n1, wg[...]))
        u = _rb(_mm(n1, wu[...]))
        y = _rb(_mm(_rb(g * jax.nn.sigmoid(g)) * u, wd[...]))
        y = _rb(y * _rb(jax.nn.sigmoid(top[:, :1])))
        hit = lax.broadcasted_iota(jnp.int32, (T, D), 0) + slot * T == sel
        x2 = (x_in[slot].astype(F32) + _rb(n1 + jnp.where(hit, y, 0.0))).astype(BF16)
        if first_layer:
            x_out[slot] = x2
        else:
            x_out[0] = x2
            head_cp.wait()
            tail_cp.wait()
            fix_cp = pltpu.make_async_copy(x_out.at[0], out_hbm.at[slot - 1], osem.at[0])
            fix_cp.start()
            fix_cp.wait()

    layer(xa, xb, True)
    layer(xb, xo, False)


@functools.partial(jax.jit, static_argnames=("A_seg_len",))
def pallas_interleave_layers__memory_aug_recurrent_mem_tr__moe_arch_mod__prompt_kernel(
    A_x, A_mem0, A_Wq, A_Wk, A_Wv, A_Wo, A_seg_len, B_x, B_w_r, B_w_gate, B_w_up, B_w_down,
):
    del B_x
    B, S, D = A_x.shape
    _, H, Dh = A_Wq.shape
    M = A_mem0.shape[1]
    T = int(A_seg_len)
    F = B_w_gate.shape[1]
    assert B == 1 and S % (T * UNROLL) == 0 and T % 16 == 0 and M % SUB == 0 and H % CHUNK == 0
    n_seg = S // T
    n_chunk = 3 * H // CHUNK

    hbm = pl.BlockSpec(memory_space=pl.ANY)
    out = pl.pallas_call(
        functools.partial(_kernel, S=S, D=D, H=H, Dh=Dh, M=M, T=T),
        out_shape=jax.ShapeDtypeStruct((n_seg, T, D), BF16),
        in_specs=[hbm] * 10,
        out_specs=hbm,
        scratch_shapes=[
            pltpu.VMEM((n_seg + 2, T, D), BF16),
            pltpu.VMEM((n_seg + 2, T, D), BF16),
            pltpu.VMEM((n_seg + 1, T, D), BF16),
            pltpu.VMEM((n_seg + 3, T, D), F32),
            pltpu.VMEM((n_seg, SUB, D), BF16),
            pltpu.VMEM((n_seg * SUB, D), BF16),
            pltpu.VMEM((N_EARLY, n_seg * SUB, CHUNK * Dh), F32),
            pltpu.VMEM((n_chunk, D, CHUNK, Dh), BF16),
            pltpu.VMEM((n_chunk, D // 2, CHUNK * Dh), U32),
            pltpu.VMEM((H * Dh, D), BF16),
            pltpu.VMEM((D, F), BF16),
            pltpu.VMEM((D, F), BF16),
            pltpu.VMEM((F, D), BF16),
            pltpu.VMEM((M, D), F32),
            pltpu.VMEM((T, D), F32),
            pltpu.VMEM((M, D), BF16),
            pltpu.VMEM((D,), BF16),
            pltpu.SemaphoreType.DMA((8,)),
            pltpu.SemaphoreType.DMA((n_chunk,)),
            pltpu.SemaphoreType.DMA((2,)),
        ],
        compiler_params=pltpu.CompilerParams(vmem_limit_bytes=100 * 1024 * 1024),
    )(
        A_x.reshape(n_seg, T, D), A_mem0.reshape(M, D), A_Wq, A_Wk, A_Wv,
        A_Wo.reshape(H * Dh, D), B_w_r, B_w_gate, B_w_up, B_w_down,
    )
    return out.reshape(B, S, D)
```

```python
import functools

import jax
import jax.numpy as jnp
from jax import lax
import jax.experimental.pallas as pl
import jax.experimental.pallas.tpu as pltpu

F32 = jnp.float32
BF16 = jnp.bfloat16
U32 = jnp.uint32
LN_EPS = 1e-5
LOG2E = 1.4426950408889634
MASK_FILL = -1000000000.0 * LOG2E
LANES = 128
SUB = 8
PACK = 16
GROUP = 4
CHUNK = 8
UNROLL = 4
N_EARLY = 7
EARLY_ROWS = 64
LAG = 5
TIMING = ((4, 20, 14, 3.67, 3, 125, 3, 132), (6, 16, 10, 3.74, 1, 128, 125, 131))


def _rb(v):
    return v.astype(BF16).astype(F32)


def _layernorm(x):
    inv_n = 1.0 / x.shape[-1]
    mean = jnp.sum(x, axis=-1, keepdims=True) * inv_n
    cen = x - mean
    var = jnp.sum(cen * cen, axis=-1, keepdims=True) * inv_n
    den = _rb(jnp.sqrt(_rb(_rb(var) + LN_EPS)))
    return _rb(_rb(x - _rb(mean)) / den)


def _mm(a, b):
    return lax.dot_general(a, b, (((1,), (0,)), ((), ())), preferred_element_type=F32)


def _mm_nt(a, b):
    return lax.dot_general(a, b, (((1,), (1,)), ((), ())), preferred_element_type=F32)


def _schedule(n_heads, n_col, timing):
    score_at, value_at, start, period, *side_at = timing
    n_groups = n_heads // GROUP
    slots = [("first", n) for n in range(n_col)]
    slots += [("proj", (i, h)) for h in range(n_heads) for i in range(3) if i or h >= GROUP]
    for groups in (range(n_groups - 2), range(n_groups - 2, n_groups)):
        slots += [("out", (g, n)) for n in range(n_col) for g in groups]
    extra = {}
    for g in range(n_groups):
        extra.setdefault(3 * GROUP * (g + 1) + score_at, []).append(("score", g))
        extra.setdefault(3 * GROUP * (g + 1) + value_at, []).append(("value", g))
    slots = [op for t, slot in enumerate(slots) for op in extra.get(t, []) + [slot]]
    order, window = [], 0
    todo = sorted((t + dt, (kind, j)) for j, t in enumerate(side_at)
                  for dt, kind in ((0, "side"), (13, "done")))
    for t, slot in enumerate(slots):
        if slot[0] not in ("score", "value"):
            while todo and todo[0][0] <= t:
                order.append(todo.pop(0)[1])
            while window < n_heads + 2 and start + window * period <= t:
                order.append(("window", window))
                window += 1
        order.append(slot)
    return order + [op for _, op in todo]


def _kernel(x_hbm, mem0_hbm, wq_hbm, wk_hbm, wv_hbm, wo_hbm, wr_hbm, wg_hbm, wu_hbm, wd_hbm,
            out_hbm,
            xa, xb, xo, routed, xe, ne, early, stage, wqkv, wo, wg, wu, wd, mem0, wr,
            att, tok, qkv, prob, head_out, paced, sems, wsem, osem,
            *, S, D, H, Dh, M, T):
    n_seg = S // T
    L = M + T
    rest = T - SUB
    scale = Dh ** -0.5 * LOG2E
    gw = GROUP * Dh
    n_col = D // LANES
    per_w = H // CHUNK
    n_chunk = 3 * per_w

    w_cps = [pltpu.make_async_copy(w_hbm.at[:, pl.ds(j * CHUNK, CHUNK), :], stage.at[i * per_w + j],
                                   wsem.at[i * per_w + j])
             for i, w_hbm in enumerate((wq_hbm, wk_hbm, wv_hbm)) for j in range(per_w)]

    def wait_chunk(c):
        pltpu.make_async_copy(stage.at[c], stage.at[c], wsem.at[c]).wait()

    xe_cp = pltpu.make_async_copy(x_hbm.at[:, pl.ds(0, SUB), :], xe, sems.at[0])
    x_cps = [pltpu.make_async_copy(x_hbm.at[pl.ds(lo, hi - lo)], xa.at[pl.ds(1 + lo, hi - lo)], sems.at[1])
             for lo, hi in ((0, UNROLL + 1), (UNROLL + 1, n_seg))]
    late_cps = []
    for j in range(per_w):
        late_cps.append(pltpu.make_async_copy(wo_hbm.bitcast(U32).at[:, pl.ds(j * LANES, LANES)], wo.at[j], sems.at[2]))
    late_cps += [pltpu.make_async_copy(mem0_hbm, mem0, sems.at[3]),
                 pltpu.make_async_copy(wr_hbm, wr, sems.at[4])]
    batches = [w_cps[2 * k + 3:2 * k + 5] for k in range(n_chunk // 2)]
    batches[-2] += x_cps[:1]
    batches[-1] += late_cps
    ffn_cps = [pltpu.make_async_copy(src, dst, sems.at[5 + i])
               for i, (src, dst) in enumerate(((wg_hbm, wg), (wu_hbm, wu), (wd_hbm, wd)))]
    xe_cp.start()
    w_cps[0].start()

    def relayout(c, lo=0, size=D):
        flat = stage[c, pl.ds(lo, size)].reshape(size, CHUNK * Dh)
        for j in range(CHUNK):
            wqkv[c, j, pl.ds(lo // 2, size // 2), :] = pltpu.bitcast(flat[:, j * Dh:(j + 1) * Dh], U32)

    def project_early(c, fresh):
        n_rows = n_seg * SUB // EARLY_ROWS
        n_piece = CHUNK * n_rows
        size = 2 * D // n_piece
        for piece in range(n_piece):
            hd, r = divmod(piece, n_rows)
            rows, cols = pl.ds(r * EARLY_ROWS, EARLY_ROWS), pl.ds(hd * Dh, Dh)
            lhs = pltpu.bitcast(ne[pl.ds(r * EARLY_ROWS // 2, EARLY_ROWS // 2), :], BF16)
            early[c, rows, cols] = _mm(lhs, pltpu.bitcast(wqkv[c, hd], BF16))
            if fresh:
                which, lo = divmod(piece * size, D)
                relayout(2 * c + which, lo, size)

    MEM, SCALE, BEST, WHERE, MARK, HEAD = range(6)

    def col(n, width=LANES):
        return pl.ds(n * width, width)

    for buf in (xa, xb):
        buf[0] = jnp.zeros((T, D), BF16)
        buf[n_seg + 1] = jnp.zeros((T, D), BF16)
    att[...] = jnp.zeros((T, D), F32)
    paced[SCALE] = jnp.full((SUB, D), scale, F32)

    xe_cp.wait()
    w_cps[1].start()
    ne[...] = pltpu.bitcast(_layernorm(xe[...].astype(F32).reshape(n_seg * SUB, D)).astype(BF16), U32)
    wait_chunk(0)
    relayout(0)
    w_cps[2].start()

    @pl.loop(0, n_chunk // 2)
    def _(c):
        wait_chunk(2 * c + 1)
        for k, batch in enumerate(batches):
            @pl.when(c == k)
            def _():
                for cp in batch:
                    cp.start()

        @pl.when(c > 0)
        def _():
            wait_chunk(2 * c)

        project_early(c, True)

    x_cps[0].wait()
    tok[0][0] = _layernorm(xa[1].astype(F32))

    @pl.loop(n_chunk // 2, N_EARLY)
    def _(c):
        project_early(c, False)

    for cp in late_cps:
        cp.wait()
    for cp in x_cps[1:] + ffn_cps:
        cp.start()

    w_r = wr[...].astype(F32).reshape(1, D)

    def softmax(raw):
        qi = lax.broadcasted_iota(jnp.int32, raw.shape, 0)
        ki = lax.broadcasted_iota(jnp.int32, raw.shape, 1)
        sc = jnp.where((qi < M) | (ki <= qi + SUB), raw * scale, MASK_FILL)
        e = jnp.exp2(sc - jnp.max(sc, axis=-1, keepdims=True))
        return e * pltpu.reciprocal(jnp.sum(e, axis=-1, keepdims=True), approx=True)

    def rolled(blocks):
        return [pltpu.roll(b, d, 0) if d else b for b in blocks for d in range(SUB)]

    def attend(s, parity, zero, n_early, timing, side_work):
        def is_early(i, h):
            return i * per_w + h // CHUNK < n_early

        def lhs(i, h, cols):
            lo = SUB if is_early(i, h) else 0
            return jnp.concatenate([paced[MEM, :, cols], tok[parity][0, pl.ds(lo, T - lo), cols]], axis=0)

        def weight(i, h, n_head=1, lo=0, size=D):
            w = [wqkv[i * per_w + h // CHUNK, h % CHUNK + j, pl.ds(lo // 2, size // 2), :] for j in range(n_head)]
            return pltpu.bitcast(jnp.concatenate(w, axis=1), BF16)

        def keep(i, h, t):
            cols = pl.ds(h % GROUP * Dh, t.shape[1])
            qkv[i][h // GROUP][zero, pl.ds(0, M), cols] = t[:M]
            qkv[i][h // GROUP][zero, pl.ds(M + L - t.shape[0], t.shape[0] - M), cols] = t[M:]

        def rows_of(i, h):
            buf, cols = qkv[i][h // GROUP], col(h % GROUP, Dh)
            if is_early(i, h):
                front = early[i * per_w + h // CHUNK, pl.ds(pl.multiple_of(s * SUB, SUB), SUB),
                              col(h % CHUNK, Dh)]
            else:
                front = buf[0, pl.ds(M, SUB), cols]
            return buf[0, pl.ds(0, M), cols], front, buf[0, pl.ds(M + SUB, rest), cols]

        def front_scores(h):
            q = rows_of(0, h)[1] * paced[SCALE, :, col(0)]
            sub = lax.broadcasted_iota(jnp.int32, q.shape, 0)
            out = []
            for j, k in enumerate(rolled(rows_of(1, h)[:2])):
                sc = jnp.broadcast_to(jnp.sum(q * k, axis=-1, keepdims=True), q.shape)
                out.append(jnp.where(sub >= j - M, sc, MASK_FILL) if j > M else sc)
            return out

        def front_values(h, scores):
            top = functools.reduce(jnp.maximum, scores)
            num = den = None
            for sc, v in zip(scores, rolled(rows_of(2, h)[:2])):
                e = jnp.exp2(sc - top)
                num, den = (e * v, e) if num is None else (num + e * v, den + e)
            return num * pltpu.reciprocal(den, approx=True)

        first, acc, scores, front, finish, marks = None, [None] * n_col, {}, {}, {}, []
        for op, arg in _schedule(H, n_col, timing):
            if op == "first":
                part = _mm(lhs(0, 0, col(arg)), weight(0, 0, GROUP, arg * LANES, LANES))
                first = part + 0.0 if first is None else first + part
                if arg == n_col - 1:
                    keep(0, 0, first)
            elif op == "proj":
                if len(marks) >= LAG:
                    tok[parity][zero + 1, pl.ds(0, SUB), col(0)] = marks[-LAG]
                part = _mm(lhs(*arg, col(0, D)), weight(*arg))
                keep(*arg, part)
                marks.append(part[-SUB:])
            elif op == "score":
                raw = []
                for h in range(arg * GROUP, (arg + 1) * GROUP):
                    q = jnp.concatenate(rows_of(0, h)[::2], axis=0)
                    raw.append(_mm_nt(q, jnp.concatenate(rows_of(1, h), axis=0).astype(BF16)))
                for j, r in enumerate(raw):
                    prob[arg][zero + j] = softmax(r)
            elif op == "value":
                for j in range(GROUP):
                    v = jnp.concatenate(rows_of(2, arg * GROUP + j), axis=0).astype(BF16)
                    head_out[arg][zero, :, col(j, Dh)] = _mm(prob[arg][j], v)
            elif op == "out":
                g, n = arg
                assert (g + 1) * GROUP - 1 not in front and (g + 1) * GROUP - 1 in scores
                if n:
                    head_out[g][zero + 1, pl.ds(0, SUB), col(0)] = marks[-LAG]
                o = jnp.concatenate([head_out[g][0, pl.ds(0, M), :], paced[HEAD + g],
                                     head_out[g][0, pl.ds(M, rest), :]], axis=0)
                part = _mm(o, pltpu.bitcast(wo[n, col(g, gw // 2), :], BF16))
                acc[n] = part + 0.0 if acc[n] is None else acc[n] + part
                marks.append(acc[n][-SUB:])
            elif op == "window":
                if arg >= 2:
                    paced[zero + HEAD + (arg - 2) // GROUP, :, col((arg - 2) % GROUP, Dh)] = front.pop(arg - 2)
                if arg < H:
                    scores[arg] = front_scores(arg)
                if 1 <= arg <= H:
                    front[arg - 1] = front_values(arg - 1, scores[arg - 1])
            elif op == "side":
                finish[arg] = side_work[arg]()
            else:
                finish[arg]()
        for n in range(n_col):
            paced[MEM, :, col(n)] = acc[n][:M]
            att[:, col(n)] = acc[n][M:]

    def layer(x_in, x_out, first_layer):
        def normalize(slot, parity, zero, half):
            rows = pl.ds(half * PACK, PACK)
            n = _layernorm(x_in[slot, rows, :].astype(F32))
            tok[parity][zero, rows, :] = n

            def finish():
                paced[zero + MARK, :, col(0)] = n[-SUB:, -LANES:]
            return finish

        def epilogue(slot, zero, half):
            rows = pl.ds(half * PACK, PACK)
            a = att[rows, :]
            x1 = (x_in[slot, rows, :].astype(F32) + _rb(a)).astype(BF16)
            n1 = _layernorm(x1.astype(F32))
            r = _rb(jnp.sum(n1 * w_r, axis=-1, keepdims=True))
            x_in[slot, rows, :] = x1
            x_out[slot, rows, :] = (x1.astype(F32) + n1).astype(BF16)
            routed[slot, rows, :] = n1

            def finish():
                best, where = paced[BEST, :, col(0)], paced[WHERE, :, col(0)]
                for j in range(PACK // SUB):
                    score = r[j * SUB:(j + 1) * SUB]
                    row = lax.broadcasted_iota(jnp.int32, best.shape, 0) + (slot * T + half * PACK + j * SUB)
                    better = (score > best) & (slot > 0)
                    best, where = jnp.where(better, score, best), jnp.where(better, row.astype(F32), where)
                paced[zero + BEST, :, col(0)] = best
                paced[zero + WHERE, :, col(0)] = where
            return finish

        n_trip = n_seg // UNROLL
        n_sent = n_seg - UNROLL - 1
        if not first_layer:
            head_cp = pltpu.make_async_copy(x_out.at[pl.ds(1, n_sent)], out_hbm.at[pl.ds(0, n_sent)],
                                            osem.at[0])
        paced[MEM] = mem0[...].astype(F32)
        paced[BEST, :, col(0)] = jnp.full((SUB, LANES), -jnp.inf, F32)
        paced[WHERE, :, col(0)] = jnp.full((SUB, LANES), T, F32)

        @pl.loop(0, n_trip)
        def _(t):
            if first_layer:
                pl.when(t == 1)(x_cps[1].wait)
            else:
                pl.when(t == n_trip - 1)(head_cp.start)
            zero = lax.shift_right_logical(t, 16)
            for u in range(UNROLL):
                s = t * UNROLL + u
                side = [functools.partial(epilogue, s, zero, half) for half in range(T // PACK)]
                side += [functools.partial(normalize, s + 2, (u + 1) % 2, zero, half) for half in range(T // PACK)]
                attend(s, u % 2, zero, N_EARLY if first_layer else 0, TIMING[not first_layer], side)

        for finish in [epilogue(n_seg, 0, half) for half in range(T // PACK)]:
            finish()
        if first_layer:
            for cp in ffn_cps:
                cp.wait()
        else:
            tail_cp = pltpu.make_async_copy(x_out.at[pl.ds(1 + n_sent, n_seg - n_sent)],
                                            out_hbm.at[pl.ds(n_sent, n_seg - n_sent)], osem.at[1])
            tail_cp.start()

        best, where = paced[BEST, :, col(0)], paced[WHERE, :, col(0)]
        top = jnp.max(best, axis=0, keepdims=True)
        sel = jnp.min(jnp.where(best == top, where, T + S - 1), axis=0, keepdims=True)
        sel = sel.astype(jnp.int32)[0, 0]
        slot = jnp.clip(sel // T, 1, n_seg)
        n1 = routed[slot]
        g = _rb(_mm(n1, wg[...]))
        u = _rb(_mm(n1, wu[...]))
        y = _rb(_mm(_rb(g * jax.nn.sigmoid(g)) * u, wd[...]))
        y = _rb(y * _rb(jax.nn.sigmoid(top[:, :1])))
        hit = lax.broadcasted_iota(jnp.int32, (T, D), 0) + slot * T == sel
        x2 = (x_in[slot].astype(F32) + _rb(n1 + jnp.where(hit, y, 0.0))).astype(BF16)
        if first_layer:
            ahead = _layernorm(x_out[1].astype(F32))
            x_out[slot] = x2
            tok[0][0] = ahead

            @pl.when(slot == 1)
            def _():
                tok[0][0] = _layernorm(x2.astype(F32))
        else:
            x_out[0] = x2
            head_cp.wait()
            tail_cp.wait()
            fix_cp = pltpu.make_async_copy(x_out.at[0], out_hbm.at[slot - 1], osem.at[0])
            fix_cp.start()
            fix_cp.wait()

    layer(xa, xb, True)
    layer(xb, xo, False)


@functools.partial(jax.jit, static_argnames=("A_seg_len",))
def pallas_interleave_layers__memory_aug_recurrent_mem_tr__moe_arch_mod__prompt_kernel(
    A_x, A_mem0, A_Wq, A_Wk, A_Wv, A_Wo, A_seg_len, B_x, B_w_r, B_w_gate, B_w_up, B_w_down,
):
    del B_x
    B, S, D = A_x.shape
    _, H, Dh = A_Wq.shape
    M = A_mem0.shape[1]
    T = int(A_seg_len)
    F = B_w_gate.shape[1]
    assert B == 1 and S % (T * UNROLL) == 0 and T == 2 * PACK and M == SUB
    assert H % CHUNK == 0 and Dh == LANES and D == GROUP * Dh
    n_seg = S // T
    n_chunk = 3 * H // CHUNK
    n_groups = H // GROUP

    hbm = pl.BlockSpec(memory_space=pl.ANY)
    out = pl.pallas_call(
        functools.partial(_kernel, S=S, D=D, H=H, Dh=Dh, M=M, T=T),
        out_shape=jax.ShapeDtypeStruct((n_seg, T, D), BF16),
        in_specs=[hbm] * 10,
        out_specs=hbm,
        scratch_shapes=[
            pltpu.VMEM((n_seg + 2, T, D), BF16),
            pltpu.VMEM((n_seg + 2, T, D), BF16),
            pltpu.VMEM((n_seg + 1, T, D), BF16),
            pltpu.VMEM((n_seg + 1, T, D), F32),
            pltpu.VMEM((n_seg, SUB, D), BF16),
            pltpu.VMEM((n_seg * SUB // 2, D), U32),
            pltpu.VMEM((N_EARLY, n_seg * SUB, CHUNK * Dh), F32),
            pltpu.VMEM((n_chunk, D, CHUNK, Dh), BF16),
            pltpu.VMEM((n_chunk, CHUNK, D // 2, Dh), U32),
            pltpu.VMEM((D // LANES, H * Dh // 2, LANES), U32),
            pltpu.VMEM((D, F), BF16),
            pltpu.VMEM((D, F), BF16),
            pltpu.VMEM((F, D), BF16),
            pltpu.VMEM((M, D), BF16),
            pltpu.VMEM((D,), BF16),
            pltpu.VMEM((T, D), F32),
            [pltpu.VMEM((2, T, D), F32)] * 2,
            [[pltpu.VMEM((2, M + T, GROUP * Dh), F32)] * n_groups] * 3,
            [pltpu.VMEM((GROUP, M + T - SUB, M + T), F32)] * n_groups,
            [pltpu.VMEM((2, M + T - SUB, GROUP * Dh), F32)] * n_groups,
            pltpu.VMEM((5 + n_groups, SUB, D), F32),
            pltpu.SemaphoreType.DMA((8,)),
            pltpu.SemaphoreType.DMA((n_chunk,)),
            pltpu.SemaphoreType.DMA((2,)),
        ],
        compiler_params=pltpu.CompilerParams(vmem_limit_bytes=100 * 1024 * 1024),
    )(
        A_x.reshape(n_seg, T, D), A_mem0.reshape(M, D), A_Wq, A_Wk, A_Wv,
        A_Wo.reshape(H * Dh, D), B_w_r, B_w_gate, B_w_up, B_w_down,
    )
    return out.reshape(B, S, D)
```

```python
import functools

import jax
import jax.numpy as jnp
from jax import lax
import jax.experimental.pallas as pl
import jax.experimental.pallas.tpu as pltpu

F32 = jnp.float32
BF16 = jnp.bfloat16
U32 = jnp.uint32
LN_EPS = 1e-5
LOG2E = 1.4426950408889634
MASK_FILL = -1000000000.0 * LOG2E
LANES = 128
SUB = 8
PACK = 16
GROUP = 4
CHUNK = 8
UNROLL = 4
EARLY_ROWS = 64
LAG = 5
TIMING = ((4, 18, 15, 3.52, 8, 125, 127, 132), (6, 16, 10, 3.74, 1, 128, 125, 131))


def _rb(v):
    return v.astype(BF16).astype(F32)


def _layernorm(x):
    inv_n = 1.0 / x.shape[-1]
    mean = jnp.sum(x, axis=-1, keepdims=True) * inv_n
    cen = x - mean
    var = jnp.sum(cen * cen, axis=-1, keepdims=True) * inv_n
    den = _rb(jnp.sqrt(_rb(_rb(var) + LN_EPS)))
    return _rb(_rb(x - _rb(mean)) / den)


def _mm(a, b):
    return lax.dot_general(a, b, (((1,), (0,)), ((), ())), preferred_element_type=F32)


def _mm_nt(a, b):
    return lax.dot_general(a, b, (((1,), (1,)), ((), ())), preferred_element_type=F32)


def _schedule(n_heads, n_col, timing):
    score_at, value_at, start, period, *side_at = timing
    n_groups = n_heads // GROUP
    slots = [("first", n) for n in range(n_col)]
    slots += [("proj", (i, h)) for h in range(n_heads) for i in range(3) if i or h >= GROUP]
    for groups in (range(n_groups - 2), range(n_groups - 2, n_groups)):
        slots += [("out", (g, n)) for n in range(n_col) for g in groups]
    extra = {}
    for g in range(n_groups):
        extra.setdefault(3 * GROUP * (g + 1) + score_at, []).append(("score", g))
        extra.setdefault(min(3 * GROUP * (g + 1) + value_at, len(slots) - n_col * 2 - 3), []).append(("value", g))
    slots = [op for t, slot in enumerate(slots) for op in extra.get(t, []) + [slot]]
    order, window = [], 0
    todo = sorted((t + dt, (kind, j)) for j, t in enumerate(side_at)
                  for dt, kind in ((0, "side"), (13, "done")))
    for t, slot in enumerate(slots):
        if slot[0] not in ("score", "value"):
            while todo and todo[0][0] <= t:
                order.append(todo.pop(0)[1])
            while window < n_heads + 2 and start + window * period <= t:
                order.append(("window", window))
                window += 1
        order.append(slot)
    return order + [op for _, op in todo]


def _kernel(x_hbm, mem0_hbm, wq_hbm, wk_hbm, wv_hbm, wo_hbm, wr_hbm, wg_hbm, wu_hbm, wd_hbm,
            out_hbm,
            xa, xb, xo, routed, xe, ne, early, raw_qkv, raw_out, tiles, wg, wu, wd, mem0, wr,
            att, tok, qkv, prob, head_out, paced, sems, wsem, osem,
            *, S, D, H, Dh, M, T):
    n_seg = S // T
    L = M + T
    rest = T - SUB
    scale = Dh ** -0.5 * LOG2E
    gw = GROUP * Dh
    n_col = D // LANES
    per_w = H // CHUNK
    n_qkv = 3 * per_w
    n_early = 2 * per_w

    w_cps = [pltpu.make_async_copy(w_hbm.at[:, pl.ds(j * CHUNK, CHUNK), :], raw_qkv.at[i * per_w + j],
                                   wsem.at[i * per_w + j])
             for i, w_hbm in enumerate((wq_hbm, wk_hbm, wv_hbm)) for j in range(per_w)]
    w_cps += [pltpu.make_async_copy(wo_hbm.at[j], raw_out.at[j], wsem.at[n_qkv + j]) for j in range(per_w)]
    xe_cp = pltpu.make_async_copy(x_hbm.at[:, pl.ds(0, SUB), :], xe, sems.at[0])
    x_cps = [pltpu.make_async_copy(x_hbm.at[pl.ds(lo, hi - lo)], xa.at[pl.ds(1 + lo, hi - lo)], sems.at[1 + i])
             for i, (lo, hi) in enumerate(((0, UNROLL + 1), (UNROLL + 1, n_seg)))]
    small_cps = x_cps[:1] + [pltpu.make_async_copy(mem0_hbm, mem0, sems.at[3]),
                             pltpu.make_async_copy(wr_hbm, wr, sems.at[4])]
    ffn_cps = [pltpu.make_async_copy(src, dst, sems.at[5 + i])
               for i, (src, dst) in enumerate(((wg_hbm, wg), (wu_hbm, wu), (wd_hbm, wd)))]
    batches = [w_cps[2 * c + 3:2 * c + 5] for c in range(n_early)]
    batches[-2] += small_cps
    batches[-1] += x_cps[1:]
    xe_cp.start()
    w_cps[0].start()

    def repack_qkv(c, lo=0, size=D):
        flat = raw_qkv[c, pl.ds(lo, size)].reshape(size, CHUNK * Dh)
        for j in range(CHUNK):
            tiles[c, j, pl.ds(lo // 2, size // 2), :] = pltpu.bitcast(flat[:, j * Dh:(j + 1) * Dh], U32)

    def repack_out(c, lo, size):
        for j in range(CHUNK):
            g, n = divmod(j, n_col)
            w = raw_out[c - n_qkv, pl.ds(g * gw + lo, size), pl.ds(n * LANES, LANES)]
            tiles[c, j, pl.ds(lo // 2, size // 2), :] = pltpu.bitcast(w, U32)

    def load_trips(lo, hi, raw, repack):
        def wait(c):
            pltpu.make_async_copy(raw.at[c - 2 * lo], raw.at[c - 2 * lo], wsem.at[c]).wait()

        @pl.loop(lo, hi)
        def _(c):
            wait(2 * c + 1)
            for k in range(lo, hi):
                @pl.when(c == k)
                def _():
                    for cp in batches[k]:
                        cp.start()

            pl.when(c > 0)(functools.partial(wait, 2 * c))
            n_rows = n_seg * SUB // EARLY_ROWS
            size = 2 * D // (CHUNK * n_rows)
            for piece in range(CHUNK * n_rows):
                j, r = divmod(piece, n_rows)
                lhs = pltpu.bitcast(ne[pl.ds(r * EARLY_ROWS // 2, EARLY_ROWS // 2), :], BF16)
                early[c, j, pl.ds(r * EARLY_ROWS, EARLY_ROWS), :] = _mm(lhs, pltpu.bitcast(tiles[c, j], BF16))
                which, row = divmod(piece * size, D)
                repack(2 * c + which, row, size)

    MEM, SCALE, BEST, WHERE, MARK, HEAD = range(6)

    def col(n, width=LANES):
        return pl.ds(n * width, width)

    for buf in (xa, xb):
        buf[0] = jnp.zeros((T, D), BF16)
        buf[n_seg + 1] = jnp.zeros((T, D), BF16)
    att[...] = jnp.zeros((T, D), F32)
    paced[SCALE] = jnp.full((SUB, D), scale, F32)

    xe_cp.wait()
    w_cps[1].start()
    ne[...] = pltpu.bitcast(_layernorm(xe[...].astype(F32).reshape(n_seg * SUB, D)).astype(BF16), U32)
    w_cps[0].wait()
    repack_qkv(0)
    w_cps[2].start()
    load_trips(0, n_qkv // 2, raw_qkv, repack_qkv)
    load_trips(n_qkv // 2, n_early, raw_out, repack_out)
    for cp in small_cps:
        cp.wait()
    for cp in ffn_cps:
        cp.start()
    tok[0][0] = _layernorm(xa[1].astype(F32))

    w_r = wr[...].astype(F32).reshape(1, D)

    def softmax(raw):
        qi = lax.broadcasted_iota(jnp.int32, raw.shape, 0)
        ki = lax.broadcasted_iota(jnp.int32, raw.shape, 1)
        sc = jnp.where((qi < M) | (ki <= qi + SUB), raw * scale, MASK_FILL)
        e = jnp.exp2(sc - jnp.max(sc, axis=-1, keepdims=True))
        return e * pltpu.reciprocal(jnp.sum(e, axis=-1, keepdims=True), approx=True)

    def rolled(blocks):
        return [pltpu.roll(b, d, 0) if d else b for b in blocks for d in range(SUB)]

    def attend(s, parity, zero, use_early, timing, side_work):
        def is_early(i, h):
            return use_early and i * per_w + h // CHUNK < n_early

        def lhs(i, h, cols):
            lo = SUB if is_early(i, h) else 0
            return jnp.concatenate([paced[MEM, :, cols], tok[parity][0, pl.ds(lo, T - lo), cols]], axis=0)

        def weight(i, h, n_head=1, lo=0, size=D):
            w = [tiles[i * per_w + h // CHUNK, h % CHUNK + j, pl.ds(lo // 2, size // 2), :] for j in range(n_head)]
            return pltpu.bitcast(jnp.concatenate(w, axis=1), BF16)

        def keep(i, h, t):
            cols = pl.ds(h % GROUP * Dh, t.shape[1])
            qkv[i][h // GROUP][zero, pl.ds(0, M), cols] = t[:M]
            qkv[i][h // GROUP][zero, pl.ds(M + L - t.shape[0], t.shape[0] - M), cols] = t[M:]

        def rows_of(i, h):
            buf, cols = qkv[i][h // GROUP], col(h % GROUP, Dh)
            if is_early(i, h):
                front = early[i * per_w + h // CHUNK, h % CHUNK, pl.ds(pl.multiple_of(s * SUB, SUB), SUB), :]
            else:
                front = buf[0, pl.ds(M, SUB), cols]
            return buf[0, pl.ds(0, M), cols], front, buf[0, pl.ds(M + SUB, rest), cols]

        def front_scores(h):
            q = rows_of(0, h)[1] * paced[SCALE, :, col(0)]
            sub = lax.broadcasted_iota(jnp.int32, q.shape, 0)
            out = []
            for j, k in enumerate(rolled(rows_of(1, h)[:2])):
                sc = jnp.broadcast_to(jnp.sum(q * k, axis=-1, keepdims=True), q.shape)
                out.append(jnp.where(sub >= j - M, sc, MASK_FILL) if j > M else sc)
            return out

        def front_values(h, scores):
            top = functools.reduce(jnp.maximum, scores)
            num = den = None
            for sc, v in zip(scores, rolled(rows_of(2, h)[:2])):
                e = jnp.exp2(sc - top)
                num, den = (e * v, e) if num is None else (num + e * v, den + e)
            return num * pltpu.reciprocal(den, approx=True)

        first, acc, scores, front, finish, marks = None, [None] * n_col, {}, {}, {}, []
        for op, arg in _schedule(H, n_col, timing):
            if op == "first":
                part = _mm(lhs(0, 0, col(arg)), weight(0, 0, GROUP, arg * LANES, LANES))
                first = part + 0.0 if first is None else first + part
                if arg == n_col - 1:
                    keep(0, 0, first)
            elif op == "proj":
                if len(marks) >= LAG:
                    tok[parity][zero + 1, pl.ds(0, SUB), col(0)] = marks[-LAG]
                part = _mm(lhs(*arg, col(0, D)), weight(*arg))
                keep(*arg, part)
                marks.append(part[-SUB:])
            elif op == "score":
                raw = []
                for h in range(arg * GROUP, (arg + 1) * GROUP):
                    q = jnp.concatenate(rows_of(0, h)[::2], axis=0)
                    raw.append(_mm_nt(q, jnp.concatenate(rows_of(1, h), axis=0).astype(BF16)))
                for j, r in enumerate(raw):
                    prob[arg][zero + j] = softmax(r)
            elif op == "value":
                for j in range(GROUP):
                    v = jnp.concatenate(rows_of(2, arg * GROUP + j), axis=0).astype(BF16)
                    head_out[arg][zero, :, col(j, Dh)] = _mm(prob[arg][j], v)
            elif op == "out":
                g, n = arg
                assert (g + 1) * GROUP - 1 not in front and (g + 1) * GROUP - 1 in scores
                if n:
                    head_out[g][zero + 1, pl.ds(0, SUB), col(0)] = marks[-LAG]
                o = jnp.concatenate([head_out[g][0, pl.ds(0, M), :], paced[HEAD + g],
                                     head_out[g][0, pl.ds(M, rest), :]], axis=0)
                part = _mm(o, weight(3, g * GROUP + n))
                acc[n] = part + 0.0 if acc[n] is None else acc[n] + part
                marks.append(acc[n][-SUB:])
            elif op == "window":
                if arg >= 2:
                    paced[zero + HEAD + (arg - 2) // GROUP, :, col((arg - 2) % GROUP, Dh)] = front.pop(arg - 2)
                if arg < H:
                    scores[arg] = front_scores(arg)
                if 1 <= arg <= H:
                    front[arg - 1] = front_values(arg - 1, scores[arg - 1])
            elif op == "side":
                finish[arg] = side_work[arg]()
            else:
                finish[arg]()
        for n in range(n_col):
            paced[MEM, :, col(n)] = acc[n][:M]
            att[:, col(n)] = acc[n][M:]

    def layer(x_in, x_out, first_layer):
        def normalize(slot, parity, zero, half):
            rows = pl.ds(half * PACK, PACK)
            n = _layernorm(x_in[slot, rows, :].astype(F32))
            tok[parity][zero, rows, :] = n

            def finish():
                paced[zero + MARK, :, col(0)] = n[-SUB:, -LANES:]
            return finish

        def epilogue(slot, zero, half):
            rows = pl.ds(half * PACK, PACK)
            a = att[rows, :]
            x1 = (x_in[slot, rows, :].astype(F32) + _rb(a)).astype(BF16)
            n1 = _layernorm(x1.astype(F32))
            r = _rb(jnp.sum(n1 * w_r, axis=-1, keepdims=True))
            x_in[slot, rows, :] = x1
            x_out[slot, rows, :] = (x1.astype(F32) + n1).astype(BF16)
            routed[slot, rows, :] = n1

            def finish():
                best, where = paced[BEST, :, col(0)], paced[WHERE, :, col(0)]
                for j in range(PACK // SUB):
                    score = r[j * SUB:(j + 1) * SUB]
                    row = lax.broadcasted_iota(jnp.int32, best.shape, 0) + (slot * T + half * PACK + j * SUB)
                    better = (score > best) & (slot > 0)
                    best, where = jnp.where(better, score, best), jnp.where(better, row.astype(F32), where)
                paced[zero + BEST, :, col(0)] = best
                paced[zero + WHERE, :, col(0)] = where
            return finish

        n_trip = n_seg // UNROLL
        n_sent = n_seg - UNROLL - 1
        if not first_layer:
            head_cp = pltpu.make_async_copy(x_out.at[pl.ds(1, n_sent)], out_hbm.at[pl.ds(0, n_sent)],
                                            osem.at[0])
        paced[MEM] = mem0[...].astype(F32)
        paced[BEST, :, col(0)] = jnp.full((SUB, LANES), -jnp.inf, F32)
        paced[WHERE, :, col(0)] = jnp.full((SUB, LANES), T, F32)

        @pl.loop(0, n_trip)
        def _(t):
            if first_layer:
                pl.when(t == 1)(x_cps[1].wait)
            else:
                pl.when(t == n_trip - 1)(head_cp.start)
            zero = lax.shift_right_logical(t, 16)
            for u in range(UNROLL):
                s = t * UNROLL + u
                side = [functools.partial(epilogue, s, zero, half) for half in range(T // PACK)]
                side += [functools.partial(normalize, s + 2, (u + 1) % 2, zero, half) for half in range(T // PACK)]
                attend(s, u % 2, zero, first_layer, TIMING[not first_layer], side)

        for finish in [epilogue(n_seg, 0, half) for half in range(T // PACK)]:
            finish()
        if first_layer:
            for cp in ffn_cps:
                cp.wait()
        else:
            tail_cp = pltpu.make_async_copy(x_out.at[pl.ds(1 + n_sent, n_seg - n_sent)],
                                            out_hbm.at[pl.ds(n_sent, n_seg - n_sent)], osem.at[1])
            tail_cp.start()

        best, where = paced[BEST, :, col(0)], paced[WHERE, :, col(0)]
        top = jnp.max(best, axis=0, keepdims=True)
        sel = jnp.min(jnp.where(best == top, where, T + S - 1), axis=0, keepdims=True)
        sel = sel.astype(jnp.int32)[0, 0]
        slot = jnp.clip(sel // T, 1, n_seg)
        n1 = routed[slot]
        g = _rb(_mm(n1, wg[...]))
        u = _rb(_mm(n1, wu[...]))
        y = _rb(_mm(_rb(g * jax.nn.sigmoid(g)) * u, wd[...]))
        y = _rb(y * _rb(jax.nn.sigmoid(top[:, :1])))
        hit = lax.broadcasted_iota(jnp.int32, (T, D), 0) + slot * T == sel
        x2 = (x_in[slot].astype(F32) + _rb(n1 + jnp.where(hit, y, 0.0))).astype(BF16)
        if first_layer:
            ahead = _layernorm(x_out[1].astype(F32))
            x_out[slot] = x2
            tok[0][0] = ahead

            @pl.when(slot == 1)
            def _():
                tok[0][0] = _layernorm(x2.astype(F32))
        else:
            x_out[0] = x2
            head_cp.wait()
            tail_cp.wait()
            fix_cp = pltpu.make_async_copy(x_out.at[0], out_hbm.at[slot - 1], osem.at[0])
            fix_cp.start()
            fix_cp.wait()

    layer(xa, xb, True)
    layer(xb, xo, False)


@functools.partial(jax.jit, static_argnames=("A_seg_len",))
def pallas_interleave_layers__memory_aug_recurrent_mem_tr__moe_arch_mod__prompt_kernel(
    A_x, A_mem0, A_Wq, A_Wk, A_Wv, A_Wo, A_seg_len, B_x, B_w_r, B_w_gate, B_w_up, B_w_down,
):
    del B_x
    B, S, D = A_x.shape
    _, H, Dh = A_Wq.shape
    M = A_mem0.shape[1]
    T = int(A_seg_len)
    F = B_w_gate.shape[1]
    assert B == 1 and S % (T * UNROLL) == 0 and T == 2 * PACK and M == SUB
    assert H % CHUNK == 0 and Dh == LANES and D == GROUP * Dh
    n_seg = S // T
    per_w = H // CHUNK
    n_groups = H // GROUP

    hbm = pl.BlockSpec(memory_space=pl.ANY)
    out = pl.pallas_call(
        functools.partial(_kernel, S=S, D=D, H=H, Dh=Dh, M=M, T=T),
        out_shape=jax.ShapeDtypeStruct((n_seg, T, D), BF16),
        in_specs=[hbm] * 10,
        out_specs=hbm,
        scratch_shapes=[
            pltpu.VMEM((n_seg + 2, T, D), BF16),
            pltpu.VMEM((n_seg + 2, T, D), BF16),
            pltpu.VMEM((n_seg + 1, T, D), BF16),
            pltpu.VMEM((n_seg + 1, T, D), F32),
            pltpu.VMEM((n_seg, SUB, D), BF16),
            pltpu.VMEM((n_seg * SUB // 2, D), U32),
            pltpu.VMEM((2 * per_w, CHUNK, n_seg * SUB, Dh), F32),
            pltpu.VMEM((3 * per_w, D, CHUNK, Dh), BF16),
            pltpu.VMEM((per_w, CHUNK * Dh, D), BF16),
            pltpu.VMEM((4 * per_w, CHUNK, D // 2, LANES), U32),
            pltpu.VMEM((D, F), BF16),
            pltpu.VMEM((D, F), BF16),
            pltpu.VMEM((F, D), BF16),
            pltpu.VMEM((M, D), BF16),
            pltpu.VMEM((D,), BF16),
            pltpu.VMEM((T, D), F32),
            [pltpu.VMEM((2, T, D), F32)] * 2,
            [[pltpu.VMEM((2, M + T, GROUP * Dh), F32)] * n_groups] * 3,
            [pltpu.VMEM((GROUP, M + T - SUB, M + T), F32)] * n_groups,
            [pltpu.VMEM((2, M + T - SUB, GROUP * Dh), F32)] * n_groups,
            pltpu.VMEM((5 + n_groups, SUB, D), F32),
            pltpu.SemaphoreType.DMA((8,)),
            pltpu.SemaphoreType.DMA((4 * per_w,)),
            pltpu.SemaphoreType.DMA((2,)),
        ],
        compiler_params=pltpu.CompilerParams(vmem_limit_bytes=100 * 1024 * 1024),
    )(
        A_x.reshape(n_seg, T, D), A_mem0.reshape(M, D), A_Wq, A_Wk, A_Wv,
        A_Wo.reshape(per_w, CHUNK * Dh, D), B_w_r, B_w_gate, B_w_up, B_w_down,
    )
    return out.reshape(B, S, D)
```

```python
import functools

import jax
import jax.numpy as jnp
from jax import lax
import jax.experimental.pallas as pl
import jax.experimental.pallas.tpu as pltpu

F32 = jnp.float32
BF16 = jnp.bfloat16
U32 = jnp.uint32
LN_EPS = 1e-5
LOG2E = 1.4426950408889634
MASK_FILL = -1000000000.0 * LOG2E
LANES = 128
SUB = 8
PACK = 16
GROUP = 4
CHUNK = 8
UNROLL = 4
EARLY_ROWS = 64
LAG = 5
TIMING = ((4, 18, 15, 3.5, 6, 124, 128, 2, 2), (6, 16, 10, 3.7, 4, 128, 124, 128, 3))


def _rb(v):
    return v.astype(BF16).astype(F32)


def _layernorm(x):
    inv_n = 1.0 / x.shape[-1]
    mean = jnp.sum(x, axis=-1, keepdims=True) * inv_n
    cen = x - mean
    var = jnp.sum(cen * cen, axis=-1, keepdims=True) * inv_n
    den = _rb(jnp.sqrt(_rb(_rb(var) + LN_EPS)))
    return _rb(_rb(x - _rb(mean)) / den)


def _mm(a, b):
    return lax.dot_general(a, b, (((1,), (0,)), ((), ())), preferred_element_type=F32)


def _mm_nt(a, b):
    return lax.dot_general(a, b, (((1,), (1,)), ((), ())), preferred_element_type=F32)


def _schedule(n_heads, n_col, timing):
    score_at, value_at, start, period, *side_at, depth = timing
    n_groups = n_heads // GROUP
    slots = [("first", n) for n in range(n_col)]
    slots += [("proj", (i, h)) for h in range(n_heads) for i in range(3) if i or h >= GROUP]
    for groups in (range(n_groups - 2), range(n_groups - 2, n_groups)):
        slots += [("out", (g, n)) for n in range(n_col) for g in groups]
    extra = {}
    for g in range(n_groups):
        extra.setdefault(3 * GROUP * (g + 1) + score_at, []).append(("score", g))
        extra.setdefault(min(3 * GROUP * (g + 1) + value_at, len(slots) - n_col * 2 - 3), []).append(("value", g))
    slots = [op for t, slot in enumerate(slots) for op in extra.get(t, []) + [slot]]
    order, window = [], 0
    todo = sorted((t + dt, (kind, j)) for j, t in enumerate(side_at)
                  for dt, kind in ((0, "side"), (13, "done")))
    for t, slot in enumerate(slots):
        if slot[0] not in ("score", "value"):
            while todo and todo[0][0] <= t:
                order.append(todo.pop(0)[1])
            while window < n_heads + depth and start + window * period <= t:
                order += [(kind, window - lag) for kind, lag in (("join", depth), ("front", 0), ("mix", 1))
                          if 0 <= window - lag < n_heads]
                window += 1
        order.append(slot)
    order += [op for _, op in todo]
    at = {op: t for t, op in enumerate(order)}
    for h in range(n_heads):
        assert at["proj", (1, h)] < at["front", h] and at["proj", (2, h)] < at["mix", h]
        assert max(at["join", h], at["value", h // GROUP]) < at["out", (h // GROUP, 0)]
        assert at["proj", (2, h)] < at["score", h // GROUP] < at["value", h // GROUP]
    assert at["done", 0] < at["done", 1]
    return order


def _kernel(x_hbm, mem0_hbm, wq_hbm, wk_hbm, wv_hbm, wo_hbm, wr_hbm, wg_hbm, wu_hbm, wd_hbm,
            out_hbm,
            xa, xb, xo, routed, xe, ne, early, raw_qkv, raw_out, tiles, wg, wu, wd, mem0, wr,
            att, tok, qkv, prob, head_out, paced, sems, wsem, osem,
            *, S, D, H, Dh, M, T):
    n_seg = S // T
    L = M + T
    rest = T - SUB
    scale = Dh ** -0.5 * LOG2E
    gw = GROUP * Dh
    n_col = D // LANES
    per_w = H // CHUNK
    n_qkv = 3 * per_w
    n_early = 2 * per_w

    w_cps = [pltpu.make_async_copy(w_hbm.at[:, pl.ds(j * CHUNK, CHUNK), :], raw_qkv.at[i * per_w + j],
                                   wsem.at[i * per_w + j])
             for i, w_hbm in enumerate((wq_hbm, wk_hbm, wv_hbm)) for j in range(per_w)]
    w_cps += [pltpu.make_async_copy(wo_hbm.at[j], raw_out.at[j], wsem.at[n_qkv + j]) for j in range(per_w)]
    xe_cp = pltpu.make_async_copy(x_hbm.at[:, pl.ds(0, SUB), :], xe, sems.at[0])
    x_cps = [pltpu.make_async_copy(x_hbm.at[pl.ds(lo, hi - lo)], xa.at[pl.ds(1 + lo, hi - lo)], sems.at[1 + i])
             for i, (lo, hi) in enumerate(((0, UNROLL + 1), (UNROLL + 1, n_seg)))]
    small_cps = x_cps[:1] + [pltpu.make_async_copy(mem0_hbm, mem0, sems.at[3]),
                             pltpu.make_async_copy(wr_hbm, wr, sems.at[4])]
    ffn_cps = [pltpu.make_async_copy(src, dst, sems.at[5 + i])
               for i, (src, dst) in enumerate(((wg_hbm, wg), (wu_hbm, wu), (wd_hbm, wd)))]
    batches = [w_cps[2 * c + 3:2 * c + 5] for c in range(n_early)]
    batches[-2] += small_cps
    batches[-1] += x_cps[1:]
    xe_cp.start()
    w_cps[0].start()

    def repack_qkv(c, lo=0, size=D):
        flat = raw_qkv[c, pl.ds(lo, size)].reshape(size, CHUNK * Dh)
        for j in range(CHUNK):
            tiles[c, j, pl.ds(lo // 2, size // 2), :] = pltpu.bitcast(flat[:, j * Dh:(j + 1) * Dh], U32)

    def repack_out(c, lo, size):
        for j in range(CHUNK):
            g, n = divmod(j, n_col)
            w = raw_out[c - n_qkv, pl.ds(g * gw + lo, size), pl.ds(n * LANES, LANES)]
            tiles[c, j, pl.ds(lo // 2, size // 2), :] = pltpu.bitcast(w, U32)

    def load_trips(lo, hi, raw, repack):
        def wait(c):
            pltpu.make_async_copy(raw.at[c - 2 * lo], raw.at[c - 2 * lo], wsem.at[c]).wait()

        @pl.loop(lo, hi)
        def _(c):
            wait(2 * c + 1)
            for k in range(lo, hi):
                @pl.when(c == k)
                def _():
                    for cp in batches[k]:
                        cp.start()

            pl.when(c > 0)(functools.partial(wait, 2 * c))
            n_rows = n_seg * SUB // EARLY_ROWS
            size = 2 * D // (CHUNK * n_rows)
            for piece in range(CHUNK * n_rows):
                j, r = divmod(piece, n_rows)
                lhs = pltpu.bitcast(ne[pl.ds(r * EARLY_ROWS // 2, EARLY_ROWS // 2), :], BF16)
                early[c, j, pl.ds(r * EARLY_ROWS, EARLY_ROWS), :] = _mm(lhs, pltpu.bitcast(tiles[c, j], BF16))
                which, row = divmod(piece * size, D)
                repack(2 * c + which, row, size)

    MEM, SCALE, BEST, WHERE, MARK, HEAD = range(6)

    def col(n, width=LANES):
        return pl.ds(n * width, width)

    for buf in (xa, xb):
        buf[0] = jnp.zeros((T, D), BF16)
        buf[n_seg + 1] = jnp.zeros((T, D), BF16)
    att[...] = jnp.zeros((T, D), F32)
    paced[SCALE] = jnp.full((SUB, D), scale, F32)

    xe_cp.wait()
    w_cps[1].start()
    ne[...] = pltpu.bitcast(_layernorm(xe[...].astype(F32).reshape(n_seg * SUB, D)).astype(BF16), U32)
    w_cps[0].wait()
    repack_qkv(0)
    w_cps[2].start()
    load_trips(0, n_qkv // 2, raw_qkv, repack_qkv)
    load_trips(n_qkv // 2, n_early, raw_out, repack_out)
    for cp in small_cps:
        cp.wait()
    for cp in ffn_cps:
        cp.start()
    tok[0][0] = _layernorm(xa[1].astype(F32))

    w_r = wr[...].astype(F32).reshape(1, D)

    def softmax(raw):
        qi = lax.broadcasted_iota(jnp.int32, raw.shape, 0)
        ki = lax.broadcasted_iota(jnp.int32, raw.shape, 1)
        sc = jnp.where((qi < M) | (ki <= qi + SUB), raw * scale, MASK_FILL)
        e = jnp.exp2(sc - jnp.max(sc, axis=-1, keepdims=True))
        return e * pltpu.reciprocal(jnp.sum(e, axis=-1, keepdims=True), approx=True)

    def rolled(blocks):
        return [pltpu.roll(b, d, 0) if d else b for b in blocks for d in range(SUB)]

    def attend(s, parity, zero, use_early, timing, side_work):
        def is_early(i, h):
            return use_early and i * per_w + h // CHUNK < n_early

        def lhs(i, h, cols):
            lo = SUB if is_early(i, h) else 0
            return jnp.concatenate([paced[MEM, :, cols], tok[parity][0, pl.ds(lo, T - lo), cols]], axis=0)

        def weight(i, h, n_head=1, lo=0, size=D):
            w = [tiles[i * per_w + h // CHUNK, h % CHUNK + j, pl.ds(lo // 2, size // 2), :] for j in range(n_head)]
            return pltpu.bitcast(jnp.concatenate(w, axis=1), BF16)

        def keep(i, h, t):
            cols = pl.ds(h % GROUP * Dh, t.shape[1])
            qkv[i][h // GROUP][zero, pl.ds(0, M), cols] = t[:M]
            qkv[i][h // GROUP][zero, pl.ds(M + L - t.shape[0], t.shape[0] - M), cols] = t[M:]

        def rows_of(i, h):
            buf, cols = qkv[i][h // GROUP], col(h % GROUP, Dh)
            if is_early(i, h):
                front = early[i * per_w + h // CHUNK, h % CHUNK, pl.ds(pl.multiple_of(s * SUB, SUB), SUB), :]
            else:
                front = buf[0, pl.ds(M, SUB), cols]
            return buf[0, pl.ds(0, M), cols], front, buf[0, pl.ds(M + SUB, rest), cols]

        def front_scores(h):
            q = rows_of(0, h)[1] * paced[SCALE, :, col(0)]
            sub = lax.broadcasted_iota(jnp.int32, q.shape, 0)
            out = []
            for j, k in enumerate(rolled(rows_of(1, h)[:2])):
                sc = jnp.broadcast_to(jnp.sum(q * k, axis=-1, keepdims=True), q.shape)
                out.append(jnp.where(sub >= j - M, sc, MASK_FILL) if j > M else sc)
            return out

        def front_values(h, scores):
            top = functools.reduce(jnp.maximum, scores)
            num = den = None
            for sc, v in zip(scores, rolled(rows_of(2, h)[:2])):
                e = jnp.exp2(sc - top)
                num, den = (e * v, e) if num is None else (num + e * v, den + e)
            return num * pltpu.reciprocal(den, approx=True)

        first, acc, scores, front, finish, marks = None, [None] * n_col, {}, {}, {}, []
        for op, arg in _schedule(H, n_col, timing):
            if op == "first":
                part = _mm(lhs(0, 0, col(arg)), weight(0, 0, GROUP, arg * LANES, LANES))
                first = part + 0.0 if first is None else first + part
                if arg == n_col - 1:
                    keep(0, 0, first)
            elif op == "proj":
                if len(marks) >= LAG:
                    tok[parity][zero + 1, pl.ds(0, SUB), col(0)] = marks[-LAG]
                part = _mm(lhs(*arg, col(0, D)), weight(*arg))
                keep(*arg, part)
                marks.append(part[-SUB:])
            elif op == "score":
                raw = []
                for h in range(arg * GROUP, (arg + 1) * GROUP):
                    q = jnp.concatenate(rows_of(0, h)[::2], axis=0)
                    raw.append(_mm_nt(q, jnp.concatenate(rows_of(1, h), axis=0).astype(BF16)))
                for j, r in enumerate(raw):
                    prob[arg][zero + j] = softmax(r)
            elif op == "value":
                for j in range(GROUP):
                    v = jnp.concatenate(rows_of(2, arg * GROUP + j), axis=0).astype(BF16)
                    head_out[arg][zero, :, col(j, Dh)] = _mm(prob[arg][j], v)
            elif op == "out":
                g, n = arg
                if n:
                    head_out[g][zero + 1, pl.ds(0, SUB), col(0)] = marks[-LAG]
                o = jnp.concatenate([head_out[g][0, pl.ds(0, M), :], paced[HEAD + g],
                                     head_out[g][0, pl.ds(M, rest), :]], axis=0)
                part = _mm(o, weight(3, g * GROUP + n))
                acc[n] = part + 0.0 if acc[n] is None else acc[n] + part
                marks.append(acc[n][-SUB:])
            elif op == "front":
                scores[arg] = front_scores(arg)
            elif op == "mix":
                front[arg] = front_values(arg, scores[arg])
            elif op == "join":
                paced[zero + HEAD + arg // GROUP, :, col(arg % GROUP, Dh)] = front[arg]
            elif op == "side":
                finish[arg] = side_work[arg]()
            else:
                finish[arg]()
        for n in range(n_col):
            paced[MEM, :, col(n)] = acc[n][:M]
            att[:, col(n)] = acc[n][M:]

    def layer(x_in, x_out, first_layer):
        def normalize(slot, parity, zero, half):
            rows = pl.ds(half * PACK, PACK)
            n = _layernorm(x_in[slot, rows, :].astype(F32))
            tok[parity][zero, rows, :] = n

            def finish():
                paced[zero + MARK, :, col(0)] = n[-SUB:, -LANES:]
            return finish

        def epilogue(slot, zero, half):
            rows = pl.ds(half * PACK, PACK)
            a = att[rows, :]
            x1 = (x_in[slot, rows, :].astype(F32) + _rb(a)).astype(BF16)
            n1 = _layernorm(x1.astype(F32))
            r = _rb(jnp.sum(n1 * w_r, axis=-1, keepdims=True))
            x_in[slot, rows, :] = x1
            x_out[slot, rows, :] = (x1.astype(F32) + n1).astype(BF16)
            routed[slot, rows, :] = n1

            def finish():
                best, where = paced[BEST, :, col(0)], paced[WHERE, :, col(0)]
                for j in range(PACK // SUB):
                    score = r[j * SUB:(j + 1) * SUB]
                    row = lax.broadcasted_iota(jnp.int32, best.shape, 0) + (slot * T + half * PACK + j * SUB)
                    better = (score > best) & (slot > 0)
                    best, where = jnp.where(better, score, best), jnp.where(better, row.astype(F32), where)
                paced[zero + BEST, :, col(0)] = best
                paced[zero + WHERE, :, col(0)] = where
            return finish

        n_trip = n_seg // UNROLL
        n_sent = n_seg - UNROLL - 1
        if not first_layer:
            head_cp = pltpu.make_async_copy(x_out.at[pl.ds(1, n_sent)], out_hbm.at[pl.ds(0, n_sent)],
                                            osem.at[0])
        paced[MEM] = mem0[...].astype(F32)
        paced[BEST, :, col(0)] = jnp.full((SUB, LANES), -jnp.inf, F32)
        paced[WHERE, :, col(0)] = jnp.full((SUB, LANES), T, F32)

        @pl.loop(0, n_trip)
        def _(t):
            if first_layer:
                pl.when(t == 1)(x_cps[1].wait)
            else:
                pl.when(t == n_trip - 1)(head_cp.start)
            zero = lax.shift_right_logical(t, 16)
            for u in range(UNROLL):
                s = t * UNROLL + u
                side = [functools.partial(epilogue, s, zero, half) for half in range(T // PACK)]
                side += [functools.partial(normalize, s + 2, (u + 1) % 2, zero, half) for half in range(T // PACK)]
                attend(s, u % 2, zero, first_layer, TIMING[not first_layer], side)

        for finish in [epilogue(n_seg, 0, half) for half in range(T // PACK)]:
            finish()
        if first_layer:
            for cp in ffn_cps:
                cp.wait()
        else:
            tail_cp = pltpu.make_async_copy(x_out.at[pl.ds(1 + n_sent, n_seg - n_sent)],
                                            out_hbm.at[pl.ds(n_sent, n_seg - n_sent)], osem.at[1])
            tail_cp.start()

        best, where = paced[BEST, :, col(0)], paced[WHERE, :, col(0)]
        top = jnp.max(best, axis=0, keepdims=True)
        sel = jnp.min(jnp.where(best == top, where, T + S - 1), axis=0, keepdims=True)
        sel = sel.astype(jnp.int32)[0, 0]
        slot = jnp.clip(sel // T, 1, n_seg)
        n1 = routed[slot]
        g = _rb(_mm(n1, wg[...]))
        u = _rb(_mm(n1, wu[...]))
        y = _rb(_mm(_rb(g * jax.nn.sigmoid(g)) * u, wd[...]))
        y = _rb(y * _rb(jax.nn.sigmoid(top[:, :1])))
        hit = lax.broadcasted_iota(jnp.int32, (T, D), 0) + slot * T == sel
        x2 = (x_in[slot].astype(F32) + _rb(n1 + jnp.where(hit, y, 0.0))).astype(BF16)
        if first_layer:
            ahead = _layernorm(x_out[1].astype(F32))
            x_out[slot] = x2
            tok[0][0] = ahead

            @pl.when(slot == 1)
            def _():
                tok[0][0] = _layernorm(x2.astype(F32))
        else:
            x_out[0] = x2
            head_cp.wait()
            tail_cp.wait()
            fix_cp = pltpu.make_async_copy(x_out.at[0], out_hbm.at[slot - 1], osem.at[0])
            fix_cp.start()
            fix_cp.wait()

    layer(xa, xb, True)
    layer(xb, xo, False)


@functools.partial(jax.jit, static_argnames=("A_seg_len",))
def pallas_interleave_layers__memory_aug_recurrent_mem_tr__moe_arch_mod__prompt_kernel(
    A_x, A_mem0, A_Wq, A_Wk, A_Wv, A_Wo, A_seg_len, B_x, B_w_r, B_w_gate, B_w_up, B_w_down,
):
    del B_x
    B, S, D = A_x.shape
    _, H, Dh = A_Wq.shape
    M = A_mem0.shape[1]
    T = int(A_seg_len)
    F = B_w_gate.shape[1]
    assert B == 1 and S % (T * UNROLL) == 0 and T == 2 * PACK and M == SUB
    assert H % CHUNK == 0 and Dh == LANES and D == GROUP * Dh
    n_seg = S // T
    per_w = H // CHUNK
    n_groups = H // GROUP

    hbm = pl.BlockSpec(memory_space=pl.ANY)
    out = pl.pallas_call(
        functools.partial(_kernel, S=S, D=D, H=H, Dh=Dh, M=M, T=T),
        out_shape=jax.ShapeDtypeStruct((n_seg, T, D), BF16),
        in_specs=[hbm] * 10,
        out_specs=hbm,
        scratch_shapes=[
            pltpu.VMEM((n_seg + 2, T, D), BF16),
            pltpu.VMEM((n_seg + 2, T, D), BF16),
            pltpu.VMEM((n_seg + 1, T, D), BF16),
            pltpu.VMEM((n_seg + 1, T, D), F32),
            pltpu.VMEM((n_seg, SUB, D), BF16),
            pltpu.VMEM((n_seg * SUB // 2, D), U32),
            pltpu.VMEM((2 * per_w, CHUNK, n_seg * SUB, Dh), F32),
            pltpu.VMEM((3 * per_w, D, CHUNK, Dh), BF16),
            pltpu.VMEM((per_w, CHUNK * Dh, D), BF16),
            pltpu.VMEM((4 * per_w, CHUNK, D // 2, LANES), U32),
            pltpu.VMEM((D, F), BF16),
            pltpu.VMEM((D, F), BF16),
            pltpu.VMEM((F, D), BF16),
            pltpu.VMEM((M, D), BF16),
            pltpu.VMEM((D,), BF16),
            pltpu.VMEM((T, D), F32),
            [pltpu.VMEM((2, T, D), F32)] * 2,
            [[pltpu.VMEM((2, M + T, GROUP * Dh), F32)] * n_groups] * 3,
            [pltpu.VMEM((GROUP, M + T - SUB, M + T), F32)] * n_groups,
            [pltpu.VMEM((2, M + T - SUB, GROUP * Dh), F32)] * n_groups,
            pltpu.VMEM((5 + n_groups, SUB, D), F32),
            pltpu.SemaphoreType.DMA((8,)),
            pltpu.SemaphoreType.DMA((4 * per_w,)),
            pltpu.SemaphoreType.DMA((2,)),
        ],
        compiler_params=pltpu.CompilerParams(vmem_limit_bytes=100 * 1024 * 1024),
    )(
        A_x.reshape(n_seg, T, D), A_mem0.reshape(M, D), A_Wq, A_Wk, A_Wv,
        A_Wo.reshape(per_w, CHUNK * Dh, D), B_w_r, B_w_gate, B_w_up, B_w_down,
    )
    return out.reshape(B, S, D)
```

```python
import functools

import jax
import jax.numpy as jnp
from jax import lax
import jax.experimental.pallas as pl
import jax.experimental.pallas.tpu as pltpu

F32 = jnp.float32
BF16 = jnp.bfloat16
U32 = jnp.uint32
LN_EPS = 1e-5
LOG2E = 1.4426950408889634
MASK_FILL = -1000000000.0 * LOG2E
LANES = 128
SUB = 8
PACK = 16
GROUP = 4
CHUNK = 8
UNROLL = 4
PAD = 2
EARLY_ROWS = 64
LAG = 5
TIMING = (((4,18,13,3.4,5,7,119,129,3), (4,26,17,3.3,5,6,130,130,3)), ((6,26,13,3.3,7,114,128,129,3), (5,18,16,3.37,124,127,131,132,2)))


def _rb(v):
    return v.astype(BF16).astype(F32)


def _layernorm(x):
    inv_n = 1.0 / x.shape[-1]
    mean = jnp.sum(x, axis=-1, keepdims=True) * inv_n
    cen = x - mean
    var = jnp.sum(cen * cen, axis=-1, keepdims=True) * inv_n
    den = _rb(jnp.sqrt(_rb(_rb(var) + LN_EPS)))
    return _rb(_rb(x - _rb(mean)) / den)


def _mm(a, b):
    return lax.dot_general(a, b, (((1,), (0,)), ((), ())), preferred_element_type=F32)


def _mm_nt(a, b):
    return lax.dot_general(a, b, (((1,), (1,)), ((), ())), preferred_element_type=F32)


def _left(odd, j, x, y):
    own, other = (y, x) if odd else (x, y)
    if j == 0:
        return x(0) + y(1)
    if j == 1:
        return own(odd)
    if j == 2:
        return own(0) + own(1)
    return own(1 - odd) - other(1 - odd)


def _right(b00, b01, b10, b11):
    f00, f01, f10, f11 = (pltpu.bitcast(b, BF16).astype(F32) for b in (b00, b01, b10, b11))
    words = lambda v: pltpu.bitcast(v.astype(BF16), U32)
    return [words(f00 + f11), words(f01 - f11), b11, words(f10 + f11),
            words(f10 - f00), b00, words(f00 + f01), b01, b10]


PLAIN = ((5, 7), (8, 2))


def _out_slots(n_groups):
    slots = []
    for groups, last in ((range(n_groups - 2), range(n_groups - 4)),
                         (range(n_groups - 2, n_groups), range(n_groups - 4, n_groups))):
        long = [(g, j) for j in (1, 2) for g in groups]
        for k, g in enumerate(groups):
            slots += long[2 * k:2 * k + 2] + [(g, 0)]
        slots += [(g, 3) for g in last]
    return slots


def _schedule(n_heads, n_direct, timing):
    score_at, value_at, start, period, *side_at, depth = timing
    n_groups = n_heads // GROUP
    slots = []
    for g in range(n_groups):
        if n_direct:
            block = [(i, j) for j in range(4) for i in range(3)]
        else:
            block = [(i, j) for i in range(3) for j in range(4)]
        if g == 0:
            lead = [(i, j) for i in ((2, 0) if n_direct else (0, 1)) for j in range(2)]
            block = lead + [ij for ij in block if ij not in lead]
        slots += [("proj", (i, g, j)) for i, j in block]
    slots += [("out", gj) for gj in _out_slots(n_groups)]
    extra = {}
    for g in range(n_groups):
        extra.setdefault(3 * GROUP * (g + 1) + score_at, []).append(("score", g))
        extra.setdefault(min(3 * GROUP * (g + 1) + value_at, len(slots) - 13), []).append(("value", g))
    slots = [op for t, slot in enumerate(slots) for op in extra.get(t, []) + [slot]]
    order, window = [], 0
    todo = sorted((t + dt, (kind, j)) for j, t in enumerate(sorted(side_at))
                  for dt, kind in ((0, "side"), (13, "done")))
    for t, slot in enumerate(slots):
        if slot[0] not in ("score", "value"):
            while todo and todo[0][0] <= t:
                order.append(todo.pop(0)[1])
            while window < n_heads + depth and start + window * period <= t:
                order += [(kind, window - lag) for kind, lag in (("join", depth), ("front", 0), ("mix", 1))
                          if 0 <= window - lag < n_heads]
                window += 1
        order.append(slot)
    order += [op for _, op in todo]
    at = {op: t for t, op in enumerate(order)}
    for h in range(n_heads):
        g = h // GROUP
        ready = [at["proj", (i, g, h % GROUP if i < n_direct and (i, g) != (0, 0) else 3)] for i in range(3)]
        assert max(ready[:2]) < at["front", h] and ready[2] < at["mix", h]
        assert max(ready) < at["score", g] < at["value", g]
        assert max(at["join", h], at["value", g]) < min(at["out", (g, j)] for j in range(4))
    return order


def _kernel(x_hbm, mem0_hbm, wq_hbm, wk_hbm, wv_hbm, wo_hbm, wr_hbm, wg_hbm, wu_hbm, wd_hbm,
            out_hbm,
            stream, routed, xe, ne, early, raw_qkv, raw_out, tiles, wg, wu, wd, mem0, wr,
            att, tok, qkv, prob, head_out, paced, sems, wsem, osem,
            *, S, D, H, Dh, M, T):
    n_seg = S // T
    L = M + T
    rest = T - SUB
    scale = Dh ** -0.5 * LOG2E
    half_d = D // 2
    n_groups = H // GROUP
    per_w = H // CHUNK
    per_chunk = CHUNK // GROUP
    n_qkv = 3 * per_w
    n_early = 2

    w_cps = [pltpu.make_async_copy(w_hbm.at[:, pl.ds(j * CHUNK, CHUNK), :], raw_qkv.at[i * per_w + j],
                                   wsem.at[i * per_w + j])
             for i, w_hbm in enumerate((wq_hbm, wk_hbm, wv_hbm)) for j in range(per_w)]
    w_cps += [pltpu.make_async_copy(wo_hbm.at[j], raw_out.at[j], wsem.at[n_qkv + j]) for j in range(per_w)]
    xe_cp = pltpu.make_async_copy(x_hbm.at[:, pl.ds(0, SUB), :], xe, sems.at[0])
    x_cps = [pltpu.make_async_copy(x_hbm.at[pl.ds(lo, hi - lo)], stream.at[0, pl.ds(PAD + lo, hi - lo)], sems.at[1 + i])
             for i, (lo, hi) in enumerate(((0, UNROLL + 2), (UNROLL + 2, n_seg)))]
    small_cps = x_cps[:1] + [pltpu.make_async_copy(mem0_hbm, mem0, sems.at[3]),
                             pltpu.make_async_copy(wr_hbm, wr, sems.at[4])]
    ffn_cps = [pltpu.make_async_copy(src, dst, sems.at[5 + i])
               for i, (src, dst) in enumerate(((wg_hbm, wg), (wu_hbm, wu), (wd_hbm, wd)))]
    batches = [w_cps[2 * c + 3:2 * c + 5] for c in range(2 * per_w)]
    batches[-2] += small_cps
    batches[-1] += x_cps[1:]
    xe_cp.start()
    w_cps[0].start()

    def qkv_rows(c, lo, size):
        pairs = pltpu.bitcast(raw_qkv[c, pl.ds(lo, size)].reshape(size // 2, 2 * CHUNK, Dh), U32)
        pairs = jnp.swapaxes(pairs, 0, 1)
        heads = []
        for j in range(CHUNK // 2):
            even, odd = pairs[j], pairs[CHUNK // 2 + j]
            heads += [(even & 0xFFFF) | (odd << 16), (even >> 16) | ((odd >> 16) << 16)]
        flat = jnp.concatenate(heads, axis=1)
        return [flat[:, g * D:(g + 1) * D] for g in range(per_chunk)]

    def out_rows(c, lo, size):
        return [pltpu.bitcast(raw_out[c - n_qkv, pl.ds(g * D + lo, size), :], U32) for g in range(per_chunk)]

    def repack(rows, c, i, size):
        words = i * (size // 2)
        words = pl.ds(words if isinstance(i, int) else pl.multiple_of(words, SUB), size // 2)
        for g, (top, bottom) in enumerate(zip(rows(c, i * size, size), rows(c, half_d + i * size, size))):
            for n in range(half_d // LANES):
                blocks = [b[:, k * half_d + n * LANES:k * half_d + (n + 1) * LANES]
                          for b in (top, bottom) for k in range(2)]
                for j, w in enumerate(_right(*blocks)):
                    tiles[c * per_chunk + g, j, n, words, :] = w
                yield

    def head_weight(block, j):
        k, n = divmod(j, half_d // LANES)
        return pltpu.bitcast(jnp.concatenate([tiles[block, row[k], n] for row in PLAIN], axis=0), BF16)

    def factor(block, j):
        return pltpu.bitcast(jnp.concatenate([tiles[block, j, n] for n in range(half_d // LANES)], axis=1), BF16)

    def load_trips(lo, hi, raw, rows):
        def wait(c):
            pltpu.make_async_copy(raw.at[c - 2 * lo], raw.at[c - 2 * lo], wsem.at[c]).wait()

        @pl.loop(lo, hi)
        def _(c):
            wait(2 * c + 1)
            for k in range(lo, hi):
                @pl.when(c == k)
                def _():
                    for cp in batches[k]:
                        cp.start()

            pl.when(c > 0)(functools.partial(wait, 2 * c))
            n_rows = n_seg * SUB // EARLY_ROWS
            work = (_ for k in range(2) for i in range(half_d // PACK) for _ in repack(rows, 2 * c + k, i, PACK))
            for piece in range(CHUNK * n_rows):
                j, r = divmod(piece, n_rows)
                lhs = pltpu.bitcast(ne[pl.ds(r * EARLY_ROWS // 2, EARLY_ROWS // 2), :], BF16)
                w = head_weight(c * per_chunk + j // GROUP, j % GROUP)
                early[c, j, pl.ds(r * EARLY_ROWS, EARLY_ROWS), :] = _mm(lhs, w)
                for _ in range(half_d // PACK // n_rows):
                    next(work)

    MEM, MEM_SUM, SCALE, BEST, WHERE, MARK, FRONT = range(7)

    def col(n, width=LANES):
        return pl.ds(n * width, width)

    @pl.loop(0, 2)
    def _(i):
        stream[i, pl.ds(0, PAD)] = jnp.zeros((PAD, T, D), BF16)
        stream[i, pl.ds(PAD + n_seg, PAD)] = jnp.zeros((PAD, T, D), BF16)
        att[i] = jnp.zeros((T, D), F32)
        paced[pl.ds(FRONT + (UNROLL - 2 + i) * n_groups, n_groups)] = jnp.zeros((n_groups, SUB, D), F32)

    @pl.loop(0, rest // SUB)
    def _(i):
        for buf in head_out[-2] + head_out[-1]:
            buf[pl.ds(pl.multiple_of(M + i * SUB, SUB), SUB), :] = jnp.zeros((SUB, D), F32)

    paced[SCALE] = jnp.full((SUB, D), scale, F32)

    xe_cp.wait()
    w_cps[1].start()
    ne[...] = pltpu.bitcast(_layernorm(xe[...].astype(F32).reshape(n_seg * SUB, D)).astype(BF16), U32)
    w_cps[0].wait()

    @pl.loop(0, half_d // (2 * PACK))
    def _(i):
        list(repack(qkv_rows, 0, i, 2 * PACK))

    w_cps[2].start()
    load_trips(0, n_qkv // 2, raw_qkv, qkv_rows)
    load_trips(n_qkv // 2, n_early * per_w, raw_out, out_rows)
    for cp in small_cps:
        cp.wait()
    for cp in ffn_cps:
        cp.start()

    w_r = wr[...].astype(F32).reshape(1, D)

    def at(zero, lo, size):
        return pl.ds(lo, size) if isinstance(zero, int) else pl.ds(pl.multiple_of(zero + lo, SUB), size)

    def softmax(raw):
        qi = lax.broadcasted_iota(jnp.int32, raw.shape, 0)
        ki = lax.broadcasted_iota(jnp.int32, raw.shape, 1)
        sc = jnp.where((qi < M) | (ki <= qi + SUB), raw * scale, MASK_FILL)
        e = jnp.exp2(sc - jnp.max(sc, axis=-1, keepdims=True))
        return e * pltpu.reciprocal(jnp.sum(e, axis=-1, keepdims=True), approx=True)

    def rolled(blocks):
        return [pltpu.roll(b, d, 0) if d else b for b in blocks for d in range(SUB)]

    def combine(odd, j, parts, put):
        def with_m(v):
            m, cut = parts[0][-PACK:], (0 if odd else PACK)
            halves = [v[lo:lo + PACK] + m if lo == cut else v[lo:lo + PACK] for lo in (0, PACK)]
            return jnp.concatenate(halves, axis=0)

        tokens, memory = [p[-T:] for p in parts], [p[:M] for p in parts]
        if j == 1:
            put(1 - odd, 1 - odd, with_m(tokens[1]), not odd)
            return None
        if j == 2:
            put(odd, 1 - odd, tokens[1] + tokens[2], False)
            return 1 - odd, memory[1] + memory[2]
        put(odd, odd, with_m(tokens[3] - tokens[2]), not odd)
        return odd, memory[0] - memory[2] + memory[3]

    def memory_left(odd, j, half, both):
        return both() if j == 2 else half(odd if j < 2 else 1 - odd)

    def project(u, zero, i, g, j, parts, with_memory=True):
        odd = u % 2
        lhs = tok[u][pl.ds(j // 2 * T, T if j else PACK), col(j % 2, half_d)]
        if with_memory:
            mem = memory_left(odd, j, lambda k: paced[MEM, :, col(k, half_d)],
                              lambda: paced[MEM_SUM, :, col(0, half_d)])
            lhs = jnp.concatenate([mem, lhs], axis=0)
        parts.append(_mm(lhs, factor(i * n_groups + g, j + 3 * odd if j else 0)))

        def put(seg, k, v, accumulate):
            buf = qkv[(u + odd + seg) % UNROLL][i][g]
            buf[at(zero, M, T), col(k, half_d)] = v + buf[pl.ds(M, T), col(k, half_d)] if accumulate else v

        if j:
            mem = combine(odd, j, parts, put)
            if mem and with_memory:
                qkv[u][i][g][at(zero, 0, M), col(mem[0], half_d)] = mem[1]

    def project_out(u, g, j, acc, with_memory=True):
        odd = u % 2

        def rows(seg):
            src = (u + odd - 2 + seg) % UNROLL
            return lambda k: jnp.concatenate([paced[FRONT + src * n_groups + g, :, col(k, half_d)],
                                              head_out[src][g][pl.ds(M, rest), col(k, half_d)]], axis=0)

        lhs = _left(odd, j, rows(0), rows(1))
        if j == 0:
            lhs = lhs[:PACK] if odd else lhs[PACK:]
        if with_memory:
            half = lambda k: head_out[u][g][pl.ds(0, M), col(k, half_d)]
            lhs = jnp.concatenate([memory_left(odd, j, half, lambda: half(0) + half(1)), lhs], axis=0)
        part = _mm(lhs, factor(3 * n_groups + g, j + 3 * odd if j else 0))
        acc[j] = part + 0.0 if acc[j] is None else acc[j] + part

    def finish_out(u, acc):
        def put(seg, k, v, accumulate):
            att[seg, :, col(k, half_d)] = v + att[seg, :, col(k, half_d)] if accumulate else v

        return [combine(u % 2, j, acc, put) for j in (1, 2, 3)][1:]

    def set_memory(halves):
        for k, v in halves:
            paced[MEM, :, col(k, half_d)] = v
        paced[MEM_SUM, :, col(0, half_d)] = halves[0][1] + halves[1][1]

    def attend(s, u, zero, n_direct, timing, side_work):
        def project_direct(i, g, j, parts):
            def lhs(cols):
                return jnp.concatenate([paced[MEM, :, cols], tok[u][pl.ds(2 * T + SUB, rest), cols]], axis=0)

            def keep(cols, v):
                qkv[u][i][g][at(zero, 0, M), cols] = v[:M]
                qkv[u][i][g][at(zero, M + SUB, rest), cols] = v[M:]

            if (i, g) != (0, 0):
                parts.append(_mm(lhs(col(0, D)), head_weight(i * n_groups + g, j)))
                keep(col(j, Dh), parts[-1])
                return
            k = (u + j // 2) % 2
            parts.append(_mm(lhs(col(k, half_d)), factor(0, PLAIN[k][j % 2])) + 0.0)
            if j >= 2:
                keep(col(j % 2, half_d), parts[j - 2] + parts[j])

        def rows_of(i, h):
            buf, cols = qkv[u][i][h // GROUP], col(h % GROUP, Dh)
            if i < n_direct:
                front = early[i * per_w + h // CHUNK, h % CHUNK, pl.ds(pl.multiple_of(s * SUB, SUB), SUB), :]
            else:
                front = buf[pl.ds(M, SUB), cols]
            return buf[pl.ds(0, M), cols], front, buf[pl.ds(M + SUB, rest), cols]

        def front_scores(h):
            q = rows_of(0, h)[1] * paced[SCALE, :, col(0)]
            sub = lax.broadcasted_iota(jnp.int32, q.shape, 0)
            out = []
            for j, k in enumerate(rolled(rows_of(1, h)[:2])):
                sc = jnp.broadcast_to(jnp.sum(q * k, axis=-1, keepdims=True), q.shape)
                out.append(jnp.where(sub >= j - M, sc, MASK_FILL) if j > M else sc)
            return out

        def front_values(h, scores):
            top = functools.reduce(jnp.maximum, scores)
            num = den = None
            for sc, v in zip(scores, rolled(rows_of(2, h)[:2])):
                e = jnp.exp2(sc - top)
                num, den = (e * v, e) if num is None else (num + e * v, den + e)
            return num * pltpu.reciprocal(den, approx=True)

        parts, acc, scores, front, finish, marks, used = {}, [None] * 4, {}, {}, {}, [], set()
        for op, arg in _schedule(H, n_direct, timing):
            if op == "proj":
                if len(marks) >= LAG:
                    tok[u][at(zero, PACK, SUB), col(0)] = marks[-LAG]
                mine = parts.setdefault(arg[:2], [])
                if arg[0] < n_direct:
                    project_direct(*arg, mine)
                else:
                    project(u, zero, *arg, mine)
                marks.append(mine[-1][-SUB:, -LANES:])
            elif op == "score":
                raw = []
                for h in range(arg * GROUP, (arg + 1) * GROUP):
                    q = jnp.concatenate(rows_of(0, h)[::2], axis=0)
                    raw.append(_mm_nt(q, jnp.concatenate(rows_of(1, h), axis=0).astype(BF16)))
                for j, r in enumerate(raw):
                    prob[arg][zero + j] = softmax(r)
            elif op == "value":
                for j in range(GROUP):
                    v = jnp.concatenate(rows_of(2, arg * GROUP + j), axis=0).astype(BF16)
                    head_out[u][arg][at(zero, 0, M + rest), col(j, Dh)] = _mm(prob[arg][j], v)
            elif op == "out":
                if arg[0] in used:
                    for src in {u, (u + u % 2 - 2) % UNROLL, (u + u % 2 - 1) % UNROLL}:
                        head_out[src][arg[0]][at(zero, M + rest, SUB), col(0)] = marks[-LAG]
                used.add(arg[0])
                project_out(u, *arg, acc)
                marks.append(acc[arg[1]][-SUB:, -LANES:])
            elif op == "front":
                scores[arg] = front_scores(arg)
            elif op == "mix":
                front[arg] = front_values(arg, scores[arg])
            elif op == "join":
                paced[zero + FRONT + u * n_groups + arg // GROUP, :, col(arg % GROUP, Dh)] = front[arg]
            elif op == "side":
                finish[arg] = side_work(arg)
            else:
                finish[arg]()
        set_memory(finish_out(u, acc))

    n_trip = n_seg // UNROLL
    n_sent = n_seg - UNROLL - 2
    out_cps = [pltpu.make_async_copy(stream.at[2, pl.ds(PAD + lo, hi - lo)], out_hbm.at[pl.ds(lo, hi - lo)],
                                     osem.at[i]) for i, (lo, hi) in enumerate(((0, n_sent), (n_sent, n_seg)))]

    @pl.loop(0, 2)
    def _(layer):
        def normalize(s, u, zero, n_direct, piece):
            half, seg = divmod(piece, 2)
            n = _layernorm(stream[layer, PAD + s + seg, pl.ds(half * PACK, PACK), :].astype(F32))
            if n_direct or not seg:
                tok[u + seg][at(zero, 2 * T + half * PACK, PACK), :] = n
            if seg:
                x = lambda k: tok[u][pl.ds(2 * T + half * PACK, PACK), col(k, half_d)]
                y = lambda k: n[:, k * half_d:(k + 1) * half_d]
                for odd in range(2):
                    for j in range(1 if odd == half else 0, 4):
                        rows = at(zero, j // 2 * T + (half * PACK if j else 0), PACK)
                        tok[u - odd][rows, col(j % 2, half_d)] = _left(odd, j, x, y)

            def finish():
                paced[zero + MARK, :, col(0)] = n[-SUB:, -LANES:]
            return finish

        def epilogue(s, zero, piece):
            seg, half = divmod(piece, 2)
            slot, rows = PAD + s + seg, pl.ds(half * PACK, PACK)
            x1 = (stream[layer, slot, rows, :].astype(F32) + _rb(att[seg, rows, :])).astype(BF16)
            n1 = _layernorm(x1.astype(F32))
            r = _rb(jnp.sum(n1 * w_r, axis=-1, keepdims=True))
            stream[layer, slot, rows, :] = x1
            stream[layer + 1, slot, rows, :] = (x1.astype(F32) + n1).astype(BF16)
            routed[slot, rows, :] = n1

            def finish():
                best, where = paced[BEST, :, col(0)], paced[WHERE, :, col(0)]
                for j in range(PACK // SUB):
                    score = r[j * SUB:(j + 1) * SUB]
                    row = lax.broadcasted_iota(jnp.int32, best.shape, 0) + (s * T + piece * PACK + j * SUB)
                    better = (score > best) & (s >= 0)
                    best, where = jnp.where(better, score, best), jnp.where(better, row.astype(F32), where)
                paced[zero + BEST, :, col(0)] = best
                paced[zero + WHERE, :, col(0)] = where
            return finish

        set_memory([(k, mem0[:, col(k, half_d)].astype(F32)) for k in range(2)])
        paced[BEST, :, col(0)] = jnp.full((SUB, LANES), -jnp.inf, F32)
        paced[WHERE, :, col(0)] = jnp.zeros((SUB, LANES), F32)
        for piece in range(4):
            normalize(0, 0, 0, n_early, piece)

        def lead_in(i):
            for g in range(n_groups):
                parts = []
                for j in range(4):
                    project(UNROLL - 1, 0, i, g, j, parts, with_memory=False)

        def trip(t, n_direct, timing):
            zero = lax.shift_right_logical(t, 16)
            for u in range(UNROLL):
                s = t * UNROLL + u
                if u % 2:
                    side = functools.partial(epilogue, s - 3, zero)
                else:
                    side = functools.partial(normalize, s + 2, (u + 2) % UNROLL, zero, n_direct)
                attend(s, u, zero, n_direct, timing[u % 2], side)

        for i in range(n_early, 3):
            lead_in(i)

        @pl.when(layer == 0)
        def _():
            @pl.loop(0, n_trip)
            def _(t):
                pl.when(t == 1)(x_cps[1].wait)
                trip(t, n_early, TIMING[0])

            for cp in ffn_cps:
                cp.wait()

        @pl.when(layer == 1)
        def _():
            for i in range(n_early):
                lead_in(i)

            @pl.loop(0, n_trip)
            def _(t):
                pl.when(t == n_trip - 1)(out_cps[0].start)
                trip(t, 0, TIMING[1])

        acc = [None] * 4
        for j in range(4):
            for g in range(n_groups):
                project_out(0, g, j, acc, with_memory=False)
        finish_out(0, acc)
        for finish in [epilogue(n_seg - 2, 0, piece) for piece in range(4)]:
            finish()
        pl.when(layer == 1)(out_cps[1].start)

        best, where = paced[BEST, :, col(0)], paced[WHERE, :, col(0)]
        top = jnp.max(best, axis=0, keepdims=True)
        sel = jnp.min(jnp.where(best == top, where, S - 1), axis=0, keepdims=True)
        sel = sel.astype(jnp.int32)[0, 0]
        seg = jnp.clip(sel // T, 0, n_seg - 1)
        n1 = routed[PAD + seg]
        g = _rb(_mm(n1, wg[...]))
        u = _rb(_mm(n1, wu[...]))
        y = _rb(_mm(_rb(g * jax.nn.sigmoid(g)) * u, wd[...]))
        y = _rb(y * _rb(jax.nn.sigmoid(top[:, :1])))
        hit = lax.broadcasted_iota(jnp.int32, (T, D), 0) + seg * T == sel
        x2 = (stream[layer, PAD + seg].astype(F32) + _rb(n1 + jnp.where(hit, y, 0.0))).astype(BF16)

        @pl.when(layer == 1)
        def _():
            for cp in out_cps:
                cp.wait()

        stream[layer + 1, PAD + seg] = x2

        @pl.when(layer == 1)
        def _():
            fix_cp = pltpu.make_async_copy(stream.at[2, PAD + seg], out_hbm.at[seg], osem.at[0])
            fix_cp.start()
            fix_cp.wait()


@functools.partial(jax.jit, static_argnames=("A_seg_len",))
def pallas_interleave_layers__memory_aug_recurrent_mem_tr__moe_arch_mod__prompt_kernel(
    A_x, A_mem0, A_Wq, A_Wk, A_Wv, A_Wo, A_seg_len, B_x, B_w_r, B_w_gate, B_w_up, B_w_down,
):
    del B_x
    B, S, D = A_x.shape
    _, H, Dh = A_Wq.shape
    M = A_mem0.shape[1]
    T = int(A_seg_len)
    F = B_w_gate.shape[1]
    assert B == 1 and S % (T * UNROLL) == 0 and T == 2 * PACK and M == SUB
    assert H % CHUNK == 0 and Dh == LANES and D == GROUP * Dh
    n_seg = S // T
    per_w = H // CHUNK
    n_groups = H // GROUP

    hbm = pl.BlockSpec(memory_space=pl.ANY)
    out = pl.pallas_call(
        functools.partial(_kernel, S=S, D=D, H=H, Dh=Dh, M=M, T=T),
        out_shape=jax.ShapeDtypeStruct((n_seg, T, D), BF16),
        in_specs=[hbm] * 10,
        out_specs=hbm,
        scratch_shapes=[
            pltpu.VMEM((3, n_seg + 2 * PAD, T, D), BF16),
            pltpu.VMEM((n_seg + PAD, T, D), F32),
            pltpu.VMEM((n_seg, SUB, D), BF16),
            pltpu.VMEM((n_seg * SUB // 2, D), U32),
            pltpu.VMEM((2 * per_w, CHUNK, n_seg * SUB, Dh), F32),
            pltpu.VMEM((3 * per_w, D, CHUNK, Dh), BF16),
            pltpu.VMEM((per_w, CHUNK * Dh, D), BF16),
            pltpu.VMEM((4 * n_groups, 9, D // 2 // LANES, D // 4, LANES), U32),
            pltpu.VMEM((D, F), BF16),
            pltpu.VMEM((D, F), BF16),
            pltpu.VMEM((F, D), BF16),
            pltpu.VMEM((M, D), BF16),
            pltpu.VMEM((D,), BF16),
            pltpu.VMEM((2, T, D), F32),
            [pltpu.VMEM((3 * T, D), F32)] * UNROLL,
            [[[pltpu.VMEM((M + T, D), F32)] * n_groups] * 3] * UNROLL,
            [pltpu.VMEM((GROUP, M + T - SUB, M + T), F32)] * n_groups,
            [[pltpu.VMEM((M + T, D), F32)] * n_groups] * UNROLL,
            pltpu.VMEM((6 + UNROLL * n_groups, SUB, D), F32),
            pltpu.SemaphoreType.DMA((8,)),
            pltpu.SemaphoreType.DMA((4 * per_w,)),
            pltpu.SemaphoreType.DMA((2,)),
        ],
        compiler_params=pltpu.CompilerParams(vmem_limit_bytes=112 * 1024 * 1024),
    )(
        A_x.reshape(n_seg, T, D), A_mem0.reshape(M, D), A_Wq, A_Wk, A_Wv,
        A_Wo.reshape(per_w, CHUNK * Dh, D), B_w_r, B_w_gate, B_w_up, B_w_down,
    )
    return out.reshape(B, S, D)
```

```python
import functools

import jax
import jax.numpy as jnp
from jax import lax
import jax.experimental.pallas as pl
import jax.experimental.pallas.tpu as pltpu

F32 = jnp.float32
BF16 = jnp.bfloat16
U32 = jnp.uint32
LN_EPS = 1e-5
LOG2E = 1.4426950408889634
MASK_FILL = -1000000000.0 * LOG2E
LANES = 128
SUB = 8
PACK = 16
GROUP = 4
CHUNK = 8
UNROLL = 4
PAD = 2
EARLY_ROWS = 64
LAG = 5
TIMING = (((6,26,17,3.9,2,6,126,126,5), (4,20,17,3.15,11,126,132,132,5)), ((6,26,17,3.8,10,117,127,129,6), (7,23,18,3.3,14,126,132,134,4)))


def _rb(v):
    return v.astype(BF16).astype(F32)


def _layernorm(x):
    inv_n = 1.0 / x.shape[-1]
    mean = jnp.sum(x, axis=-1, keepdims=True) * inv_n
    cen = x - mean
    var = jnp.sum(cen * cen, axis=-1, keepdims=True) * inv_n
    den = _rb(jnp.sqrt(_rb(_rb(var) + LN_EPS)))
    return _rb(_rb(x - _rb(mean)) / den)


def _mm(a, b):
    return lax.dot_general(a, b, (((1,), (0,)), ((), ())), preferred_element_type=F32)


def _mm_nt(a, b):
    return lax.dot_general(a, b, (((1,), (1,)), ((), ())), preferred_element_type=F32)


def _left(odd, j, x, y):
    own, other = (y, x) if odd else (x, y)
    if j == 0:
        return x(0) + y(1)
    if j == 1:
        return own(odd)
    if j == 2:
        return own(0) + own(1)
    return own(1 - odd) - other(1 - odd)


def _right(b00, b01, b10, b11):
    f00, f01, f10, f11 = (pltpu.bitcast(b, BF16).astype(F32) for b in (b00, b01, b10, b11))
    words = lambda v: pltpu.bitcast(v.astype(BF16), U32)
    return [words(f00 + f11), words(f01 - f11), b11, words(f10 + f11),
            words(f10 - f00), b00, words(f00 + f01), b01, b10]


PLAIN = ((5, 7), (8, 2))


def _out_slots(n_groups):
    slots = []
    for groups, last in ((range(n_groups - 2), range(n_groups - 4)),
                         (range(n_groups - 2, n_groups), range(n_groups - 4, n_groups))):
        long = [(g, j) for j in (1, 2) for g in groups]
        for k, g in enumerate(groups):
            slots += long[2 * k:2 * k + 2] + [(g, 0)]
        slots += [(g, 3) for g in last]
    return slots


def _schedule(n_heads, odd, timing, carried=()):
    score_at, value_at, start, period, *side_at, depth = timing
    n_groups = n_heads // GROUP
    slots = []
    for g in range(n_groups):
        block = [(i, j) for i in range(3) for j in range(4)]
        if g == 0:
            lead = [(i, j) for i in (2, 0) for j in range(2)]
            block = lead + [(2, 2), (2, 3)] + [ij for ij in block[:8] if ij not in lead]
        slots += [("proj", (i, g, j)) for i, j in block]
    slots += [("out", gj) for gj in _out_slots(n_groups)]
    extra = {}
    for g in range(n_groups):
        extra.setdefault(3 * GROUP * (g + 1) + score_at, []).append(("score", g))
        extra.setdefault(min(3 * GROUP * (g + 1) + value_at, len(slots) - 13), []).append(("value", g))
    slots = [op for t, slot in enumerate(slots) for op in extra.get(t, []) + [slot]]
    vector = [(start + w * period, (kind, (odd, w - lag))) for w in range(n_heads + depth)
              for kind, lag in (("join", depth), ("front", 0), ("mix", 1)) if 0 <= w - lag < n_heads]
    vector += [(min(t + dt, len(slots)), (kind, j)) for j, t in enumerate(side_at)
               for dt, kind in ((0, "side"), (13, "done"))]
    vector = sorted(list(carried) + vector, key=lambda item: item[0])
    order = []
    for t, slot in enumerate(slots + [("end", None)]):
        while vector and vector[0][0] <= t and slot[0] not in ("score", "value"):
            order.append(vector.pop(0)[1])
        order.append(slot)
    at = {op: t for t, op in enumerate(order + [op for _, op in vector])}
    for h in range(n_heads):
        g = h // GROUP
        ready = [at["proj", (i, g, 3)] for i in range(3)]
        used = min(at["out", (g, j)] for j in range(4))
        assert max(ready[:2]) < at["front", (odd, h)] and ready[2] < at["mix", (odd, h)]
        assert max(ready) < at["score", g] < at["value", g] < used
        assert not odd or max(at["join", (odd, h)], at.get(("join", (0, h)), 0)) < used
    return order, [(max(t - len(slots), LAG), op) for t, op in vector]


def _kernel(x_hbm, mem0_hbm, wq_hbm, wk_hbm, wv_hbm, wo_hbm, wr_hbm, wg_hbm, wu_hbm, wd_hbm,
            out_hbm,
            stream, routed, xe, ne, early, raw_qkv, raw_out, tiles, wg, wu, wd, mem0, wr,
            att, tok, qkv, prob, head_out, paced, sems, wsem, osem,
            *, S, D, H, Dh, M, T):
    n_seg = S // T
    L = M + T
    rest = T - SUB
    scale = Dh ** -0.5 * LOG2E
    half_d = D // 2
    n_groups = H // GROUP
    per_w = H // CHUNK
    per_chunk = CHUNK // GROUP
    n_qkv = 3 * per_w
    n_early = 2

    w_cps = [pltpu.make_async_copy(w_hbm.at[:, pl.ds(j * CHUNK, CHUNK), :], raw_qkv.at[i * per_w + j],
                                   wsem.at[i * per_w + j])
             for i, w_hbm in enumerate((wq_hbm, wk_hbm, wv_hbm)) for j in range(per_w)]
    w_cps += [pltpu.make_async_copy(wo_hbm.at[j], raw_out.at[j], wsem.at[n_qkv + j]) for j in range(per_w)]
    xe_cp = pltpu.make_async_copy(x_hbm.at[:, pl.ds(0, SUB), :], xe, sems.at[0])
    x_cps = [pltpu.make_async_copy(x_hbm.at[pl.ds(lo, hi - lo)], stream.at[0, pl.ds(PAD + lo, hi - lo)], sems.at[1 + i])
             for i, (lo, hi) in enumerate(((0, UNROLL + 2), (UNROLL + 2, n_seg)))]
    small_cps = x_cps[:1] + [pltpu.make_async_copy(mem0_hbm, mem0, sems.at[3]),
                             pltpu.make_async_copy(wr_hbm, wr, sems.at[4])]
    ffn_cps = [pltpu.make_async_copy(src, dst, sems.at[5 + i])
               for i, (src, dst) in enumerate(((wg_hbm, wg), (wu_hbm, wu), (wd_hbm, wd)))]
    batches = [w_cps[2 * c + 3:2 * c + 5] for c in range(2 * per_w)]
    batches[-2] += small_cps
    batches[-1] += x_cps[1:]
    xe_cp.start()
    w_cps[0].start()

    def qkv_rows(c, lo, size):
        pairs = pltpu.bitcast(raw_qkv[c, pl.ds(lo, size)].reshape(size // 2, 2 * CHUNK, Dh), U32)
        pairs = jnp.swapaxes(pairs, 0, 1)
        heads = []
        for j in range(CHUNK // 2):
            even, odd = pairs[j], pairs[CHUNK // 2 + j]
            heads += [(even & 0xFFFF) | (odd << 16), (even >> 16) | ((odd >> 16) << 16)]
        flat = jnp.concatenate(heads, axis=1)
        return [flat[:, g * D:(g + 1) * D] for g in range(per_chunk)]

    def out_rows(c, lo, size):
        return [pltpu.bitcast(raw_out[c - n_qkv, pl.ds(g * D + lo, size), :], U32) for g in range(per_chunk)]

    def repack(rows, c, i, size):
        words = i * (size // 2)
        words = pl.ds(words if isinstance(i, int) else pl.multiple_of(words, SUB), size // 2)
        for g, (top, bottom) in enumerate(zip(rows(c, i * size, size), rows(c, half_d + i * size, size))):
            for n in range(half_d // LANES):
                blocks = [b[:, k * half_d + n * LANES:k * half_d + (n + 1) * LANES]
                          for b in (top, bottom) for k in range(2)]
                for j, w in enumerate(_right(*blocks)):
                    tiles[c * per_chunk + g, j, n, words, :] = w
                yield

    def head_weight(block, j):
        k, n = divmod(j, half_d // LANES)
        return pltpu.bitcast(jnp.concatenate([tiles[block, row[k], n] for row in PLAIN], axis=0), BF16)

    def factor(block, j):
        return pltpu.bitcast(jnp.concatenate([tiles[block, j, n] for n in range(half_d // LANES)], axis=1), BF16)

    def load_trips(lo, hi, raw, rows):
        def wait(c):
            pltpu.make_async_copy(raw.at[c - 2 * lo], raw.at[c - 2 * lo], wsem.at[c]).wait()

        @pl.loop(lo, hi)
        def _(c):
            wait(2 * c + 1)
            for k in range(lo, hi):
                @pl.when(c == k)
                def _():
                    for cp in batches[k]:
                        cp.start()

            pl.when(c > 0)(functools.partial(wait, 2 * c))
            n_rows = n_seg * SUB // EARLY_ROWS
            work = (_ for k in range(2) for i in range(half_d // PACK) for _ in repack(rows, 2 * c + k, i, PACK))
            for piece in range(CHUNK * n_rows):
                j, r = divmod(piece, n_rows)
                lhs = pltpu.bitcast(ne[pl.ds(r * EARLY_ROWS // 2, EARLY_ROWS // 2), :], BF16)
                w = head_weight(c * per_chunk + j // GROUP, j % GROUP)
                early[c, j, pl.ds(r * EARLY_ROWS, EARLY_ROWS), :] = _mm(lhs, w)
                for _ in range(half_d // PACK // n_rows):
                    next(work)

    MEM, MEM_SUM, SCALE, BEST, WHERE, MARK, FRONT = range(7)

    def col(n, width=LANES):
        return pl.ds(n * width, width)

    @pl.loop(0, 2)
    def _(i):
        stream[i, pl.ds(0, PAD)] = jnp.zeros((PAD, T, D), BF16)
        stream[i, pl.ds(PAD + n_seg, PAD)] = jnp.zeros((PAD, T, D), BF16)
        att[i] = jnp.zeros((T, D), F32)
        paced[pl.ds(FRONT + (UNROLL - 2 + i) * n_groups, n_groups)] = jnp.zeros((n_groups, SUB, D), F32)

    @pl.loop(0, rest // SUB)
    def _(i):
        for buf in head_out[-2] + head_out[-1]:
            buf[pl.ds(pl.multiple_of(M + i * SUB, SUB), SUB), :] = jnp.zeros((SUB, D), F32)

    paced[SCALE] = jnp.full((SUB, D), scale, F32)

    xe_cp.wait()
    w_cps[1].start()
    ne[...] = pltpu.bitcast(_layernorm(xe[...].astype(F32).reshape(n_seg * SUB, D)).astype(BF16), U32)
    w_cps[0].wait()

    @pl.loop(0, half_d // (2 * PACK))
    def _(i):
        list(repack(qkv_rows, 0, i, 2 * PACK))

    w_cps[2].start()
    load_trips(0, n_qkv // 2, raw_qkv, qkv_rows)
    load_trips(n_qkv // 2, n_early * per_w, raw_out, out_rows)
    for cp in small_cps:
        cp.wait()
    for cp in ffn_cps:
        cp.start()

    w_r = wr[...].astype(F32).reshape(1, D)

    def at(zero, lo, size):
        return pl.ds(lo, size) if isinstance(zero, int) else pl.ds(pl.multiple_of(zero + lo, SUB), size)

    def softmax(raw):
        qi = lax.broadcasted_iota(jnp.int32, raw.shape, 0)
        ki = lax.broadcasted_iota(jnp.int32, raw.shape, 1)
        sc = jnp.where((qi < M) | (ki <= qi + SUB), raw * scale, MASK_FILL)
        e = jnp.exp2(sc - jnp.max(sc, axis=-1, keepdims=True))
        return e * pltpu.reciprocal(jnp.sum(e, axis=-1, keepdims=True), approx=True)

    def rolled(blocks):
        return [pltpu.roll(b, d, 0) if d else b for b in blocks for d in range(SUB)]

    def combine(odd, j, parts, put, skip=0):
        def with_m(v):
            if odd:
                return jnp.concatenate([v[:-PACK] + parts[0][skip - PACK:], v[-PACK:]], axis=0)
            return jnp.concatenate([v[:-PACK], v[-PACK:] + parts[0][-PACK:]], axis=0)

        tokens, memory = [p[skip - T:] for p in parts], [p[:M] for p in parts]
        if j == 1:
            put(1 - odd, 1 - odd, with_m(tokens[1]), not odd)
            return None
        if j == 2:
            put(odd, 1 - odd, tokens[1] + tokens[2], False)
            return 1 - odd, memory[1] + memory[2]
        put(odd, odd, with_m(tokens[3] - tokens[2]), not odd)
        return odd, memory[0] - memory[2] + memory[3]

    def memory_left(odd, j, half, both):
        return both() if j == 2 else half(odd if j < 2 else 1 - odd)

    def project(u, zero, skip, i, g, j, parts, with_memory=True):
        odd = u % 2
        lo = skip if j or odd else 0
        lhs = tok[u][pl.ds(j // 2 * T + lo, (T if j else PACK) - lo), col(j % 2, half_d)]
        if with_memory:
            mem = memory_left(odd, j, lambda k: paced[MEM, :, col(k, half_d)],
                              lambda: paced[MEM_SUM, :, col(0, half_d)])
            lhs = jnp.concatenate([mem, lhs], axis=0)
        parts.append(_mm(lhs, factor(i * n_groups + g, j + 3 * odd if j else 0)))

        def put(seg, k, v, accumulate):
            buf, cols = qkv[(u + odd + seg) % UNROLL][i][g], col(k, half_d)
            buf[at(zero, M + skip, T - skip), cols] = v + buf[M + skip:, cols] if accumulate else v

        if j:
            mem = combine(odd, j, parts, put, skip)
            if mem and with_memory:
                qkv[u][i][g][at(zero, 0, M), col(mem[0], half_d)] = mem[1]

    def project_out(u, g, j, acc, with_memory=True):
        odd = u % 2

        def rows(seg):
            src = (u + odd - 2 + seg) % UNROLL
            return lambda k: jnp.concatenate([paced[FRONT + src * n_groups + g, :, col(k, half_d)],
                                              head_out[src][g][pl.ds(M, rest), col(k, half_d)]], axis=0)

        lhs = _left(odd, j, rows(0), rows(1))
        if j == 0:
            lhs = lhs[:PACK] if odd else lhs[PACK:]
        if with_memory:
            half = lambda k: head_out[u][g][pl.ds(0, M), col(k, half_d)]
            lhs = jnp.concatenate([memory_left(odd, j, half, lambda: half(0) + half(1)), lhs], axis=0)
        part = _mm(lhs, factor(3 * n_groups + g, j + 3 * odd if j else 0))
        acc[j] = part + 0.0 if acc[j] is None else acc[j] + part

    def finish_out(u, acc):
        def put(seg, k, v, accumulate):
            att[seg, :, col(k, half_d)] = v + att[seg, :, col(k, half_d)] if accumulate else v

        return [combine(u % 2, j, acc, put) for j in (1, 2, 3)][1:]

    def set_memory(halves):
        for k, v in halves:
            paced[MEM, :, col(k, half_d)] = v
        paced[MEM_SUM, :, col(0, half_d)] = halves[0][1] + halves[1][1]

    def attend_pair(s0, u0, zero, n_ahead, timing, side_work):
        def rows_of(i, odd, h):
            buf, cols = qkv[u0 + odd][i][h // GROUP], col(h % GROUP, Dh)
            if i < n_ahead:
                rows = pl.ds(pl.multiple_of((s0 + odd) * SUB, SUB), SUB)
                front = early[i * per_w + h // CHUNK, h % CHUNK, rows, :]
            else:
                front = buf[pl.ds(M, SUB), cols]
            return buf[pl.ds(0, M), cols], front, buf[pl.ds(M + SUB, rest), cols]

        def front_scores(odd, h):
            q = rows_of(0, odd, h)[1] * paced[SCALE, :, col(0)]
            sub = lax.broadcasted_iota(jnp.int32, q.shape, 0)
            out = []
            for j, k in enumerate(rolled(rows_of(1, odd, h)[:2])):
                sc = jnp.broadcast_to(jnp.sum(q * k, axis=-1, keepdims=True), q.shape)
                out.append(jnp.where(sub >= j - M, sc, MASK_FILL) if j > M else sc)
            return out

        def front_values(odd, h, scores):
            top = functools.reduce(jnp.maximum, scores)
            num = den = None
            for sc, v in zip(scores, rolled(rows_of(2, odd, h)[:2])):
                e = jnp.exp2(sc - top)
                num, den = (e * v, e) if num is None else (num + e * v, den + e)
            return num * pltpu.reciprocal(den, approx=True)

        carried, scores, front = (), {}, {}
        for odd in range(2):
            u = u0 + odd
            order, carried = _schedule(H, odd, timing[odd], carried)
            parts, acc, finish, marks, used = {}, [None] * 4, {}, [], set()
            for op, arg in order:
                if op == "proj":
                    if len(marks) >= LAG:
                        tok[u][at(zero, PACK, SUB), col(0)] = marks[-LAG]
                    mine = parts.setdefault(arg[:2], [])
                    project(u, zero, SUB if arg[0] < n_ahead else 0, *arg, mine)
                    marks.append(mine[-1][-SUB:, -LANES:])
                elif op == "score":
                    raw = []
                    for h in range(arg * GROUP, (arg + 1) * GROUP):
                        q = jnp.concatenate(rows_of(0, odd, h)[::2], axis=0)
                        raw.append(_mm_nt(q, jnp.concatenate(rows_of(1, odd, h), axis=0).astype(BF16)))
                    for j, r in enumerate(raw):
                        prob[arg][zero + j] = softmax(r)
                elif op == "value":
                    for j in range(GROUP):
                        v = jnp.concatenate(rows_of(2, odd, arg * GROUP + j), axis=0).astype(BF16)
                        head_out[u][arg][at(zero, 0, M + rest), col(j, Dh)] = _mm(prob[arg][j], v)
                elif op == "out":
                    if arg[0] in used:
                        for src in range(u + odd - 2, u + 1):
                            head_out[src][arg[0]][at(zero, M + rest, SUB), col(0)] = marks[-LAG]
                    used.add(arg[0])
                    project_out(u, *arg, acc)
                    marks.append(acc[arg[1]][-SUB:, -LANES:])
                elif op == "front":
                    scores[arg] = front_scores(*arg)
                elif op == "mix":
                    front[arg] = front_values(*arg, scores[arg])
                elif op == "join":
                    g, j = divmod(arg[1], GROUP)
                    paced[zero + FRONT + (u0 + arg[0]) * n_groups + g, :, col(j, Dh)] = front[arg]
                elif op == "side":
                    finish[arg] = side_work[odd](arg)
                elif op == "done":
                    finish[arg]()
            set_memory(finish_out(u, acc))

    n_trip = n_seg // UNROLL
    n_sent = n_seg - UNROLL - 2
    out_cps = [pltpu.make_async_copy(stream.at[2, pl.ds(PAD + lo, hi - lo)], out_hbm.at[pl.ds(lo, hi - lo)],
                                     osem.at[i]) for i, (lo, hi) in enumerate(((0, n_sent), (n_sent, n_seg)))]

    @pl.loop(0, 2)
    def _(layer):
        def normalize(s, u, zero, piece):
            half, seg = divmod(piece, 2)
            n = _layernorm(stream[layer, PAD + s + seg, pl.ds(half * PACK, PACK), :].astype(F32))
            if seg == 0:
                tok[u][at(zero, 2 * T, PACK), :] = n
            else:
                x = lambda k: tok[u][pl.ds(2 * T, PACK), col(k, half_d)]
                y = lambda k: n[:, k * half_d:(k + 1) * half_d]
                for odd in range(2):
                    for j in range(1 if odd == half else 0, 4):
                        rows = at(zero, j // 2 * T + (half * PACK if j else 0), PACK)
                        tok[u - odd][rows, col(j % 2, half_d)] = _left(odd, j, x, y)

            def finish():
                paced[zero + MARK, :, col(0)] = n[-SUB:, -LANES:]
            return finish

        def epilogue(s, zero, piece):
            seg, half = divmod(piece, 2)
            slot, rows = PAD + s + seg, pl.ds(half * PACK, PACK)
            x1 = (stream[layer, slot, rows, :].astype(F32) + _rb(att[seg, rows, :])).astype(BF16)
            n1 = _layernorm(x1.astype(F32))
            r = _rb(jnp.sum(n1 * w_r, axis=-1, keepdims=True))
            stream[layer, slot, rows, :] = x1
            stream[layer + 1, slot, rows, :] = (x1.astype(F32) + n1).astype(BF16)
            routed[slot, rows, :] = n1

            def finish():
                best, where = paced[BEST, :, col(0)], paced[WHERE, :, col(0)]
                for j in range(PACK // SUB):
                    score = r[j * SUB:(j + 1) * SUB]
                    row = lax.broadcasted_iota(jnp.int32, best.shape, 0) + (s * T + piece * PACK + j * SUB)
                    better = (score > best) & (s >= 0)
                    best, where = jnp.where(better, score, best), jnp.where(better, row.astype(F32), where)
                paced[zero + BEST, :, col(0)] = best
                paced[zero + WHERE, :, col(0)] = where
            return finish

        set_memory([(k, mem0[:, col(k, half_d)].astype(F32)) for k in range(2)])
        paced[BEST, :, col(0)] = jnp.full((SUB, LANES), -jnp.inf, F32)
        paced[WHERE, :, col(0)] = jnp.zeros((SUB, LANES), F32)
        for piece in range(4):
            normalize(0, 0, 0, piece)
        for i in range(3):
            for g in range(n_groups):
                parts = []
                for j in range(4):
                    project(UNROLL - 1, 0, 0, i, g, j, parts, with_memory=False)

        def trip(t, n_ahead, timing):
            zero = lax.shift_right_logical(t, 16)
            for u in range(0, UNROLL, 2):
                s = t * UNROLL + u
                side = (functools.partial(normalize, s + 2, (u + 2) % UNROLL, zero),
                        functools.partial(epilogue, s - 2, zero))
                attend_pair(s, u, zero, n_ahead, timing, side)

        @pl.when(layer == 0)
        def _():
            @pl.loop(0, n_trip)
            def _(t):
                pl.when(t == 1)(x_cps[1].wait)
                trip(t, n_early, TIMING[0])

            for cp in ffn_cps:
                cp.wait()

        @pl.when(layer == 1)
        def _():
            @pl.loop(0, n_trip)
            def _(t):
                pl.when(t == n_trip - 1)(out_cps[0].start)
                trip(t, 0, TIMING[1])

        acc = [None] * 4
        for j in range(4):
            for g in range(n_groups):
                project_out(0, g, j, acc, with_memory=False)
        finish_out(0, acc)
        for finish in [epilogue(n_seg - 2, 0, piece) for piece in range(4)]:
            finish()
        pl.when(layer == 1)(out_cps[1].start)

        best, where = paced[BEST, :, col(0)], paced[WHERE, :, col(0)]
        top = jnp.max(best, axis=0, keepdims=True)
        sel = jnp.min(jnp.where(best == top, where, S - 1), axis=0, keepdims=True)
        sel = sel.astype(jnp.int32)[0, 0]
        seg = jnp.clip(sel // T, 0, n_seg - 1)
        n1 = routed[PAD + seg]
        g = _rb(_mm(n1, wg[...]))
        u = _rb(_mm(n1, wu[...]))
        y = _rb(_mm(_rb(g * jax.nn.sigmoid(g)) * u, wd[...]))
        y = _rb(y * _rb(jax.nn.sigmoid(top[:, :1])))
        hit = lax.broadcasted_iota(jnp.int32, (T, D), 0) + seg * T == sel
        x2 = (stream[layer, PAD + seg].astype(F32) + _rb(n1 + jnp.where(hit, y, 0.0))).astype(BF16)

        @pl.when(layer == 1)
        def _():
            for cp in out_cps:
                cp.wait()

        stream[layer + 1, PAD + seg] = x2

        @pl.when(layer == 1)
        def _():
            fix_cp = pltpu.make_async_copy(stream.at[2, PAD + seg], out_hbm.at[seg], osem.at[0])
            fix_cp.start()
            fix_cp.wait()


@functools.partial(jax.jit, static_argnames=("A_seg_len",))
def pallas_interleave_layers__memory_aug_recurrent_mem_tr__moe_arch_mod__prompt_kernel(
    A_x, A_mem0, A_Wq, A_Wk, A_Wv, A_Wo, A_seg_len, B_x, B_w_r, B_w_gate, B_w_up, B_w_down,
):
    del B_x
    B, S, D = A_x.shape
    _, H, Dh = A_Wq.shape
    M = A_mem0.shape[1]
    T = int(A_seg_len)
    F = B_w_gate.shape[1]
    assert B == 1 and S % (T * UNROLL) == 0 and T == 2 * PACK and M == SUB
    assert H % CHUNK == 0 and Dh == LANES and D == GROUP * Dh
    n_seg = S // T
    per_w = H // CHUNK
    n_groups = H // GROUP

    hbm = pl.BlockSpec(memory_space=pl.ANY)
    out = pl.pallas_call(
        functools.partial(_kernel, S=S, D=D, H=H, Dh=Dh, M=M, T=T),
        out_shape=jax.ShapeDtypeStruct((n_seg, T, D), BF16),
        in_specs=[hbm] * 10,
        out_specs=hbm,
        scratch_shapes=[
            pltpu.VMEM((3, n_seg + 2 * PAD, T, D), BF16),
            pltpu.VMEM((n_seg + PAD, T, D), F32),
            pltpu.VMEM((n_seg, SUB, D), BF16),
            pltpu.VMEM((n_seg * SUB // 2, D), U32),
            pltpu.VMEM((2 * per_w, CHUNK, n_seg * SUB, Dh), F32),
            pltpu.VMEM((3 * per_w, D, CHUNK, Dh), BF16),
            pltpu.VMEM((per_w, CHUNK * Dh, D), BF16),
            pltpu.VMEM((4 * n_groups, 9, D // 2 // LANES, D // 4, LANES), U32),
            pltpu.VMEM((D, F), BF16),
            pltpu.VMEM((D, F), BF16),
            pltpu.VMEM((F, D), BF16),
            pltpu.VMEM((M, D), BF16),
            pltpu.VMEM((D,), BF16),
            pltpu.VMEM((2, T, D), F32),
            [pltpu.VMEM((2 * T + PACK, D), F32)] * UNROLL,
            [[[pltpu.VMEM((M + T, D), F32)] * n_groups] * 3] * UNROLL,
            [pltpu.VMEM((GROUP, M + T - SUB, M + T), F32)] * n_groups,
            [[pltpu.VMEM((M + T, D), F32)] * n_groups] * UNROLL,
            pltpu.VMEM((6 + UNROLL * n_groups, SUB, D), F32),
            pltpu.SemaphoreType.DMA((8,)),
            pltpu.SemaphoreType.DMA((4 * per_w,)),
            pltpu.SemaphoreType.DMA((2,)),
        ],
        compiler_params=pltpu.CompilerParams(vmem_limit_bytes=112 * 1024 * 1024),
    )(
        A_x.reshape(n_seg, T, D), A_mem0.reshape(M, D), A_Wq, A_Wk, A_Wv,
        A_Wo.reshape(per_w, CHUNK * Dh, D), B_w_r, B_w_gate, B_w_up, B_w_down,
    )
    return out.reshape(B, S, D)
```

```python
import functools

import jax
import jax.numpy as jnp
from jax import lax
import jax.experimental.pallas as pl
import jax.experimental.pallas.tpu as pltpu

F32 = jnp.float32
BF16 = jnp.bfloat16
U32 = jnp.uint32
LN_EPS = 1e-5
LOG2E = 1.4426950408889634
MASK_FILL = -1000000000.0 * LOG2E
LANES = 128
SUB = 8
PACK = 16
GROUP = 4
CHUNK = 8
UNROLL = 4
PAD = 2
EARLY_ROWS = 64
TIMING = (((6,26,17,3.88,0,116,126,127,4,6), (6,27,16,3.17,13,127,132,134,6,6)), ((7,23,18,3.35,15,128,132,133,5,5), (7,23,18,3.32,15,129,131,132,4,5)))


def _rb(v):
    return v.astype(BF16).astype(F32)


def _layernorm(x):
    inv_n = 1.0 / x.shape[-1]
    mean = jnp.sum(x, axis=-1, keepdims=True) * inv_n
    cen = x - mean
    var = jnp.sum(cen * cen, axis=-1, keepdims=True) * inv_n
    den = _rb(jnp.sqrt(_rb(_rb(var) + LN_EPS)))
    return _rb(_rb(x - _rb(mean)) / den)


def _mm(a, b):
    return lax.dot_general(a, b, (((1,), (0,)), ((), ())), preferred_element_type=F32)


def _mm_nt(a, b):
    return lax.dot_general(a, b, (((1,), (1,)), ((), ())), preferred_element_type=F32)


def _left(odd, j, x, y):
    own, other = (y, x) if odd else (x, y)
    if j == 0:
        return x(0) + y(1)
    if j == 1:
        return own(odd)
    if j == 2:
        return own(0) + own(1)
    return own(1 - odd) - other(1 - odd)


def _right(b00, b01, b10, b11):
    f00, f01, f10, f11 = (pltpu.bitcast(b, BF16).astype(F32) for b in (b00, b01, b10, b11))
    words = lambda v: pltpu.bitcast(v.astype(BF16), U32)
    return [words(f00 + f11), words(f01 - f11), b11, words(f10 + f11),
            words(f10 - f00), b00, words(f00 + f01), b01, b10]


PLAIN = ((5, 7), (8, 2))


def _out_slots(n_groups):
    slots = []
    for groups, last in ((range(n_groups - 2), range(n_groups - 4)),
                         (range(n_groups - 2, n_groups), range(n_groups - 4, n_groups))):
        long = [(g, j) for j in (1, 2) for g in groups]
        for k, g in enumerate(groups):
            slots += long[2 * k:2 * k + 2] + [(g, 0)]
        slots += [(g, 3) for g in last]
    return slots


def _schedule(n_heads, odd, timing, carried=()):
    score_at, value_at, start, period, *side_at, depth, _ = timing
    n_groups = n_heads // GROUP
    slots = []
    for g in range(n_groups):
        block = [(i, j) for i in range(3) for j in (1, 0, 2, 3)]
        if g == 0:
            block = block[8:10] + block[0:2] + block[10:11] + block[2:6] + block[11:] + block[6:8]
        elif g < 3:
            block = block[:2] + block[8:9] + block[2:8] + block[9:]
        slots += [("proj", (i, g, j)) for i, j in block]
    slots += [("out", gj) for gj in _out_slots(n_groups)]
    extra = {}
    for g in range(n_groups):
        extra.setdefault(3 * GROUP * (g + 1) + score_at + (g < 2), []).append(("score", g))
        extra.setdefault(min(3 * GROUP * (g + 1) + value_at, len(slots) - 13), []).append(("value", g))
    slots = [op for t, slot in enumerate(slots) for op in extra.get(t, []) + [slot]]
    vector = [(start + w * period, (kind, (odd, w - lag))) for w in range(n_heads + depth)
              for kind, lag in (("join", depth), ("front", 0), ("mix", 1)) if 0 <= w - lag < n_heads]
    vector += [(min(t + dt, len(slots)), (kind, j)) for j, t in enumerate(side_at)
               for dt, kind in ((0, "side"), (13, "done"))]
    vector = sorted(list(carried) + vector, key=lambda item: item[0])
    order = []
    for t, slot in enumerate(slots + [("end", None)]):
        while vector and vector[0][0] <= t and slot[0] not in ("score", "value"):
            order.append(vector.pop(0)[1])
        order.append(slot)
    at = {op: t for t, op in enumerate(order + [op for _, op in vector])}
    for h in range(n_heads):
        g = h // GROUP
        ready = [max(at["proj", (i, g, j)] for j in range(4)) for i in range(3)]
        used = min(at["out", (g, j)] for j in range(4))
        assert max(ready[:2]) < at["front", (odd, h)] and ready[2] < at["mix", (odd, h)]
        assert max(ready[:2]) < at["score", g] < at["value", g] < used
        assert not odd or max(at["join", (odd, h)], at.get(("join", (0, h)), 0)) < used
    return order, [(max(t - len(slots), timing[-1]), op) for t, op in vector]


def _kernel(x_hbm, mem0_hbm, wq_hbm, wk_hbm, wv_hbm, wo_hbm, wr_hbm, wg_hbm, wu_hbm, wd_hbm,
            out_hbm,
            stream, routed, xe, ne, early, raw_qkv, raw_out, tiles, wg, wu, wd, mem0, wr,
            att, tok, qkv, prob, head_out, paced, sems, wsem, osem,
            *, S, D, H, Dh, M, T):
    n_seg = S // T
    L = M + T
    rest = T - SUB
    scale = Dh ** -0.5 * LOG2E
    half_d = D // 2
    n_groups = H // GROUP
    per_w = H // CHUNK
    per_chunk = CHUNK // GROUP
    n_qkv = 3 * per_w
    n_early = 2

    w_cps = [pltpu.make_async_copy(w_hbm.at[:, pl.ds(j * CHUNK, CHUNK), :], raw_qkv.at[i * per_w + j],
                                   wsem.at[i * per_w + j])
             for i, w_hbm in enumerate((wq_hbm, wk_hbm, wv_hbm)) for j in range(per_w)]
    w_cps += [pltpu.make_async_copy(wo_hbm.at[j], raw_out.at[j], wsem.at[n_qkv + j]) for j in range(per_w)]
    xe_cp = pltpu.make_async_copy(x_hbm.at[:, pl.ds(0, SUB), :], xe, sems.at[0])
    x_cps = [pltpu.make_async_copy(x_hbm.at[pl.ds(lo, hi - lo)], stream.at[0, pl.ds(PAD + lo, hi - lo)], sems.at[1 + i])
             for i, (lo, hi) in enumerate(((0, UNROLL + 2), (UNROLL + 2, n_seg)))]
    small_cps = x_cps[:1] + [pltpu.make_async_copy(mem0_hbm, mem0, sems.at[3]),
                             pltpu.make_async_copy(wr_hbm, wr, sems.at[4])]
    ffn_cps = [pltpu.make_async_copy(src, dst, sems.at[5 + i])
               for i, (src, dst) in enumerate(((wg_hbm, wg), (wu_hbm, wu), (wd_hbm, wd)))]
    batches = [w_cps[2 * c + 3:2 * c + 5] for c in range(2 * per_w)]
    batches[-2] += small_cps
    batches[-1] += x_cps[1:]
    xe_cp.start()
    w_cps[0].start()

    def qkv_rows(c, lo, size):
        pairs = pltpu.bitcast(raw_qkv[c, pl.ds(lo, size)].reshape(size // 2, 2 * CHUNK, Dh), U32)
        pairs = jnp.swapaxes(pairs, 0, 1)
        heads = []
        for j in range(CHUNK // 2):
            even, odd = pairs[j], pairs[CHUNK // 2 + j]
            heads += [(even & 0xFFFF) | (odd << 16), (even >> 16) | ((odd >> 16) << 16)]
        flat = jnp.concatenate(heads, axis=1)
        return [flat[:, g * D:(g + 1) * D] for g in range(per_chunk)]

    def out_rows(c, lo, size):
        return [pltpu.bitcast(raw_out[c - n_qkv, pl.ds(g * D + lo, size), :], U32) for g in range(per_chunk)]

    def repack(rows, c, i, size):
        words = i * (size // 2)
        words = pl.ds(words if isinstance(i, int) else pl.multiple_of(words, SUB), size // 2)
        for g, (top, bottom) in enumerate(zip(rows(c, i * size, size), rows(c, half_d + i * size, size))):
            for n in range(half_d // LANES):
                blocks = [b[:, k * half_d + n * LANES:k * half_d + (n + 1) * LANES]
                          for b in (top, bottom) for k in range(2)]
                for j, w in enumerate(_right(*blocks)):
                    tiles[c * per_chunk + g, j, n, words, :] = w
                yield

    def head_weight(block, j):
        k, n = divmod(j, half_d // LANES)
        return pltpu.bitcast(jnp.concatenate([tiles[block, row[k], n] for row in PLAIN], axis=0), BF16)

    def factor(block, j):
        return pltpu.bitcast(jnp.concatenate([tiles[block, j, n] for n in range(half_d // LANES)], axis=1), BF16)

    def load_trips(lo, hi, raw, rows):
        def wait(c):
            pltpu.make_async_copy(raw.at[c - 2 * lo], raw.at[c - 2 * lo], wsem.at[c]).wait()

        @pl.loop(lo, hi)
        def _(c):
            wait(2 * c + 1)
            for k in range(lo, hi):
                @pl.when(c == k)
                def _():
                    for cp in batches[k]:
                        cp.start()

            pl.when(c > 0)(functools.partial(wait, 2 * c))
            n_rows = n_seg * SUB // EARLY_ROWS
            work = (_ for k in range(2) for i in range(half_d // PACK) for _ in repack(rows, 2 * c + k, i, PACK))
            for piece in range(CHUNK * n_rows):
                j, r = divmod(piece, n_rows)
                lhs = pltpu.bitcast(ne[pl.ds(r * EARLY_ROWS // 2, EARLY_ROWS // 2), :], BF16)
                w = head_weight(c * per_chunk + j // GROUP, j % GROUP)
                early[c, j, pl.ds(r * EARLY_ROWS, EARLY_ROWS), :] = _mm(lhs, w)
                for _ in range(half_d // PACK // n_rows):
                    next(work)

    MEM, MEM_SUM, SCALE, BEST, WHERE, MARK, FRONT = range(7)

    def col(n, width=LANES):
        return pl.ds(n * width, width)

    @pl.loop(0, 2)
    def _(i):
        stream[i, pl.ds(0, PAD)] = jnp.zeros((PAD, T, D), BF16)
        stream[i, pl.ds(PAD + n_seg, PAD)] = jnp.zeros((PAD, T, D), BF16)
        att[i] = jnp.zeros((T, D), F32)
        paced[pl.ds(FRONT + (UNROLL - 2 + i) * n_groups, n_groups)] = jnp.zeros((n_groups, SUB, D), F32)

    @pl.loop(0, rest // SUB)
    def _(i):
        for buf in head_out[-2] + head_out[-1]:
            buf[pl.ds(pl.multiple_of(M + i * SUB, SUB), SUB), :] = jnp.zeros((SUB, D), F32)

    paced[SCALE] = jnp.full((SUB, D), scale, F32)

    xe_cp.wait()
    w_cps[1].start()
    ne[...] = pltpu.bitcast(_layernorm(xe[...].astype(F32).reshape(n_seg * SUB, D)).astype(BF16), U32)
    w_cps[0].wait()

    @pl.loop(0, half_d // (2 * PACK))
    def _(i):
        list(repack(qkv_rows, 0, i, 2 * PACK))

    w_cps[2].start()
    load_trips(0, n_qkv // 2, raw_qkv, qkv_rows)
    load_trips(n_qkv // 2, n_early * per_w, raw_out, out_rows)
    for cp in small_cps:
        cp.wait()
    for cp in ffn_cps:
        cp.start()

    w_r = wr[...].astype(F32).reshape(1, D)

    def at(zero, lo, size):
        return pl.ds(lo, size) if isinstance(zero, int) else pl.ds(pl.multiple_of(zero + lo, SUB), size)

    def softmax(raw):
        qi = lax.broadcasted_iota(jnp.int32, raw.shape, 0)
        ki = lax.broadcasted_iota(jnp.int32, raw.shape, 1)
        sc = jnp.where((qi < M) | (ki <= qi + SUB), raw * scale, MASK_FILL)
        e = jnp.exp2(sc - jnp.max(sc, axis=-1, keepdims=True))
        return e * pltpu.reciprocal(jnp.sum(e, axis=-1, keepdims=True), approx=True)

    def rolled(blocks):
        return [pltpu.roll(b, d, 0) if d else b for b in blocks for d in range(SUB)]

    def combine(odd, k, parts, put, skip=0):
        def with_m(v, op=jnp.add):
            if odd:
                return jnp.concatenate([op(v[:-PACK], parts[0][skip - PACK:]), v[-PACK:]], axis=0)
            return jnp.concatenate([v[:-PACK], op(v[-PACK:], parts[0][-PACK:])], axis=0)

        tokens, memory = (lambda j: parts[j][skip - T:]), (lambda j: parts[j][:M])
        if k == 0:
            put(1 - odd, 1 - odd, with_m(tokens(1)), not odd)
            return None
        if k == 1:
            put(odd, 1 - odd, tokens(1) + tokens(2), False)
            return 1 - odd, memory(1) + memory(2)
        put(odd, odd, tokens(3) - with_m(tokens(2), jnp.subtract), not odd)
        return odd, memory(0) - memory(2) + memory(3)

    def memory_left(odd, j, half, both):
        return both() if j == 2 else half(odd if j < 2 else 1 - odd)

    def project(u, zero, skip, i, g, j, parts, with_memory=True):
        odd = u % 2
        lo = skip if j or odd else 0
        lhs = tok[u][pl.ds(j // 2 * T + lo, (T if j else PACK) - lo), col(j % 2, half_d)]
        if with_memory:
            mem = memory_left(odd, j, lambda k: paced[MEM, :, col(k, half_d)],
                              lambda: paced[MEM_SUM, :, col(0, half_d)])
            lhs = jnp.concatenate([mem, lhs], axis=0)
        parts[j] = _mm(lhs, factor(i * n_groups + g, j + 3 * odd if j else 0))

        def put(seg, k, v, accumulate):
            buf, cols = qkv[(u + odd + seg) % UNROLL][i][g], col(k, half_d)
            buf[at(zero, M + skip, T - skip), cols] = v + buf[M + skip:, cols] if accumulate else v

        for k, needs in enumerate(((0, 1), (1, 2), (0, 2, 3))):
            if j in needs and all(n in parts for n in needs):
                mem = combine(odd, k, parts, put, skip)
                if mem and with_memory:
                    qkv[u][i][g][at(zero, 0, M), col(mem[0], half_d)] = mem[1]

    def project_out(u, g, j, acc, with_memory=True):
        odd = u % 2

        def rows(seg):
            src = (u + odd - 2 + seg) % UNROLL
            return lambda k: jnp.concatenate([paced[FRONT + src * n_groups + g, :, col(k, half_d)],
                                              head_out[src][g][pl.ds(M, rest), col(k, half_d)]], axis=0)

        lhs = _left(odd, j, rows(0), rows(1))
        if j == 0:
            lhs = lhs[:PACK] if odd else lhs[PACK:]
        if with_memory:
            half = lambda k: head_out[u][g][pl.ds(0, M), col(k, half_d)]
            lhs = jnp.concatenate([memory_left(odd, j, half, lambda: half(0) + half(1)), lhs], axis=0)
        part = _mm(lhs, factor(3 * n_groups + g, j + 3 * odd if j else 0))
        acc[j] = part + 0.0 if acc[j] is None else acc[j] + part

    def finish_out(u, acc):
        def put(seg, k, v, accumulate):
            att[seg, :, col(k, half_d)] = v + att[seg, :, col(k, half_d)] if accumulate else v

        return [combine(u % 2, k, acc, put) for k in range(3)][1:]

    def set_memory(halves):
        for k, v in halves:
            paced[MEM, :, col(k, half_d)] = v
        paced[MEM_SUM, :, col(0, half_d)] = halves[0][1] + halves[1][1]

    def attend_pair(s0, u0, zero, n_ahead, timing, side_work):
        def rows_of(i, odd, h):
            buf, cols = qkv[u0 + odd][i][h // GROUP], col(h % GROUP, Dh)
            if i < n_ahead:
                rows = pl.ds(pl.multiple_of((s0 + odd) * SUB, SUB), SUB)
                front = early[i * per_w + h // CHUNK, h % CHUNK, rows, :]
            else:
                front = buf[pl.ds(M, SUB), cols]
            return buf[pl.ds(0, M), cols], front, buf[pl.ds(M + SUB, rest), cols]

        def front_scores(odd, h):
            q = rows_of(0, odd, h)[1] * paced[SCALE, :, col(0)]
            sub = lax.broadcasted_iota(jnp.int32, q.shape, 0)
            out = []
            for j, k in enumerate(rolled(rows_of(1, odd, h)[:2])):
                sc = jnp.broadcast_to(jnp.sum(q * k, axis=-1, keepdims=True), q.shape)
                out.append(jnp.where(sub >= j - M, sc, MASK_FILL) if j > M else sc)
            return out

        def front_values(odd, h, scores):
            top = functools.reduce(jnp.maximum, scores)
            num = den = None
            for sc, v in zip(scores, rolled(rows_of(2, odd, h)[:2])):
                e = jnp.exp2(sc - top)
                num, den = (e * v, e) if num is None else (num + e * v, den + e)
            return num * pltpu.reciprocal(den, approx=True)

        carried, scores, front = (), {}, {}
        for odd in range(2):
            u, lag = u0 + odd, timing[odd][-1]
            order, carried = _schedule(H, odd, timing[odd], carried)
            parts, acc, finish, marks, used = {}, [None] * 4, {}, [], set()
            for op, arg in order:
                if op == "proj":
                    if len(marks) >= lag:
                        tok[u][at(zero, PACK, SUB), col(0)] = marks[-lag]
                    mine = parts.setdefault(arg[:2], {})
                    project(u, zero, SUB if arg[0] < n_ahead else 0, *arg, mine)
                    marks.append(mine[arg[2]][-SUB:, -LANES:])
                elif op == "score":
                    raw = []
                    for h in range(arg * GROUP, (arg + 1) * GROUP):
                        q = jnp.concatenate(rows_of(0, odd, h)[::2], axis=0)
                        raw.append(_mm_nt(q, jnp.concatenate(rows_of(1, odd, h), axis=0).astype(BF16)))
                    for j, r in enumerate(raw):
                        prob[arg][zero + j] = softmax(r)
                elif op == "value":
                    for j in range(GROUP):
                        v = jnp.concatenate(rows_of(2, odd, arg * GROUP + j), axis=0).astype(BF16)
                        head_out[u][arg][at(zero, 0, M + rest), col(j, Dh)] = _mm(prob[arg][j], v)
                elif op == "out":
                    if arg[0] in used:
                        for src in range(u + odd - 2, u + 1):
                            head_out[src][arg[0]][at(zero, M + rest, SUB), col(0)] = marks[-6]
                    used.add(arg[0])
                    project_out(u, *arg, acc)
                    marks.append(acc[arg[1]][-SUB:, -LANES:])
                elif op == "front":
                    scores[arg] = front_scores(*arg)
                elif op == "mix":
                    front[arg] = front_values(*arg, scores[arg])
                elif op == "join":
                    g, j = divmod(arg[1], GROUP)
                    paced[zero + FRONT + (u0 + arg[0]) * n_groups + g, :, col(j, Dh)] = front[arg]
                elif op == "side":
                    finish[arg] = side_work[odd](arg)
                elif op == "done":
                    finish[arg]()
            set_memory(finish_out(u, acc))

    n_trip = n_seg // UNROLL
    n_sent = n_seg - UNROLL - 2
    out_cps = [pltpu.make_async_copy(stream.at[2, pl.ds(PAD + lo, hi - lo)], out_hbm.at[pl.ds(lo, hi - lo)],
                                     osem.at[i]) for i, (lo, hi) in enumerate(((0, n_sent), (n_sent, n_seg)))]

    @pl.loop(0, 2)
    def _(layer):
        def normalize(s, u, zero, piece):
            half, seg = divmod(piece, 2)
            n = _layernorm(stream[layer, PAD + s + seg, pl.ds(half * PACK, PACK), :].astype(F32))
            if seg == 0:
                tok[u][at(zero, 2 * T, PACK), :] = n
            else:
                x = lambda k: tok[u][pl.ds(2 * T, PACK), col(k, half_d)]
                y = lambda k: n[:, k * half_d:(k + 1) * half_d]
                for odd in range(2):
                    for j in range(1 if odd == half else 0, 4):
                        rows = at(zero, j // 2 * T + (half * PACK if j else 0), PACK)
                        tok[u - odd][rows, col(j % 2, half_d)] = _left(odd, j, x, y)

            def finish():
                paced[zero + MARK, :, col(0)] = n[-SUB:, -LANES:]
            return finish

        def epilogue(s, zero, piece):
            seg, half = divmod(piece, 2)
            slot, rows = PAD + s + seg, pl.ds(half * PACK, PACK)
            x1 = (stream[layer, slot, rows, :].astype(F32) + _rb(att[seg, rows, :])).astype(BF16)
            n1 = _layernorm(x1.astype(F32))
            r = _rb(jnp.sum(n1 * w_r, axis=-1, keepdims=True))
            stream[layer, slot, rows, :] = x1
            stream[layer + 1, slot, rows, :] = (x1.astype(F32) + n1).astype(BF16)
            routed[slot, rows, :] = n1

            def finish():
                best, where = paced[BEST, :, col(0)], paced[WHERE, :, col(0)]
                for j in range(PACK // SUB):
                    score = r[j * SUB:(j + 1) * SUB]
                    row = lax.broadcasted_iota(jnp.int32, best.shape, 0) + (s * T + piece * PACK + j * SUB)
                    better = (score > best) & (s >= 0)
                    best, where = jnp.where(better, score, best), jnp.where(better, row.astype(F32), where)
                paced[zero + BEST, :, col(0)] = best
                paced[zero + WHERE, :, col(0)] = where
            return finish

        set_memory([(k, mem0[:, col(k, half_d)].astype(F32)) for k in range(2)])
        paced[BEST, :, col(0)] = jnp.full((SUB, LANES), -jnp.inf, F32)
        paced[WHERE, :, col(0)] = jnp.zeros((SUB, LANES), F32)
        for piece in range(4):
            normalize(0, 0, 0, piece)
        for i in range(3):
            for g in range(n_groups):
                parts = {}
                for j in range(4):
                    project(UNROLL - 1, 0, 0, i, g, j, parts, with_memory=False)

        def trip(t, n_ahead, timing):
            zero = lax.shift_right_logical(t, 16)
            for u in range(0, UNROLL, 2):
                s = t * UNROLL + u
                side = (functools.partial(normalize, s + 2, (u + 2) % UNROLL, zero),
                        functools.partial(epilogue, s - 2, zero))
                attend_pair(s, u, zero, n_ahead, timing, side)

        @pl.when(layer == 0)
        def _():
            @pl.loop(0, n_trip)
            def _(t):
                pl.when(t == 1)(x_cps[1].wait)
                trip(t, n_early, TIMING[0])

            for cp in ffn_cps:
                cp.wait()

        @pl.when(layer == 1)
        def _():
            @pl.loop(0, n_trip)
            def _(t):
                pl.when(t == n_trip - 1)(out_cps[0].start)
                trip(t, 0, TIMING[1])

        acc = [None] * 4
        for j in range(4):
            for g in range(n_groups):
                project_out(0, g, j, acc, with_memory=False)
        finish_out(0, acc)
        for finish in [epilogue(n_seg - 2, 0, piece) for piece in range(4)]:
            finish()
        pl.when(layer == 1)(out_cps[1].start)

        best, where = paced[BEST, :, col(0)], paced[WHERE, :, col(0)]
        top = jnp.max(best, axis=0, keepdims=True)
        sel = jnp.min(jnp.where(best == top, where, S - 1), axis=0, keepdims=True)
        sel = sel.astype(jnp.int32)[0, 0]
        seg = jnp.clip(sel // T, 0, n_seg - 1)
        n1 = routed[PAD + seg]
        g = _rb(_mm(n1, wg[...]))
        u = _rb(_mm(n1, wu[...]))
        y = _rb(_mm(_rb(g * jax.nn.sigmoid(g)) * u, wd[...]))
        y = _rb(y * _rb(jax.nn.sigmoid(top[:, :1])))
        hit = lax.broadcasted_iota(jnp.int32, (T, D), 0) + seg * T == sel
        x2 = (stream[layer, PAD + seg].astype(F32) + _rb(n1 + jnp.where(hit, y, 0.0))).astype(BF16)

        @pl.when(layer == 1)
        def _():
            for cp in out_cps:
                cp.wait()

        stream[layer + 1, PAD + seg] = x2

        @pl.when(layer == 1)
        def _():
            fix_cp = pltpu.make_async_copy(stream.at[2, PAD + seg], out_hbm.at[seg], osem.at[0])
            fix_cp.start()
            fix_cp.wait()


@functools.partial(jax.jit, static_argnames=("A_seg_len",))
def pallas_interleave_layers__memory_aug_recurrent_mem_tr__moe_arch_mod__prompt_kernel(
    A_x, A_mem0, A_Wq, A_Wk, A_Wv, A_Wo, A_seg_len, B_x, B_w_r, B_w_gate, B_w_up, B_w_down,
):
    del B_x
    B, S, D = A_x.shape
    _, H, Dh = A_Wq.shape
    M = A_mem0.shape[1]
    T = int(A_seg_len)
    F = B_w_gate.shape[1]
    assert B == 1 and S % (T * UNROLL) == 0 and T == 2 * PACK and M == SUB
    assert H % CHUNK == 0 and Dh == LANES and D == GROUP * Dh
    n_seg = S // T
    per_w = H // CHUNK
    n_groups = H // GROUP

    hbm = pl.BlockSpec(memory_space=pl.ANY)
    out = pl.pallas_call(
        functools.partial(_kernel, S=S, D=D, H=H, Dh=Dh, M=M, T=T),
        out_shape=jax.ShapeDtypeStruct((n_seg, T, D), BF16),
        in_specs=[hbm] * 10,
        out_specs=hbm,
        scratch_shapes=[
            pltpu.VMEM((3, n_seg + 2 * PAD, T, D), BF16),
            pltpu.VMEM((n_seg + PAD, T, D), F32),
            pltpu.VMEM((n_seg, SUB, D), BF16),
            pltpu.VMEM((n_seg * SUB // 2, D), U32),
            pltpu.VMEM((2 * per_w, CHUNK, n_seg * SUB, Dh), F32),
            pltpu.VMEM((3 * per_w, D, CHUNK, Dh), BF16),
            pltpu.VMEM((per_w, CHUNK * Dh, D), BF16),
            pltpu.VMEM((4 * n_groups, 9, D // 2 // LANES, D // 4, LANES), U32),
            pltpu.VMEM((D, F), BF16),
            pltpu.VMEM((D, F), BF16),
            pltpu.VMEM((F, D), BF16),
            pltpu.VMEM((M, D), BF16),
            pltpu.VMEM((D,), BF16),
            pltpu.VMEM((2, T, D), F32),
            [pltpu.VMEM((2 * T + PACK, D), F32)] * UNROLL,
            [[[pltpu.VMEM((M + T, D), F32)] * n_groups] * 3] * UNROLL,
            [pltpu.VMEM((GROUP, M + T - SUB, M + T), F32)] * n_groups,
            [[pltpu.VMEM((M + T, D), F32)] * n_groups] * UNROLL,
            pltpu.VMEM((6 + UNROLL * n_groups, SUB, D), F32),
            pltpu.SemaphoreType.DMA((8,)),
            pltpu.SemaphoreType.DMA((4 * per_w,)),
            pltpu.SemaphoreType.DMA((2,)),
        ],
        compiler_params=pltpu.CompilerParams(vmem_limit_bytes=112 * 1024 * 1024),
    )(
        A_x.reshape(n_seg, T, D), A_mem0.reshape(M, D), A_Wq, A_Wk, A_Wv,
        A_Wo.reshape(per_w, CHUNK * Dh, D), B_w_r, B_w_gate, B_w_up, B_w_down,
    )
    return out.reshape(B, S, D)
```

```python
import functools

import jax
import jax.numpy as jnp
from jax import lax
import jax.experimental.pallas as pl
import jax.experimental.pallas.tpu as pltpu

F32 = jnp.float32
BF16 = jnp.bfloat16
U32 = jnp.uint32
LN_EPS = 1e-5
LOG2E = 1.4426950408889634
MASK_FILL = -1000000000.0 * LOG2E
LANES = 128
SUB = 8
PACK = 16
GROUP = 4
CHUNK = 8
UNROLL = 4
PAD = 2
EARLY_ROWS = 64
TIMING = (((6,26,17,3.78,0,114,127,127,4,6), (6,27,21,3.25,12,129,131,133,4,6)), ((7,23,18,3.35,15,128,132,133,5,5), (7,23,18,3.32,15,129,131,132,4,5)))


def _rb(v):
    return v.astype(BF16).astype(F32)


def _layernorm(x):
    inv_n = 1.0 / x.shape[-1]
    mean = jnp.sum(x, axis=-1, keepdims=True) * inv_n
    cen = x - mean
    var = jnp.sum(cen * cen, axis=-1, keepdims=True) * inv_n
    den = _rb(jnp.sqrt(_rb(_rb(var) + LN_EPS)))
    return _rb(_rb(x - _rb(mean)) / den)


def _mm(a, b):
    return lax.dot_general(a, b, (((1,), (0,)), ((), ())), preferred_element_type=F32)


def _mm_nt(a, b):
    return lax.dot_general(a, b, (((1,), (1,)), ((), ())), preferred_element_type=F32)


def _left(odd, j, x, y):
    own, other = (y, x) if odd else (x, y)
    if j == 0:
        return x(0) + y(1)
    if j == 1:
        return own(odd)
    if j == 2:
        return own(0) + own(1)
    return own(1 - odd) - other(1 - odd)


def _right(b00, b01, b10, b11):
    f00, f01, f10, f11 = (pltpu.bitcast(b, BF16).astype(F32) for b in (b00, b01, b10, b11))
    words = lambda v: pltpu.bitcast(v.astype(BF16), U32)
    return [words(f00 + f11), words(f01 - f11), b11, words(f10 + f11),
            words(f10 - f00), b00, words(f00 + f01), b01, b10]


PLAIN = ((5, 7), (8, 2))


def _out_slots(n_groups):
    slots = []
    for groups, last in ((range(n_groups - 2), range(n_groups - 4)),
                         (range(n_groups - 2, n_groups), range(n_groups - 4, n_groups))):
        long = [(g, j) for j in (1, 2) for g in groups]
        for k, g in enumerate(groups):
            slots += long[2 * k:2 * k + 2] + [(g, 0)]
        slots += [(g, 3) for g in last]
    return slots


def _schedule(n_heads, odd, timing, carried=()):
    score_at, value_at, start, period, *side_at, depth, _ = timing
    n_groups = n_heads // GROUP
    slots = []
    for g in range(n_groups):
        block = [(i, j) for i in range(3) for j in (1, 0, 2, 3)]
        if g == 0:
            block = block[8:10] + block[0:2] + block[10:11] + block[2:6] + block[11:] + block[6:8]
        elif g < 3:
            block = block[:2] + block[8:9] + block[2:8] + block[9:]
        slots += [("proj", (i, g, j)) for i, j in block]
    slots += [("out", gj) for gj in _out_slots(n_groups)]
    extra = {}
    for g in range(n_groups):
        extra.setdefault(3 * GROUP * (g + 1) + score_at + (g < 2), []).append(("score", g))
        extra.setdefault(min(3 * GROUP * (g + 1) + value_at, len(slots) - 13), []).append(("value", g))
    slots = [op for t, slot in enumerate(slots) for op in extra.get(t, []) + [slot]]
    vector = [(start + w * period, (kind, (odd, w - lag))) for w in range(n_heads + depth)
              for kind, lag in (("join", depth), ("front", 0), ("mix", 1)) if 0 <= w - lag < n_heads]
    vector += [(min(t + dt, len(slots)), (kind, j)) for j, t in enumerate(side_at)
               for dt, kind in ((0, "side"), (13, "done"))]
    vector = sorted(list(carried) + vector, key=lambda item: item[0])
    order = []
    for t, slot in enumerate(slots + [("end", None)]):
        while vector and vector[0][0] <= t and slot[0] not in ("score", "value"):
            order.append(vector.pop(0)[1])
        order.append(slot)
    at = {op: t for t, op in enumerate(order + [op for _, op in vector])}
    for h in range(n_heads):
        g = h // GROUP
        ready = [max(at["proj", (i, g, j)] for j in range(4)) for i in range(3)]
        used = min(at["out", (g, j)] for j in range(4))
        assert max(ready[:2]) < at["front", (odd, h)] and ready[2] < at["mix", (odd, h)]
        assert max(ready[:2]) < at["score", g] < at["value", g] < used
        assert not odd or max(at["join", (odd, h)], at.get(("join", (0, h)), 0)) < used
    return order, [(max(t - len(slots), timing[-1]), op) for t, op in vector]


def _kernel(x_hbm, mem0_hbm, wq_hbm, wk_hbm, wv_hbm, wo_hbm, wr_hbm, wg_hbm, wu_hbm, wd_hbm,
            out_hbm,
            stream, routed, xe, ne, early, raw_qkv, raw_out, tiles, wg, wu, wd, mem0, wr,
            att, tok, qkv, prob, head_out, paced, sems, wsem, osem,
            *, S, D, H, Dh, M, T):
    n_seg = S // T
    L = M + T
    rest = T - SUB
    scale = Dh ** -0.5 * LOG2E
    half_d = D // 2
    n_groups = H // GROUP
    per_w = H // CHUNK
    per_chunk = CHUNK // GROUP
    n_qkv = 3 * per_w
    ahead = {(i, g) for i in range(2) for g in range(i * per_chunk, n_groups)}

    w_cps = [pltpu.make_async_copy(w_hbm.at[:, pl.ds(j * CHUNK, CHUNK), :], raw_qkv.at[i * per_w + j],
                                   wsem.at[i * per_w + j])
             for i, w_hbm in enumerate((wq_hbm, wk_hbm, wv_hbm)) for j in range(per_w)]
    w_cps += [pltpu.make_async_copy(wo_hbm.at[j], raw_out.at[j], wsem.at[n_qkv + j]) for j in range(per_w)]
    xe_cp = pltpu.make_async_copy(x_hbm.at[:, pl.ds(0, SUB), :], xe, sems.at[0])
    x_cps = [pltpu.make_async_copy(x_hbm.at[pl.ds(lo, hi - lo)], stream.at[0, pl.ds(PAD + lo, hi - lo)], sems.at[1 + i])
             for i, (lo, hi) in enumerate(((0, UNROLL + 2), (UNROLL + 2, n_seg)))]
    small_cps = x_cps[:1] + [pltpu.make_async_copy(mem0_hbm, mem0, sems.at[3]),
                             pltpu.make_async_copy(wr_hbm, wr, sems.at[4])]
    ffn_cps = [pltpu.make_async_copy(src, dst, sems.at[5 + i])
               for i, (src, dst) in enumerate(((wg_hbm, wg), (wu_hbm, wu), (wd_hbm, wd)))]
    batches = [w_cps[lo:hi] for lo, hi in ((3, 5), (5, 7), (7, 10), (10, 12), (12, 14), (14, 16))]
    batches[-2] += small_cps
    xe_cp.start()
    w_cps[0].start()

    def qkv_rows(c, lo, size):
        pairs = pltpu.bitcast(raw_qkv[c, pl.ds(lo, size)].reshape(size // 2, 2 * CHUNK, Dh), U32)
        pairs = jnp.swapaxes(pairs, 0, 1)
        heads = []
        for j in range(CHUNK // 2):
            even, odd = pairs[j], pairs[CHUNK // 2 + j]
            heads += [(even & 0xFFFF) | (odd << 16), (even >> 16) | ((odd >> 16) << 16)]
        flat = jnp.concatenate(heads, axis=1)
        return [flat[:, g * D:(g + 1) * D] for g in range(per_chunk)]

    def out_rows(c, lo, size):
        return [pltpu.bitcast(raw_out[c - n_qkv, pl.ds(g * D + lo, size), :], U32) for g in range(per_chunk)]

    def repack(rows, c, i, size):
        words = i * (size // 2)
        words = pl.ds(words if isinstance(i, int) else pl.multiple_of(words, SUB), size // 2)
        for g, (top, bottom) in enumerate(zip(rows(c, i * size, size), rows(c, half_d + i * size, size))):
            for n in range(half_d // LANES):
                blocks = [b[:, k * half_d + n * LANES:k * half_d + (n + 1) * LANES]
                          for b in (top, bottom) for k in range(2)]
                for j, w in enumerate(_right(*blocks)):
                    tiles[c * per_chunk + g, j, n, words, :] = w
                yield

    def head_weight(block, j):
        k, n = divmod(j, half_d // LANES)
        return pltpu.bitcast(jnp.concatenate([tiles[block, row[k], n] for row in PLAIN], axis=0), BF16)

    def factor(block, j):
        return pltpu.bitcast(jnp.concatenate([tiles[block, j, n] for n in range(half_d // LANES)], axis=1), BF16)

    def project_early(c, rows, fresh):
        src = c + jnp.where(c >= per_w, 1, 0)
        n_rows = n_seg * SUB // EARLY_ROWS
        work = (_ for k in fresh for i in range(half_d // PACK) for _ in repack(rows, k, i, PACK))
        for piece in range(CHUNK * n_rows):
            j, r = divmod(piece, n_rows)
            lhs = pltpu.bitcast(ne[pl.ds(r * EARLY_ROWS // 2, EARLY_ROWS // 2), :], BF16)
            w = head_weight(src * per_chunk + j // GROUP, j % GROUP)
            early[src, j, pl.ds(r * EARLY_ROWS, EARLY_ROWS), :] = _mm(lhs, w)
            for _ in range(len(fresh) * half_d // PACK // (2 * n_rows)):
                next(work)

    MEM, MEM_SUM, SCALE, BEST, WHERE, MARK, FRONT = range(7)

    def col(n, width=LANES):
        return pl.ds(n * width, width)

    def at(zero, lo, size):
        return pl.ds(lo, size) if isinstance(zero, int) else pl.ds(pl.multiple_of(zero + lo, SUB), size)

    def normalize(layer, s, u, zero, piece):
        half, seg = divmod(piece, 2)
        n = _layernorm(stream[layer, PAD + s + seg, pl.ds(half * PACK, PACK), :].astype(F32))
        if seg == 0:
            tok[u][at(zero, 2 * T, PACK), :] = n
        else:
            x = lambda k: tok[u][pl.ds(2 * T, PACK), col(k, half_d)]
            y = lambda k: n[:, k * half_d:(k + 1) * half_d]
            for odd in range(2):
                for j in range(1 if odd == half else 0, 4):
                    rows = at(zero, j // 2 * T + (half * PACK if j else 0), PACK)
                    tok[u - odd][rows, col(j % 2, half_d)] = _left(odd, j, x, y)

        def finish():
            paced[zero + MARK, :, col(0)] = n[-SUB:, -LANES:]
        return finish

    def normalize_first(layer):
        for piece in range(4):
            normalize(layer, 0, 0, 0, piece)

    @pl.loop(0, 2)
    def _(i):
        stream[i, pl.ds(0, PAD)] = jnp.zeros((PAD, T, D), BF16)
        stream[i, pl.ds(PAD + n_seg, PAD)] = jnp.zeros((PAD, T, D), BF16)
        att[i] = jnp.zeros((T, D), F32)
        paced[pl.ds(FRONT + (UNROLL - 2 + i) * n_groups, n_groups)] = jnp.zeros((n_groups, SUB, D), F32)

    @pl.loop(0, rest // SUB)
    def _(i):
        for buf in head_out[-2] + head_out[-1]:
            buf[pl.ds(pl.multiple_of(M + i * SUB, SUB), SUB), :] = jnp.zeros((SUB, D), F32)

    paced[SCALE] = jnp.full((SUB, D), scale, F32)

    xe_cp.wait()
    w_cps[1].start()
    ne[...] = pltpu.bitcast(_layernorm(xe[...].astype(F32).reshape(n_seg * SUB, D)).astype(BF16), U32)
    w_cps[0].wait()

    @pl.loop(0, half_d // (2 * PACK))
    def _(i):
        list(repack(qkv_rows, 0, i, 2 * PACK))

    w_cps[2].start()

    @pl.loop(0, n_qkv // 2 + 1)
    def _(c):
        @pl.when(c < n_qkv // 2)
        def _():
            def wait(k):
                pltpu.make_async_copy(raw_qkv.at[k], raw_qkv.at[k], wsem.at[k]).wait()

            wait(2 * c + 1)
            for k, batch in enumerate(batches):
                @pl.when(c == k)
                def _():
                    for cp in batch:
                        cp.start()

            pl.when(c > 0)(functools.partial(wait, 2 * c))
            project_early(c, qkv_rows, [2 * c, 2 * c + 1])

        @pl.when(c >= n_qkv // 2)
        def _():
            for cp in w_cps[n_qkv:] + small_cps:
                cp.wait()
            normalize_first(0)
            project_early(c, out_rows, [2 * c + j for j in range(per_w)])

    for cp in x_cps[1:] + ffn_cps:
        cp.start()

    w_r = wr[...].astype(F32).reshape(1, D)

    def softmax(raw):
        qi = lax.broadcasted_iota(jnp.int32, raw.shape, 0)
        ki = lax.broadcasted_iota(jnp.int32, raw.shape, 1)
        sc = jnp.where((qi < M) | (ki <= qi + SUB), raw * scale, MASK_FILL)
        e = jnp.exp2(sc - jnp.max(sc, axis=-1, keepdims=True))
        return e * pltpu.reciprocal(jnp.sum(e, axis=-1, keepdims=True), approx=True)

    def rolled(blocks):
        return [pltpu.roll(b, d, 0) if d else b for b in blocks for d in range(SUB)]

    def combine(odd, k, parts, put, skip=0):
        def with_m(v, op=jnp.add):
            if odd:
                return jnp.concatenate([op(v[:-PACK], parts[0][skip - PACK:]), v[-PACK:]], axis=0)
            return jnp.concatenate([v[:-PACK], op(v[-PACK:], parts[0][-PACK:])], axis=0)

        tokens, memory = (lambda j: parts[j][skip - T:]), (lambda j: parts[j][:M])
        if k == 0:
            put(1 - odd, 1 - odd, with_m(tokens(1)), not odd)
            return None
        if k == 1:
            put(odd, 1 - odd, tokens(1) + tokens(2), False)
            return 1 - odd, memory(1) + memory(2)
        put(odd, odd, tokens(3) - with_m(tokens(2), jnp.subtract), not odd)
        return odd, memory(0) - memory(2) + memory(3)

    def memory_left(odd, j, half, both):
        return both() if j == 2 else half(odd if j < 2 else 1 - odd)

    def project(u, zero, skip, i, g, j, parts, with_memory=True):
        odd = u % 2
        lo = skip if j or odd else 0
        lhs = tok[u][pl.ds(j // 2 * T + lo, (T if j else PACK) - lo), col(j % 2, half_d)]
        if with_memory:
            mem = memory_left(odd, j, lambda k: paced[MEM, :, col(k, half_d)],
                              lambda: paced[MEM_SUM, :, col(0, half_d)])
            lhs = jnp.concatenate([mem, lhs], axis=0)
        parts[j] = _mm(lhs, factor(i * n_groups + g, j + 3 * odd if j else 0))

        def put(seg, k, v, accumulate):
            buf, cols = qkv[(u + odd + seg) % UNROLL][i][g], col(k, half_d)
            buf[at(zero, M + skip, T - skip), cols] = v + buf[M + skip:, cols] if accumulate else v

        for k, needs in enumerate(((0, 1), (1, 2), (0, 2, 3))):
            if j in needs and all(n in parts for n in needs):
                mem = combine(odd, k, parts, put, skip)
                if mem and with_memory:
                    qkv[u][i][g][at(zero, 0, M), col(mem[0], half_d)] = mem[1]

    def project_out(u, g, j, acc, with_memory=True):
        odd = u % 2

        def rows(seg):
            src = (u + odd - 2 + seg) % UNROLL
            return lambda k: jnp.concatenate([paced[FRONT + src * n_groups + g, :, col(k, half_d)],
                                              head_out[src][g][pl.ds(M, rest), col(k, half_d)]], axis=0)

        lhs = _left(odd, j, rows(0), rows(1))
        if j == 0:
            lhs = lhs[:PACK] if odd else lhs[PACK:]
        if with_memory:
            half = lambda k: head_out[u][g][pl.ds(0, M), col(k, half_d)]
            lhs = jnp.concatenate([memory_left(odd, j, half, lambda: half(0) + half(1)), lhs], axis=0)
        part = _mm(lhs, factor(3 * n_groups + g, j + 3 * odd if j else 0))
        acc[j] = part + 0.0 if acc[j] is None else acc[j] + part

    def finish_out(u, acc):
        def put(seg, k, v, accumulate):
            att[seg, :, col(k, half_d)] = v + att[seg, :, col(k, half_d)] if accumulate else v

        return [combine(u % 2, k, acc, put) for k in range(3)][1:]

    def set_memory(halves):
        for k, v in halves:
            paced[MEM, :, col(k, half_d)] = v
        paced[MEM_SUM, :, col(0, half_d)] = halves[0][1] + halves[1][1]

    def attend_pair(s0, u0, zero, ahead, timing, side_work):
        def rows_of(i, odd, h):
            buf, cols = qkv[u0 + odd][i][h // GROUP], col(h % GROUP, Dh)
            if (i, h // GROUP) in ahead:
                rows = pl.ds(pl.multiple_of((s0 + odd) * SUB, SUB), SUB)
                front = early[i * per_w + h // CHUNK, h % CHUNK, rows, :]
            else:
                front = buf[pl.ds(M, SUB), cols]
            return buf[pl.ds(0, M), cols], front, buf[pl.ds(M + SUB, rest), cols]

        def front_scores(odd, h):
            q = rows_of(0, odd, h)[1] * paced[SCALE, :, col(0)]
            sub = lax.broadcasted_iota(jnp.int32, q.shape, 0)
            out = []
            for j, k in enumerate(rolled(rows_of(1, odd, h)[:2])):
                sc = jnp.broadcast_to(jnp.sum(q * k, axis=-1, keepdims=True), q.shape)
                out.append(jnp.where(sub >= j - M, sc, MASK_FILL) if j > M else sc)
            return out

        def front_values(odd, h, scores):
            top = functools.reduce(jnp.maximum, scores)
            num = den = None
            for sc, v in zip(scores, rolled(rows_of(2, odd, h)[:2])):
                e = jnp.exp2(sc - top)
                num, den = (e * v, e) if num is None else (num + e * v, den + e)
            return num * pltpu.reciprocal(den, approx=True)

        carried, scores, front = (), {}, {}
        for odd in range(2):
            u, lag = u0 + odd, timing[odd][-1]
            order, carried = _schedule(H, odd, timing[odd], carried)
            parts, acc, finish, marks, used = {}, [None] * 4, {}, [], set()
            for op, arg in order:
                if op == "proj":
                    if len(marks) >= lag:
                        tok[u][at(zero, PACK, SUB), col(0)] = marks[-lag]
                    mine = parts.setdefault(arg[:2], {})
                    project(u, zero, SUB if arg[:2] in ahead else 0, *arg, mine)
                    marks.append(mine[arg[2]][-SUB:, -LANES:])
                elif op == "score":
                    raw = []
                    for h in range(arg * GROUP, (arg + 1) * GROUP):
                        q = jnp.concatenate(rows_of(0, odd, h)[::2], axis=0)
                        raw.append(_mm_nt(q, jnp.concatenate(rows_of(1, odd, h), axis=0).astype(BF16)))
                    for j, r in enumerate(raw):
                        prob[arg][zero + j] = softmax(r)
                elif op == "value":
                    for j in range(GROUP):
                        v = jnp.concatenate(rows_of(2, odd, arg * GROUP + j), axis=0).astype(BF16)
                        head_out[u][arg][at(zero, 0, M + rest), col(j, Dh)] = _mm(prob[arg][j], v)
                elif op == "out":
                    if arg[0] in used:
                        for src in range(u + odd - 2, u + 1):
                            head_out[src][arg[0]][at(zero, M + rest, SUB), col(0)] = marks[-6]
                    used.add(arg[0])
                    project_out(u, *arg, acc)
                    marks.append(acc[arg[1]][-SUB:, -LANES:])
                elif op == "front":
                    scores[arg] = front_scores(*arg)
                elif op == "mix":
                    front[arg] = front_values(*arg, scores[arg])
                elif op == "join":
                    g, j = divmod(arg[1], GROUP)
                    paced[zero + FRONT + (u0 + arg[0]) * n_groups + g, :, col(j, Dh)] = front[arg]
                elif op == "side":
                    finish[arg] = side_work[odd](arg)
                elif op == "done":
                    finish[arg]()
            set_memory(finish_out(u, acc))

    n_trip = n_seg // UNROLL
    n_sent = n_seg - UNROLL - 2
    out_cps = [pltpu.make_async_copy(stream.at[2, pl.ds(PAD + lo, hi - lo)], out_hbm.at[pl.ds(lo, hi - lo)],
                                     osem.at[i]) for i, (lo, hi) in enumerate(((0, n_sent), (n_sent, n_seg)))]

    @pl.loop(0, 2)
    def _(layer):
        def epilogue(s, zero, piece):
            seg, half = divmod(piece, 2)
            slot, rows = PAD + s + seg, pl.ds(half * PACK, PACK)
            x1 = (stream[layer, slot, rows, :].astype(F32) + _rb(att[seg, rows, :])).astype(BF16)
            n1 = _layernorm(x1.astype(F32))
            r = _rb(jnp.sum(n1 * w_r, axis=-1, keepdims=True))
            stream[layer, slot, rows, :] = x1
            stream[layer + 1, slot, rows, :] = (x1.astype(F32) + n1).astype(BF16)
            routed[slot, rows, :] = n1

            def finish():
                best, where = paced[BEST, :, col(0)], paced[WHERE, :, col(0)]
                for j in range(PACK // SUB):
                    score = r[j * SUB:(j + 1) * SUB]
                    row = lax.broadcasted_iota(jnp.int32, best.shape, 0) + (s * T + piece * PACK + j * SUB)
                    better = (score > best) & (s >= 0)
                    best, where = jnp.where(better, score, best), jnp.where(better, row.astype(F32), where)
                paced[zero + BEST, :, col(0)] = best
                paced[zero + WHERE, :, col(0)] = where
            return finish

        set_memory([(k, mem0[:, col(k, half_d)].astype(F32)) for k in range(2)])
        paced[BEST, :, col(0)] = jnp.full((SUB, LANES), -jnp.inf, F32)
        paced[WHERE, :, col(0)] = jnp.zeros((SUB, LANES), F32)
        for i in range(3):
            for g in range(n_groups):
                parts = {}
                for j in range(4):
                    project(UNROLL - 1, 0, 0, i, g, j, parts, with_memory=False)

        def trip(t, ahead, timing):
            zero = lax.shift_right_logical(t, 16)
            for u in range(0, UNROLL, 2):
                s = t * UNROLL + u
                side = (functools.partial(normalize, layer, s + 2, (u + 2) % UNROLL, zero),
                        functools.partial(epilogue, s - 2, zero))
                attend_pair(s, u, zero, ahead, timing, side)

        @pl.when(layer == 0)
        def _():
            @pl.loop(0, n_trip)
            def _(t):
                pl.when(t == 1)(x_cps[1].wait)
                trip(t, ahead, TIMING[0])

            for cp in ffn_cps:
                cp.wait()

        @pl.when(layer == 1)
        def _():
            @pl.loop(0, n_trip)
            def _(t):
                pl.when(t == n_trip - 1)(out_cps[0].start)
                trip(t, (), TIMING[1])

        acc = [None] * 4
        for j in range(4):
            for g in range(n_groups):
                project_out(0, g, j, acc, with_memory=False)
        finish_out(0, acc)
        for finish in [epilogue(n_seg - 2, 0, piece) for piece in (3, 2, 1, 0)][::-1]:
            finish()
        pl.when(layer == 1)(out_cps[1].start)

        normalize_first(layer + 1)

        best, where = paced[BEST, :, col(0)], paced[WHERE, :, col(0)]
        top = jnp.max(best, axis=0, keepdims=True)
        sel = jnp.min(jnp.where(best == top, where, S - 1), axis=0, keepdims=True)
        sel = sel.astype(jnp.int32)[0, 0]
        seg = jnp.clip(sel // T, 0, n_seg - 1)
        n1 = routed[PAD + seg]
        g = _rb(_mm(n1, wg[...]))
        u = _rb(_mm(n1, wu[...]))
        y = _rb(_mm(_rb(g * jax.nn.sigmoid(g)) * u, wd[...]))
        y = _rb(y * _rb(jax.nn.sigmoid(top[:, :1])))
        hit = lax.broadcasted_iota(jnp.int32, (T, D), 0) + seg * T == sel
        x2 = (stream[layer, PAD + seg].astype(F32) + _rb(n1 + jnp.where(hit, y, 0.0))).astype(BF16)

        @pl.when(layer == 1)
        def _():
            for cp in out_cps:
                cp.wait()

        stream[layer + 1, PAD + seg] = x2
        pl.when(seg < 2)(functools.partial(normalize_first, layer + 1))

        @pl.when(layer == 1)
        def _():
            fix_cp = pltpu.make_async_copy(stream.at[2, PAD + seg], out_hbm.at[seg], osem.at[0])
            fix_cp.start()
            fix_cp.wait()


@functools.partial(jax.jit, static_argnames=("A_seg_len",))
def pallas_interleave_layers__memory_aug_recurrent_mem_tr__moe_arch_mod__prompt_kernel(
    A_x, A_mem0, A_Wq, A_Wk, A_Wv, A_Wo, A_seg_len, B_x, B_w_r, B_w_gate, B_w_up, B_w_down,
):
    del B_x
    B, S, D = A_x.shape
    _, H, Dh = A_Wq.shape
    M = A_mem0.shape[1]
    T = int(A_seg_len)
    F = B_w_gate.shape[1]
    assert B == 1 and S % (T * UNROLL) == 0 and T == 2 * PACK and M == SUB
    assert H % CHUNK == 0 and Dh == LANES and D == GROUP * Dh
    n_seg = S // T
    per_w = H // CHUNK
    n_groups = H // GROUP

    hbm = pl.BlockSpec(memory_space=pl.ANY)
    out = pl.pallas_call(
        functools.partial(_kernel, S=S, D=D, H=H, Dh=Dh, M=M, T=T),
        out_shape=jax.ShapeDtypeStruct((n_seg, T, D), BF16),
        in_specs=[hbm] * 10,
        out_specs=hbm,
        scratch_shapes=[
            pltpu.VMEM((3, n_seg + 2 * PAD, T, D), BF16),
            pltpu.VMEM((n_seg + PAD, T, D), F32),
            pltpu.VMEM((n_seg, SUB, D), BF16),
            pltpu.VMEM((n_seg * SUB // 2, D), U32),
            pltpu.VMEM((2 * per_w, CHUNK, n_seg * SUB, Dh), F32),
            pltpu.VMEM((3 * per_w, D, CHUNK, Dh), BF16),
            pltpu.VMEM((per_w, CHUNK * Dh, D), BF16),
            pltpu.VMEM((4 * n_groups, 9, D // 2 // LANES, D // 4, LANES), U32),
            pltpu.VMEM((D, F), BF16),
            pltpu.VMEM((D, F), BF16),
            pltpu.VMEM((F, D), BF16),
            pltpu.VMEM((M, D), BF16),
            pltpu.VMEM((D,), BF16),
            pltpu.VMEM((2, T, D), F32),
            [pltpu.VMEM((2 * T + PACK, D), F32)] * UNROLL,
            [[[pltpu.VMEM((M + T, D), F32)] * n_groups] * 3] * UNROLL,
            [pltpu.VMEM((GROUP, M + T - SUB, M + T), F32)] * n_groups,
            [[pltpu.VMEM((M + T, D), F32)] * n_groups] * UNROLL,
            pltpu.VMEM((6 + UNROLL * n_groups, SUB, D), F32),
            pltpu.SemaphoreType.DMA((8,)),
            pltpu.SemaphoreType.DMA((4 * per_w,)),
            pltpu.SemaphoreType.DMA((2,)),
        ],
        compiler_params=pltpu.CompilerParams(vmem_limit_bytes=112 * 1024 * 1024),
    )(
        A_x.reshape(n_seg, T, D), A_mem0.reshape(M, D), A_Wq, A_Wk, A_Wv,
        A_Wo.reshape(per_w, CHUNK * Dh, D), B_w_r, B_w_gate, B_w_up, B_w_down,
    )
    return out.reshape(B, S, D)
```

```python
import functools

import jax
import jax.numpy as jnp
from jax import lax
import jax.experimental.pallas as pl
import jax.experimental.pallas.tpu as pltpu

F32 = jnp.float32
BF16 = jnp.bfloat16
U32 = jnp.uint32
LN_EPS = 1e-5
LOG2E = 1.4426950408889634
MASK_FILL = -1000000000.0 * LOG2E
LANES = 128
SUB = 8
PACK = 16
GROUP = 4
CHUNK = 8
UNROLL = 4
PAD = 2
EARLY_ROWS = 64
TIMING = (((6, 26, 17, 3.78, 2, 116, 127, 127, 4, 6), (6, 27, 19, 3.28, 11, 128, 131, 133, 4, 6)),
          ((7, 23, 18, 3.3, 5, 128, 130, 131, 4, 5), (7, 23, 18, 3.32, 13, 129, 132, 132, 4, 5)))


def _rb(v):
    return v.astype(BF16).astype(F32)


def _layernorm(x):
    inv_n = 1.0 / x.shape[-1]
    mean = jnp.sum(x, axis=-1, keepdims=True) * inv_n
    cen = x - mean
    var = jnp.sum(cen * cen, axis=-1, keepdims=True) * inv_n
    den = _rb(jnp.sqrt(_rb(_rb(var) + LN_EPS)))
    return _rb(_rb(x - _rb(mean)) / den)


def _mm(a, b):
    return lax.dot_general(a, b, (((1,), (0,)), ((), ())), preferred_element_type=F32)


def _mm_nt(a, b):
    return lax.dot_general(a, b, (((1,), (1,)), ((), ())), preferred_element_type=F32)


def _left(odd, j, x, y):
    own, other = (y, x) if odd else (x, y)
    if j == 0:
        return x(0) + y(1)
    if j == 1:
        return own(odd)
    if j == 2:
        return own(0) + own(1)
    return own(1 - odd) - other(1 - odd)


def _right(b00, b01, b10, b11):
    f00, f01, f10, f11 = (pltpu.bitcast(b, BF16).astype(F32) for b in (b00, b01, b10, b11))
    words = lambda v: pltpu.bitcast(v.astype(BF16), U32)
    return [words(f00 + f11), words(f01 - f11), b11, words(f10 + f11),
            words(f10 - f00), b00, words(f00 + f01), b01, b10]


PLAIN = ((5, 7), (8, 2))


def _out_slots(n_groups):
    slots = []
    for groups, last in ((range(n_groups - 2), range(n_groups - 4)),
                         (range(n_groups - 2, n_groups), range(n_groups - 4, n_groups))):
        long = [(g, j) for j in (1, 2) for g in groups]
        for k, g in enumerate(groups):
            slots += long[2 * k:2 * k + 2] + [(g, 0)]
        slots += [(g, 3) for g in last]
    return slots


def _schedule(n_heads, odd, timing, carried=()):
    score_at, value_at, start, period, *side_at, depth, _ = timing
    n_groups = n_heads // GROUP
    slots = []
    for g in range(n_groups):
        block = [(i, j) for i in range(3) for j in (1, 0, 2, 3)]
        if g == 0:
            block = block[8:10] + block[0:2] + block[10:11] + block[2:6] + block[11:] + block[6:8]
        elif g < 3:
            block = block[:2] + block[8:9] + block[2:8] + block[9:]
        slots += [("proj", (i, g, j)) for i, j in block]
    slots += [("out", gj) for gj in _out_slots(n_groups)]
    extra = {}
    for g in range(n_groups):
        extra.setdefault(3 * GROUP * (g + 1) + score_at + (g < 2), []).append(("score", g))
        extra.setdefault(min(3 * GROUP * (g + 1) + value_at, len(slots) - 13), []).append(("value", g))
    slots = [op for t, slot in enumerate(slots) for op in extra.get(t, []) + [slot]]
    vector = [(start + w * period, (kind, (odd, w - lag))) for w in range(n_heads + depth)
              for kind, lag in (("join", depth), ("front", 0), ("mix", 1)) if 0 <= w - lag < n_heads]
    vector += [(min(t + dt, len(slots)), (kind, j)) for j, t in enumerate(side_at)
               for dt, kind in ((0, "side"), (13, "done"))]
    vector = sorted(list(carried) + vector, key=lambda item: item[0])
    order = []
    for t, slot in enumerate(slots + [("end", None)]):
        while vector and vector[0][0] <= t and slot[0] not in ("score", "value"):
            order.append(vector.pop(0)[1])
        order.append(slot)
    at = {op: t for t, op in enumerate(order + [op for _, op in vector])}
    for h in range(n_heads):
        g = h // GROUP
        ready = [max(at["proj", (i, g, j)] for j in range(4)) for i in range(3)]
        used = min(at["out", (g, j)] for j in range(4))
        assert max(ready[:2]) < at["front", (odd, h)] and ready[2] < at["mix", (odd, h)]
        assert max(ready[:2]) < at["score", g] < at["value", g] < used
        assert not odd or max(at["join", (odd, h)], at.get(("join", (0, h)), 0)) < used
    return order, [(max(t - len(slots), timing[-1]), op) for t, op in vector]


def _kernel(x_hbm, mem0_hbm, wq_hbm, wk_hbm, wv_hbm, wo_hbm, wr_hbm, wg_hbm, wu_hbm, wd_hbm,
            out_hbm,
            stream, routed, xe, ne, early, raw_qkv, raw_out, tiles, wg, wu, wd, mem0, wr,
            att, tok, qkv, prob, head_out, paced, sems, wsem, osem,
            *, S, D, H, Dh, M, T):
    n_seg = S // T
    rest = T - SUB
    scale = Dh ** -0.5 * LOG2E
    half_d = D // 2
    n_groups = H // GROUP
    per_w = H // CHUNK
    per_chunk = CHUNK // GROUP
    n_qkv = 3 * per_w
    ahead = {(i, g) for i in range(2) for g in range(i * per_chunk, n_groups)}

    w_cps = [pltpu.make_async_copy(w_hbm.at[:, pl.ds(j * CHUNK, CHUNK), :], raw_qkv.at[i * per_w + j],
                                   wsem.at[i * per_w + j])
             for i, w_hbm in enumerate((wq_hbm, wk_hbm, wv_hbm)) for j in range(per_w)]
    w_cps += [pltpu.make_async_copy(wo_hbm.at[j], raw_out.at[j], wsem.at[n_qkv + j]) for j in range(per_w)]
    xe_cp = pltpu.make_async_copy(x_hbm.at[:, pl.ds(0, SUB), :], xe, sems.at[0])
    x_cps = [pltpu.make_async_copy(x_hbm.at[pl.ds(lo, hi - lo)], stream.at[0, pl.ds(PAD + lo, hi - lo)], sems.at[1 + i])
             for i, (lo, hi) in enumerate(((0, UNROLL + 2), (UNROLL + 2, n_seg)))]
    small_cps = x_cps[:1] + [pltpu.make_async_copy(mem0_hbm, mem0, sems.at[3]),
                             pltpu.make_async_copy(wr_hbm, wr, sems.at[4])]
    ffn_cps = [pltpu.make_async_copy(src, dst, sems.at[5 + i])
               for i, (src, dst) in enumerate(((wg_hbm, wg), (wu_hbm, wu), (wd_hbm, wd)))]
    batches = [w_cps[lo:hi] for lo, hi in ((3, 5), (5, 7), (7, 10), (10, 12), (12, 14), (14, 16))]
    batches[-2] += small_cps
    xe_cp.start()
    w_cps[0].start()

    def qkv_rows(c, lo, size):
        pairs = pltpu.bitcast(raw_qkv[c, pl.ds(lo, size)].reshape(size // 2, 2 * CHUNK, Dh), U32)
        pairs = jnp.swapaxes(pairs, 0, 1)
        heads = []
        for j in range(CHUNK // 2):
            even, odd = pairs[j], pairs[CHUNK // 2 + j]
            heads += [(even & 0xFFFF) | (odd << 16), (even >> 16) | ((odd >> 16) << 16)]
        flat = jnp.concatenate(heads, axis=1)
        return [flat[:, g * D:(g + 1) * D] for g in range(per_chunk)]

    def out_rows(c, lo, size):
        return [pltpu.bitcast(raw_out[c - n_qkv, pl.ds(g * D + lo, size), :], U32) for g in range(per_chunk)]

    def repack(rows, c, i, size):
        words = i * (size // 2)
        words = pl.ds(words if isinstance(i, int) else pl.multiple_of(words, SUB), size // 2)
        for g, (top, bottom) in enumerate(zip(rows(c, i * size, size), rows(c, half_d + i * size, size))):
            for n in range(half_d // LANES):
                blocks = [b[:, k * half_d + n * LANES:k * half_d + (n + 1) * LANES]
                          for b in (top, bottom) for k in range(2)]
                for j, w in enumerate(_right(*blocks)):
                    tiles[c * per_chunk + g, j, n, words, :] = w
                yield

    def head_weight(block, j):
        k, n = divmod(j, half_d // LANES)
        return pltpu.bitcast(jnp.concatenate([tiles[block, row[k], n] for row in PLAIN], axis=0), BF16)

    def factor(block, j):
        return pltpu.bitcast(jnp.concatenate([tiles[block, j, n] for n in range(half_d // LANES)], axis=1), BF16)

    def project_early(c, rows, fresh):
        src = c + jnp.where(c >= per_w, 1, 0)
        n_rows = n_seg * SUB // EARLY_ROWS
        work = (_ for k in fresh for i in range(half_d // PACK) for _ in repack(rows, k, i, PACK))
        for piece in range(CHUNK * n_rows):
            j, r = divmod(piece, n_rows)
            lhs = pltpu.bitcast(ne[pl.ds(r * EARLY_ROWS // 2, EARLY_ROWS // 2), :], BF16)
            w = head_weight(src * per_chunk + j // GROUP, j % GROUP)
            early[src, j, pl.ds(r * EARLY_ROWS, EARLY_ROWS), :] = _mm(lhs, w)
            for _ in range(len(fresh) * half_d // PACK // (2 * n_rows)):
                next(work)

    MEM, MEM_SUM, SCALE, BEST, WHERE, MARK, FRONT = range(7)

    def col(n, width=LANES):
        return pl.ds(n * width, width)

    def at(zero, lo, size):
        return pl.ds(lo, size) if isinstance(zero, int) else pl.ds(pl.multiple_of(zero + lo, SUB), size)

    def normalize(layer, s, u, zero, piece):
        half, seg = divmod(piece, 2)
        n = _layernorm(stream[layer, PAD + s + seg, pl.ds(half * PACK, PACK), :].astype(F32))
        if seg == 0:
            tok[u][at(zero, 2 * T, PACK), :] = n
        else:
            x = lambda k: tok[u][pl.ds(2 * T, PACK), col(k, half_d)]
            y = lambda k: n[:, k * half_d:(k + 1) * half_d]
            for odd in range(2):
                for j in range(1 if odd == half else 0, 4):
                    rows = at(zero, j // 2 * T + (half * PACK if j else 0), PACK)
                    tok[u - odd][rows, col(j % 2, half_d)] = _left(odd, j, x, y)

        def finish():
            paced[zero + MARK, :, col(0)] = n[-SUB:, -LANES:]
        return finish

    def normalize_first(layer):
        for piece in range(4):
            normalize(layer, 0, 0, 0, piece)

    @pl.loop(0, 2)
    def _(i):
        stream[i, pl.ds(0, PAD)] = jnp.zeros((PAD, T, D), BF16)
        stream[i, pl.ds(PAD + n_seg, PAD)] = jnp.zeros((PAD, T, D), BF16)
        att[i] = jnp.zeros((T, D), F32)
        paced[pl.ds(FRONT + (UNROLL - 2 + i) * n_groups, n_groups)] = jnp.zeros((n_groups, SUB, D), F32)

    @pl.loop(0, rest // SUB)
    def _(i):
        for buf in head_out[-2] + head_out[-1]:
            buf[pl.ds(pl.multiple_of(M + i * SUB, SUB), SUB), :] = jnp.zeros((SUB, D), F32)

    paced[SCALE] = jnp.full((SUB, D), scale, F32)

    xe_cp.wait()
    w_cps[1].start()
    ne[...] = pltpu.bitcast(_layernorm(xe[...].astype(F32).reshape(n_seg * SUB, D)).astype(BF16), U32)
    w_cps[0].wait()

    @pl.loop(0, half_d // (2 * PACK))
    def _(i):
        list(repack(qkv_rows, 0, i, 2 * PACK))

    w_cps[2].start()

    @pl.loop(0, n_qkv // 2 + 1)
    def _(c):
        @pl.when(c < n_qkv // 2)
        def _():
            def wait(k):
                pltpu.make_async_copy(raw_qkv.at[k], raw_qkv.at[k], wsem.at[k]).wait()

            wait(2 * c + 1)
            for k, batch in enumerate(batches):
                @pl.when(c == k)
                def _():
                    for cp in batch:
                        cp.start()

            pl.when(c > 0)(functools.partial(wait, 2 * c))
            project_early(c, qkv_rows, [2 * c, 2 * c + 1])

        @pl.when(c >= n_qkv // 2)
        def _():
            for cp in w_cps[n_qkv:] + small_cps:
                cp.wait()
            normalize_first(0)
            project_early(c, out_rows, [2 * c + j for j in range(per_w)])

    for cp in x_cps[1:] + ffn_cps:
        cp.start()

    w_r = wr[...].astype(F32).reshape(1, D)

    def softmax(raw):
        qi = lax.broadcasted_iota(jnp.int32, raw.shape, 0)
        ki = lax.broadcasted_iota(jnp.int32, raw.shape, 1)
        sc = jnp.where((qi < M) | (ki <= qi + SUB), raw * scale, MASK_FILL)
        e = jnp.exp2(sc - jnp.max(sc, axis=-1, keepdims=True))
        return e * pltpu.reciprocal(jnp.sum(e, axis=-1, keepdims=True), approx=True)

    def rolled(memory, tokens):
        both = jnp.concatenate([memory, tokens], axis=0).reshape(2, SUB, Dh)
        turns = [both] + [pltpu.roll(both, d, 1) for d in range(1, SUB)]
        return jnp.concatenate(turns, axis=1).reshape(2 * SUB, SUB, Dh)

    def combine(odd, k, parts, put, skip=0):
        def with_m(v, op=jnp.add):
            if odd:
                return jnp.concatenate([op(v[:-PACK], parts[0][skip - PACK:]), v[-PACK:]], axis=0)
            return jnp.concatenate([v[:-PACK], op(v[-PACK:], parts[0][-PACK:])], axis=0)

        tokens, memory = (lambda j: parts[j][skip - T:]), (lambda j: parts[j][:M])
        if k == 0:
            put(1 - odd, 1 - odd, with_m(tokens(1)), not odd)
            return None
        if k == 1:
            put(odd, 1 - odd, tokens(1) + tokens(2), False)
            return 1 - odd, memory(1) + memory(2)
        put(odd, odd, tokens(3) - with_m(tokens(2), jnp.subtract), not odd)
        return odd, memory(0) - memory(2) + memory(3)

    def memory_left(odd, j, half, both):
        return both() if j == 2 else half(odd if j < 2 else 1 - odd)

    def project(u, zero, skip, i, g, j, parts, with_memory=True):
        odd = u % 2
        lo = skip if j or odd else 0
        lhs = tok[u][pl.ds(j // 2 * T + lo, (T if j else PACK) - lo), col(j % 2, half_d)]
        if with_memory:
            mem = memory_left(odd, j, lambda k: paced[MEM, :, col(k, half_d)],
                              lambda: paced[MEM_SUM, :, col(0, half_d)])
            lhs = jnp.concatenate([mem, lhs], axis=0)
        parts[j] = _mm(lhs, factor(i * n_groups + g, j + 3 * odd if j else 0))

        def put(seg, k, v, accumulate):
            buf, cols = qkv[(u + odd + seg) % UNROLL][i][g], col(k, half_d)
            buf[at(zero, M + skip, T - skip), cols] = v + buf[M + skip:, cols] if accumulate else v

        for k, needs in enumerate(((0, 1), (1, 2), (0, 2, 3))):
            if j in needs and all(n in parts for n in needs):
                mem = combine(odd, k, parts, put, skip)
                if mem and with_memory:
                    qkv[u][i][g][at(zero, 0, M), col(mem[0], half_d)] = mem[1]

    def project_out(u, g, j, acc, with_memory=True):
        odd = u % 2

        def rows(seg):
            src = (u + odd - 2 + seg) % UNROLL
            return lambda k: jnp.concatenate([paced[FRONT + src * n_groups + g, :, col(k, half_d)],
                                              head_out[src][g][pl.ds(M, rest), col(k, half_d)]], axis=0)

        lhs = _left(odd, j, rows(0), rows(1))
        if j == 0:
            lhs = lhs[:PACK] if odd else lhs[PACK:]
        if with_memory:
            half = lambda k: head_out[u][g][pl.ds(0, M), col(k, half_d)]
            lhs = jnp.concatenate([memory_left(odd, j, half, lambda: half(0) + half(1)), lhs], axis=0)
        part = _mm(lhs, factor(3 * n_groups + g, j + 3 * odd if j else 0))
        acc[j] = part + 0.0 if acc[j] is None else acc[j] + part

    def finish_out(u, acc):
        def put(seg, k, v, accumulate):
            att[seg, :, col(k, half_d)] = v + att[seg, :, col(k, half_d)] if accumulate else v

        return [combine(u % 2, k, acc, put) for k in range(3)][1:]

    def set_memory(halves):
        for k, v in halves:
            paced[MEM, :, col(k, half_d)] = v
        paced[MEM_SUM, :, col(0, half_d)] = halves[0][1] + halves[1][1]

    def attend_pair(s0, u0, zero, ahead, timing, side_work):
        def rows_of(i, odd, h):
            buf, cols = qkv[u0 + odd][i][h // GROUP], col(h % GROUP, Dh)
            if (i, h // GROUP) in ahead:
                rows = pl.ds(pl.multiple_of((s0 + odd) * SUB, SUB), SUB)
                front = early[i * per_w + h // CHUNK, h % CHUNK, rows, :]
            else:
                front = buf[pl.ds(M, SUB), cols]
            return buf[pl.ds(0, M), cols], front, buf[pl.ds(M + SUB, rest), cols]

        def front_scores(odd, h):
            q = rows_of(0, odd, h)[1] * paced[SCALE, :, col(0)]
            k = rolled(*rows_of(1, odd, h)[:2])
            sc = jnp.broadcast_to(jnp.sum(q * k, axis=-1, keepdims=True), k.shape)
            turn = lax.broadcasted_iota(jnp.int32, (SUB - 1, SUB, Dh), 0)
            row = lax.broadcasted_iota(jnp.int32, (SUB - 1, SUB, Dh), 1)
            return jnp.concatenate([sc[:SUB + 1], jnp.where(row > turn, sc[SUB + 1:], MASK_FILL)], axis=0)

        def front_values(odd, h, sc):
            e = jnp.exp2(sc - jnp.max(sc, axis=0))
            num = jnp.sum(e * rolled(*rows_of(2, odd, h)[:2]), axis=0)
            return num * pltpu.reciprocal(jnp.sum(e, axis=0), approx=True)

        carried, scores, front = (), {}, {}
        for odd in range(2):
            u, lag = u0 + odd, timing[odd][-1]
            order, carried = _schedule(H, odd, timing[odd], carried)
            parts, acc, finish, marks, used = {}, [None] * 4, {}, [], set()
            for op, arg in order:
                if op == "proj":
                    if len(marks) >= lag:
                        tok[u][at(zero, PACK, SUB), col(0)] = marks[-lag]
                    mine = parts.setdefault(arg[:2], {})
                    project(u, zero, SUB if arg[:2] in ahead else 0, *arg, mine)
                    marks.append(mine[arg[2]][-SUB:, -LANES:])
                elif op == "score":
                    raw = []
                    for h in range(arg * GROUP, (arg + 1) * GROUP):
                        q = jnp.concatenate(rows_of(0, odd, h)[::2], axis=0)
                        raw.append(_mm_nt(q, jnp.concatenate(rows_of(1, odd, h), axis=0).astype(BF16)))
                    for j, r in enumerate(raw):
                        prob[arg][zero + j] = softmax(r)
                elif op == "value":
                    for j in range(GROUP):
                        v = jnp.concatenate(rows_of(2, odd, arg * GROUP + j), axis=0).astype(BF16)
                        head_out[u][arg][at(zero, 0, M + rest), col(j, Dh)] = _mm(prob[arg][j], v)
                elif op == "out":
                    if arg[0] in used:
                        for src in range(u + odd - 2, u + 1):
                            head_out[src][arg[0]][at(zero, M + rest, SUB), col(0)] = marks[-6]
                    used.add(arg[0])
                    project_out(u, *arg, acc)
                    marks.append(acc[arg[1]][-SUB:, -LANES:])
                elif op == "front":
                    scores[arg] = front_scores(*arg)
                elif op == "mix":
                    front[arg] = front_values(*arg, scores[arg])
                elif op == "join":
                    g, j = divmod(arg[1], GROUP)
                    paced[zero + FRONT + (u0 + arg[0]) * n_groups + g, :, col(j, Dh)] = front[arg]
                elif op == "side":
                    finish[arg] = side_work[odd](arg)
                elif op == "done":
                    finish[arg]()
            set_memory(finish_out(u, acc))

    n_trip = n_seg // UNROLL
    n_sent = n_seg - UNROLL - 2
    out_cps = [pltpu.make_async_copy(stream.at[2, pl.ds(PAD + lo, hi - lo)], out_hbm.at[pl.ds(lo, hi - lo)],
                                     osem.at[i]) for i, (lo, hi) in enumerate(((0, n_sent), (n_sent, n_seg)))]

    @pl.loop(0, 2)
    def _(layer):
        def epilogue(s, zero, piece):
            seg, half = divmod(piece, 2)
            slot, rows = PAD + s + seg, pl.ds(half * PACK, PACK)
            x1 = (stream[layer, slot, rows, :].astype(F32) + _rb(att[seg, rows, :])).astype(BF16)
            n1 = _layernorm(x1.astype(F32))
            r = _rb(jnp.sum(n1 * w_r, axis=-1, keepdims=True))
            stream[layer, slot, rows, :] = x1
            stream[layer + 1, slot, rows, :] = (x1.astype(F32) + n1).astype(BF16)
            routed[slot, rows, :] = n1

            def finish():
                best, where = paced[BEST, :, col(0)], paced[WHERE, :, col(0)]
                for j in range(PACK // SUB):
                    score = r[j * SUB:(j + 1) * SUB]
                    row = lax.broadcasted_iota(jnp.int32, best.shape, 0) + (s * T + piece * PACK + j * SUB)
                    better = (score > best) & (s >= 0)
                    best, where = jnp.where(better, score, best), jnp.where(better, row.astype(F32), where)
                paced[zero + BEST, :, col(0)] = best
                paced[zero + WHERE, :, col(0)] = where
            return finish

        set_memory([(k, mem0[:, col(k, half_d)].astype(F32)) for k in range(2)])
        paced[BEST, :, col(0)] = jnp.full((SUB, LANES), -jnp.inf, F32)
        paced[WHERE, :, col(0)] = jnp.zeros((SUB, LANES), F32)
        for i in range(3):
            for g in range(n_groups):
                parts = {}
                for j in range(4):
                    project(UNROLL - 1, 0, 0, i, g, j, parts, with_memory=False)

        def trip(t, ahead, timing):
            zero = lax.shift_right_logical(t, 16)
            for u in range(0, UNROLL, 2):
                s = t * UNROLL + u
                side = (functools.partial(normalize, layer, s + 2, (u + 2) % UNROLL, zero),
                        functools.partial(epilogue, s - 2, zero))
                attend_pair(s, u, zero, ahead, timing, side)

        @pl.when(layer == 0)
        def _():
            @pl.loop(0, n_trip)
            def _(t):
                pl.when(t == 1)(x_cps[1].wait)
                trip(t, ahead, TIMING[0])

            for cp in ffn_cps:
                cp.wait()

        @pl.when(layer == 1)
        def _():
            @pl.loop(0, n_trip)
            def _(t):
                pl.when(t == n_trip - 1)(out_cps[0].start)
                trip(t, (), TIMING[1])

        acc = [None] * 4
        for j in range(4):
            for g in range(n_groups):
                project_out(0, g, j, acc, with_memory=False)
        finish_out(0, acc)
        for finish in [epilogue(n_seg - 2, 0, piece) for piece in (3, 2, 1, 0)][::-1]:
            finish()
        pl.when(layer == 1)(out_cps[1].start)

        normalize_first(layer + 1)

        best, where = paced[BEST, :, col(0)], paced[WHERE, :, col(0)]
        top = jnp.max(best, axis=0, keepdims=True)
        sel = jnp.min(jnp.where(best == top, where, S - 1), axis=0, keepdims=True)
        sel = sel.astype(jnp.int32)[0, 0]
        seg = jnp.clip(sel // T, 0, n_seg - 1)
        n1 = routed[PAD + seg]
        g = _rb(_mm(n1, wg[...]))
        u = _rb(_mm(n1, wu[...]))
        y = _rb(_mm(_rb(g * jax.nn.sigmoid(g)) * u, wd[...]))
        y = _rb(y * _rb(jax.nn.sigmoid(top[:, :1])))
        hit = lax.broadcasted_iota(jnp.int32, (T, D), 0) + seg * T == sel
        x2 = (stream[layer, PAD + seg].astype(F32) + _rb(n1 + jnp.where(hit, y, 0.0))).astype(BF16)

        @pl.when(layer == 1)
        def _():
            for cp in out_cps:
                cp.wait()

        stream[layer + 1, PAD + seg] = x2
        pl.when(seg < 2)(functools.partial(normalize_first, layer + 1))

        @pl.when(layer == 1)
        def _():
            fix_cp = pltpu.make_async_copy(stream.at[2, PAD + seg], out_hbm.at[seg], osem.at[0])
            fix_cp.start()
            fix_cp.wait()


@functools.partial(jax.jit, static_argnames=("A_seg_len",))
def pallas_interleave_layers__memory_aug_recurrent_mem_tr__moe_arch_mod__prompt_kernel(
    A_x, A_mem0, A_Wq, A_Wk, A_Wv, A_Wo, A_seg_len, B_x, B_w_r, B_w_gate, B_w_up, B_w_down,
):
    del B_x
    B, S, D = A_x.shape
    _, H, Dh = A_Wq.shape
    M = A_mem0.shape[1]
    T = int(A_seg_len)
    F = B_w_gate.shape[1]
    assert B == 1 and S % (T * UNROLL) == 0 and T == 2 * PACK and M == SUB
    assert H == 4 * CHUNK and Dh == LANES and D == GROUP * Dh
    n_seg = S // T
    per_w = H // CHUNK
    n_groups = H // GROUP

    hbm = pl.BlockSpec(memory_space=pl.ANY)
    out = pl.pallas_call(
        functools.partial(_kernel, S=S, D=D, H=H, Dh=Dh, M=M, T=T),
        out_shape=jax.ShapeDtypeStruct((n_seg, T, D), BF16),
        in_specs=[hbm] * 10,
        out_specs=hbm,
        scratch_shapes=[
            pltpu.VMEM((3, n_seg + 2 * PAD, T, D), BF16),
            pltpu.VMEM((n_seg + PAD, T, D), F32),
            pltpu.VMEM((n_seg, SUB, D), BF16),
            pltpu.VMEM((n_seg * SUB // 2, D), U32),
            pltpu.VMEM((2 * per_w, CHUNK, n_seg * SUB, Dh), F32),
            pltpu.VMEM((3 * per_w, D, CHUNK, Dh), BF16),
            pltpu.VMEM((per_w, CHUNK * Dh, D), BF16),
            pltpu.VMEM((4 * n_groups, 9, D // 2 // LANES, D // 4, LANES), U32),
            pltpu.VMEM((D, F), BF16),
            pltpu.VMEM((D, F), BF16),
            pltpu.VMEM((F, D), BF16),
            pltpu.VMEM((M, D), BF16),
            pltpu.VMEM((D,), BF16),
            pltpu.VMEM((2, T, D), F32),
            [pltpu.VMEM((2 * T + PACK, D), F32)] * UNROLL,
            [[[pltpu.VMEM((M + T, D), F32)] * n_groups] * 3] * UNROLL,
            [pltpu.VMEM((GROUP, M + T - SUB, M + T), F32)] * n_groups,
            [[pltpu.VMEM((M + T, D), F32)] * n_groups] * UNROLL,
            pltpu.VMEM((6 + UNROLL * n_groups, SUB, D), F32),
            pltpu.SemaphoreType.DMA((8,)),
            pltpu.SemaphoreType.DMA((4 * per_w,)),
            pltpu.SemaphoreType.DMA((2,)),
        ],
        compiler_params=pltpu.CompilerParams(vmem_limit_bytes=112 * 1024 * 1024),
    )(
        A_x.reshape(n_seg, T, D), A_mem0.reshape(M, D), A_Wq, A_Wk, A_Wv,
        A_Wo.reshape(per_w, CHUNK * Dh, D), B_w_r, B_w_gate, B_w_up, B_w_down,
    )
    return out.reshape(B, S, D)
```

```python
import functools

import jax
import jax.numpy as jnp
from jax import lax
import jax.experimental.pallas as pl
import jax.experimental.pallas.tpu as pltpu

F32 = jnp.float32
BF16 = jnp.bfloat16
U32 = jnp.uint32
LN_EPS = 1e-5
LOG2E = 1.4426950408889634
MASK_FILL = -1000000000.0 * LOG2E
LANES = 128
SUB = 8
PACK = 16
GROUP = 4
CHUNK = 8
UNROLL = 4
PAD = 2
EARLY_ROWS = 64
TIMING = (((6, 26, 17, 3.78, 2, 116, 127, 127, 4, 6), (6, 27, 19, 3.28, 11, 128, 131, 133, 4, 6)),
          ((7, 23, 18, 3.3, 5, 128, 130, 131, 4, 5), (7, 23, 18, 3.32, 13, 129, 132, 132, 4, 5)))


def _rb(v):
    return v.astype(BF16).astype(F32)


def _layernorm(x):
    inv_n = 1.0 / x.shape[-1]
    mean = jnp.sum(x, axis=-1, keepdims=True) * inv_n
    cen = x - mean
    var = jnp.sum(cen * cen, axis=-1, keepdims=True) * inv_n
    den = _rb(jnp.sqrt(_rb(_rb(var) + LN_EPS)))
    return _rb(_rb(x - _rb(mean)) / den)


def _mm(a, b):
    return lax.dot_general(a, b, (((1,), (0,)), ((), ())), preferred_element_type=F32)


def _mm_nt(a, b):
    return lax.dot_general(a, b, (((1,), (1,)), ((), ())), preferred_element_type=F32)


def _left(odd, j, x, y):
    own, other = (y, x) if odd else (x, y)
    if j == 0:
        return x(0) + y(1)
    if j == 1:
        return own(odd)
    if j == 2:
        return own(0) + own(1)
    return own(1 - odd) - other(1 - odd)


def _right(b00, b01, b10, b11):
    f00, f01, f10, f11 = (pltpu.bitcast(b, BF16).astype(F32) for b in (b00, b01, b10, b11))
    words = lambda v: pltpu.bitcast(v.astype(BF16), U32)
    return [words(f00 + f11), words(f01 - f11), b11, words(f10 + f11),
            words(f10 - f00), b00, words(f00 + f01), b01, b10]


PLAIN = ((5, 7), (8, 2))


def _out_slots(n_groups):
    slots = []
    for groups, last in ((range(n_groups - 2), range(n_groups - 4)),
                         (range(n_groups - 2, n_groups), range(n_groups - 4, n_groups))):
        long = [(g, j) for j in (1, 2) for g in groups]
        for k, g in enumerate(groups):
            slots += long[2 * k:2 * k + 2] + [(g, 0)]
        slots += [(g, 3) for g in last]
    return slots


def _schedule(n_heads, odd, timing, carried=()):
    score_at, value_at, start, period, *side_at, depth, _ = timing
    n_groups = n_heads // GROUP
    slots = []
    for g in range(n_groups):
        block = [(i, j) for i in range(3) for j in (1, 0, 2, 3)]
        if g == 0:
            block = block[8:10] + block[0:2] + block[10:11] + block[2:6] + block[11:] + block[6:8]
        elif g < 3:
            block = block[:2] + block[8:9] + block[2:8] + block[9:]
        slots += [("proj", (i, g, j)) for i, j in block]
    slots += [("out", gj) for gj in _out_slots(n_groups)]
    extra = {}
    for g in range(n_groups):
        extra.setdefault(3 * GROUP * (g + 1) + score_at + (g < 2), []).append(("score", g))
        extra.setdefault(min(3 * GROUP * (g + 1) + value_at, len(slots) - 13), []).append(("value", g))
    slots = [op for t, slot in enumerate(slots) for op in extra.get(t, []) + [slot]]
    vector = [(start + w * period, (kind, (odd, w - lag))) for w in range(n_heads + depth)
              for kind, lag in (("join", depth), ("front", 0), ("mix", 1)) if 0 <= w - lag < n_heads]
    vector += [(min(t + dt, len(slots)), (kind, j)) for j, t in enumerate(side_at)
               for dt, kind in ((0, "side"), (13, "done"))]
    vector = sorted(list(carried) + vector, key=lambda item: item[0])
    order = []
    for t, slot in enumerate(slots + [("end", None)]):
        while vector and vector[0][0] <= t and slot[0] not in ("score", "value"):
            order.append(vector.pop(0)[1])
        order.append(slot)
    at = {op: t for t, op in enumerate(order + [op for _, op in vector])}
    for h in range(n_heads):
        g = h // GROUP
        ready = [max(at["proj", (i, g, j)] for j in range(4)) for i in range(3)]
        used = min(at["out", (g, j)] for j in range(4))
        assert max(ready[:2]) < at["front", (odd, h)] and ready[2] < at["mix", (odd, h)]
        assert max(ready[:2]) < at["score", g] < at["value", g] < used
        assert not odd or max(at["join", (odd, h)], at.get(("join", (0, h)), 0)) < used
    return order, [(max(t - len(slots), timing[-1]), op) for t, op in vector]


def _kernel(x_hbm, mem0_hbm, wq_hbm, wk_hbm, wv_hbm, wo_hbm, wr_hbm, wg_hbm, wu_hbm, wd_hbm,
            out_hbm,
            stream, routed, xe, ne, early, raw_qkv, raw_out, tiles, wg, wu, wd, mem0, wr,
            att, tok, qkv, prob, head_out, paced, sems, wsem, osem,
            *, S, D, H, Dh, M, T):
    n_seg = S // T
    rest = T - SUB
    scale = Dh ** -0.5 * LOG2E
    half_d = D // 2
    n_groups = H // GROUP
    per_w = H // CHUNK
    per_chunk = CHUNK // GROUP
    n_qkv = 3 * per_w
    ahead = {(i, g) for i in range(2) for g in range(i * per_chunk, n_groups)}

    w_cps = [pltpu.make_async_copy(w_hbm.at[:, pl.ds(j * CHUNK, CHUNK), :], raw_qkv.at[i * per_w + j],
                                   wsem.at[i * per_w + j])
             for i, w_hbm in enumerate((wq_hbm, wk_hbm, wv_hbm)) for j in range(per_w)]
    w_cps += [pltpu.make_async_copy(wo_hbm.at[j], raw_out.at[j], wsem.at[n_qkv + j]) for j in range(per_w)]
    xe_cp = pltpu.make_async_copy(x_hbm.at[:, pl.ds(0, SUB), :], xe, sems.at[0])
    x_cps = [pltpu.make_async_copy(x_hbm.at[pl.ds(lo, hi - lo)], stream.at[pl.ds(lo, hi - lo)], sems.at[1 + i])
             for i, (lo, hi) in enumerate(((0, UNROLL + 2), (UNROLL + 2, n_seg)))]
    small_cps = x_cps[:1] + [pltpu.make_async_copy(mem0_hbm, mem0, sems.at[3]),
                             pltpu.make_async_copy(wr_hbm, wr, sems.at[4])]
    ffn_cps = [pltpu.make_async_copy(src, dst, sems.at[5 + i])
               for i, (src, dst) in enumerate(((wg_hbm, wg), (wu_hbm, wu), (wd_hbm, wd)))]
    batches = [w_cps[lo:hi] for lo, hi in ((3, 5), (5, 7), (7, 10), (10, 12), (12, 14), (14, 16))]
    batches[-2] += small_cps
    xe_cp.start()
    w_cps[0].start()

    def qkv_rows(c, lo, size):
        pairs = pltpu.bitcast(raw_qkv[c, pl.ds(lo, size)].reshape(size // 2, 2 * CHUNK, Dh), U32)
        pairs = jnp.swapaxes(pairs, 0, 1)
        heads = []
        for j in range(CHUNK // 2):
            even, odd = pairs[j], pairs[CHUNK // 2 + j]
            heads += [(even & 0xFFFF) | (odd << 16), (even >> 16) | ((odd >> 16) << 16)]
        flat = jnp.concatenate(heads, axis=1)
        return [flat[:, g * D:(g + 1) * D] for g in range(per_chunk)]

    def out_rows(c, lo, size):
        return [pltpu.bitcast(raw_out[c - n_qkv, pl.ds(g * D + lo, size), :], U32) for g in range(per_chunk)]

    def repack(rows, c, i, size):
        words = i * (size // 2)
        words = pl.ds(words if isinstance(i, int) else pl.multiple_of(words, SUB), size // 2)
        for g, (top, bottom) in enumerate(zip(rows(c, i * size, size), rows(c, half_d + i * size, size))):
            for n in range(half_d // LANES):
                blocks = [b[:, k * half_d + n * LANES:k * half_d + (n + 1) * LANES]
                          for b in (top, bottom) for k in range(2)]
                for j, w in enumerate(_right(*blocks)):
                    tiles[c * per_chunk + g, j, n, words, :] = w
                yield

    def head_weight(block, j):
        k, n = divmod(j, half_d // LANES)
        return pltpu.bitcast(jnp.concatenate([tiles[block, row[k], n] for row in PLAIN], axis=0), BF16)

    def factor(block, j):
        return pltpu.bitcast(jnp.concatenate([tiles[block, j, n] for n in range(half_d // LANES)], axis=1), BF16)

    def project_early(c, rows, fresh):
        src = c + jnp.where(c >= per_w, 1, 0)
        n_rows = n_seg * SUB // EARLY_ROWS
        work = (_ for k in fresh for i in range(half_d // PACK) for _ in repack(rows, k, i, PACK))
        for piece in range(CHUNK * n_rows):
            j, r = divmod(piece, n_rows)
            lhs = pltpu.bitcast(ne[pl.ds(r * EARLY_ROWS // 2, EARLY_ROWS // 2), :], BF16)
            w = head_weight(src * per_chunk + j // GROUP, j % GROUP)
            early[src, j, pl.ds(r * EARLY_ROWS, EARLY_ROWS), :] = _mm(lhs, w)
            for _ in range(len(fresh) * half_d // PACK // (2 * n_rows)):
                next(work)

    MEM, MEM_SUM, SCALE, BEST, WHERE, MARK, FRONT = range(7)

    def col(n, width=LANES):
        return pl.ds(n * width, width)

    def at(zero, lo, size):
        return pl.ds(lo, size) if isinstance(zero, int) else pl.ds(pl.multiple_of(zero + lo, SUB), size)

    def normalize(slot, u, zero, piece):
        half, seg = divmod(piece, 2)
        n = _layernorm(stream[slot + seg, pl.ds(half * PACK, PACK), :].astype(F32))
        if seg == 0:
            tok[u][at(zero, 2 * T, PACK), :] = n
        else:
            x = lambda k: tok[u][pl.ds(2 * T, PACK), col(k, half_d)]
            y = lambda k: n[:, k * half_d:(k + 1) * half_d]
            for odd in range(2):
                for j in range(1 if odd == half else 0, 4):
                    rows = at(zero, j // 2 * T + (half * PACK if j else 0), PACK)
                    tok[u - odd][rows, col(j % 2, half_d)] = _left(odd, j, x, y)

        def finish():
            paced[zero + MARK, :, col(0)] = n[-SUB:, -LANES:]
        return finish

    def normalize_first(slot):
        for piece in range(4):
            normalize(slot, 0, 0, piece)

    @pl.loop(0, 2)
    def _(i):
        stream[3 * n_seg + i] = jnp.zeros((T, D), BF16)
        att[i] = jnp.zeros((T, D), F32)
        paced[pl.ds(FRONT + (UNROLL - 2 + i) * n_groups, n_groups)] = jnp.zeros((n_groups, SUB, D), F32)

    @pl.loop(0, rest // SUB)
    def _(i):
        for buf in head_out[-2] + head_out[-1]:
            buf[pl.ds(pl.multiple_of(M + i * SUB, SUB), SUB), :] = jnp.zeros((SUB, D), F32)

    paced[SCALE] = jnp.full((SUB, D), scale, F32)

    xe_cp.wait()
    w_cps[1].start()
    ne[...] = pltpu.bitcast(_layernorm(xe[...].astype(F32).reshape(n_seg * SUB, D)).astype(BF16), U32)
    w_cps[0].wait()

    @pl.loop(0, half_d // (2 * PACK))
    def _(i):
        list(repack(qkv_rows, 0, i, 2 * PACK))

    w_cps[2].start()

    @pl.loop(0, n_qkv // 2 + 1)
    def _(c):
        @pl.when(c < n_qkv // 2)
        def _():
            def wait(k):
                pltpu.make_async_copy(raw_qkv.at[k], raw_qkv.at[k], wsem.at[k]).wait()

            wait(2 * c + 1)
            for k, batch in enumerate(batches):
                @pl.when(c == k)
                def _():
                    for cp in batch:
                        cp.start()

            pl.when(c > 0)(functools.partial(wait, 2 * c))
            project_early(c, qkv_rows, [2 * c, 2 * c + 1])

        @pl.when(c >= n_qkv // 2)
        def _():
            for cp in w_cps[n_qkv:] + small_cps:
                cp.wait()
            normalize_first(0)
            project_early(c, out_rows, [2 * c + j for j in range(per_w)])

    for cp in x_cps[1:] + ffn_cps:
        cp.start()

    w_r = wr[...].astype(F32).reshape(1, D)

    def softmax(raw):
        qi = lax.broadcasted_iota(jnp.int32, raw.shape, 0)
        ki = lax.broadcasted_iota(jnp.int32, raw.shape, 1)
        sc = jnp.where((qi < M) | (ki <= qi + SUB), raw * scale, MASK_FILL)
        e = jnp.exp2(sc - jnp.max(sc, axis=-1, keepdims=True))
        return e * pltpu.reciprocal(jnp.sum(e, axis=-1, keepdims=True), approx=True)

    def rolled(memory, tokens):
        both = jnp.concatenate([memory, tokens], axis=0).reshape(2, SUB, Dh)
        turns = [both] + [pltpu.roll(both, d, 1) for d in range(1, SUB)]
        return jnp.concatenate(turns, axis=1).reshape(2 * SUB, SUB, Dh)

    def combine(odd, k, parts, put, skip=0):
        def with_m(v, op=jnp.add):
            if odd:
                return jnp.concatenate([op(v[:-PACK], parts[0][skip - PACK:]), v[-PACK:]], axis=0)
            return jnp.concatenate([v[:-PACK], op(v[-PACK:], parts[0][-PACK:])], axis=0)

        tokens, memory = (lambda j: parts[j][skip - T:]), (lambda j: parts[j][:M])
        if k == 0:
            put(1 - odd, 1 - odd, with_m(tokens(1)), not odd)
            return None
        if k == 1:
            put(odd, 1 - odd, tokens(1) + tokens(2), False)
            return 1 - odd, memory(1) + memory(2)
        put(odd, odd, tokens(3) - with_m(tokens(2), jnp.subtract), not odd)
        return odd, memory(0) - memory(2) + memory(3)

    def memory_left(odd, j, half, both):
        return both() if j == 2 else half(odd if j < 2 else 1 - odd)

    def project(u, zero, skip, i, g, j, parts, with_memory=True):
        odd = u % 2
        lo = skip if j or odd else 0
        lhs = tok[u][pl.ds(j // 2 * T + lo, (T if j else PACK) - lo), col(j % 2, half_d)]
        if with_memory:
            mem = memory_left(odd, j, lambda k: paced[MEM, :, col(k, half_d)],
                              lambda: paced[MEM_SUM, :, col(0, half_d)])
            lhs = jnp.concatenate([mem, lhs], axis=0)
        parts[j] = _mm(lhs, factor(i * n_groups + g, j + 3 * odd if j else 0))

        def put(seg, k, v, accumulate):
            buf, cols = qkv[(u + odd + seg) % UNROLL][i][g], col(k, half_d)
            buf[at(zero, M + skip, T - skip), cols] = v + buf[M + skip:, cols] if accumulate else v

        for k, needs in enumerate(((0, 1), (1, 2), (0, 2, 3))):
            if j in needs and all(n in parts for n in needs):
                mem = combine(odd, k, parts, put, skip)
                if mem and with_memory:
                    qkv[u][i][g][at(zero, 0, M), col(mem[0], half_d)] = mem[1]

    def project_out(u, g, j, acc, with_memory=True):
        odd = u % 2

        def rows(seg):
            src = (u + odd - 2 + seg) % UNROLL
            return lambda k: jnp.concatenate([paced[FRONT + src * n_groups + g, :, col(k, half_d)],
                                              head_out[src][g][pl.ds(M, rest), col(k, half_d)]], axis=0)

        lhs = _left(odd, j, rows(0), rows(1))
        if j == 0:
            lhs = lhs[:PACK] if odd else lhs[PACK:]
        if with_memory:
            half = lambda k: head_out[u][g][pl.ds(0, M), col(k, half_d)]
            lhs = jnp.concatenate([memory_left(odd, j, half, lambda: half(0) + half(1)), lhs], axis=0)
        part = _mm(lhs, factor(3 * n_groups + g, j + 3 * odd if j else 0))
        acc[j] = part + 0.0 if acc[j] is None else acc[j] + part

    def finish_out(u, acc):
        def put(seg, k, v, accumulate):
            att[seg, :, col(k, half_d)] = v + att[seg, :, col(k, half_d)] if accumulate else v

        return [combine(u % 2, k, acc, put) for k in range(3)][1:]

    def set_memory(halves):
        for k, v in halves:
            paced[MEM, :, col(k, half_d)] = v
        paced[MEM_SUM, :, col(0, half_d)] = halves[0][1] + halves[1][1]

    def attend_pair(s0, u0, zero, ahead, timing, side_work):
        def rows_of(i, odd, h):
            buf, cols = qkv[u0 + odd][i][h // GROUP], col(h % GROUP, Dh)
            if (i, h // GROUP) in ahead:
                rows = pl.ds(pl.multiple_of((s0 + odd) * SUB, SUB), SUB)
                front = early[i * per_w + h // CHUNK, h % CHUNK, rows, :]
            else:
                front = buf[pl.ds(M, SUB), cols]
            return buf[pl.ds(0, M), cols], front, buf[pl.ds(M + SUB, rest), cols]

        def front_scores(odd, h):
            q = rows_of(0, odd, h)[1] * paced[SCALE, :, col(0)]
            k = rolled(*rows_of(1, odd, h)[:2])
            sc = jnp.broadcast_to(jnp.sum(q * k, axis=-1, keepdims=True), k.shape)
            turn = lax.broadcasted_iota(jnp.int32, (SUB - 1, SUB, Dh), 0)
            row = lax.broadcasted_iota(jnp.int32, (SUB - 1, SUB, Dh), 1)
            return jnp.concatenate([sc[:SUB + 1], jnp.where(row > turn, sc[SUB + 1:], MASK_FILL)], axis=0)

        def front_values(odd, h, sc):
            e = jnp.exp2(sc - jnp.max(sc, axis=0))
            num = jnp.sum(e * rolled(*rows_of(2, odd, h)[:2]), axis=0)
            return num * pltpu.reciprocal(jnp.sum(e, axis=0), approx=True)

        carried, scores, front = (), {}, {}
        for odd in range(2):
            u, lag = u0 + odd, timing[odd][-1]
            order, carried = _schedule(H, odd, timing[odd], carried)
            parts, acc, finish, marks, used = {}, [None] * 4, {}, [], set()
            for op, arg in order:
                if op == "proj":
                    if len(marks) >= lag:
                        tok[u][at(zero, PACK, SUB), col(0)] = marks[-lag]
                    mine = parts.setdefault(arg[:2], {})
                    project(u, zero, SUB if arg[:2] in ahead else 0, *arg, mine)
                    marks.append(mine[arg[2]][-SUB:, -LANES:])
                elif op == "score":
                    raw = []
                    for h in range(arg * GROUP, (arg + 1) * GROUP):
                        q = jnp.concatenate(rows_of(0, odd, h)[::2], axis=0)
                        raw.append(_mm_nt(q, jnp.concatenate(rows_of(1, odd, h), axis=0).astype(BF16)))
                    for j, r in enumerate(raw):
                        prob[arg][zero + j] = softmax(r)
                elif op == "value":
                    for j in range(GROUP):
                        v = jnp.concatenate(rows_of(2, odd, arg * GROUP + j), axis=0).astype(BF16)
                        head_out[u][arg][at(zero, 0, M + rest), col(j, Dh)] = _mm(prob[arg][j], v)
                elif op == "out":
                    if arg[0] in used:
                        for src in range(u + odd - 2, u + 1):
                            head_out[src][arg[0]][at(zero, M + rest, SUB), col(0)] = marks[-6]
                    used.add(arg[0])
                    project_out(u, *arg, acc)
                    marks.append(acc[arg[1]][-SUB:, -LANES:])
                elif op == "front":
                    scores[arg] = front_scores(*arg)
                elif op == "mix":
                    front[arg] = front_values(*arg, scores[arg])
                elif op == "join":
                    g, j = divmod(arg[1], GROUP)
                    paced[zero + FRONT + (u0 + arg[0]) * n_groups + g, :, col(j, Dh)] = front[arg]
                elif op == "side":
                    finish[arg] = side_work[odd](arg)
                elif op == "done":
                    finish[arg]()
            set_memory(finish_out(u, acc))

    n_trip = n_seg // UNROLL
    n_sent = n_seg - UNROLL - 2
    out_cps = [pltpu.make_async_copy(stream.at[pl.ds(2 * n_seg + lo, hi - lo)],
                                     out_hbm.at[pl.ds(lo, hi - lo)], osem.at[i])
               for i, (lo, hi) in enumerate(((0, n_sent), (n_sent, n_seg)))]

    def run_layer(layer, changed):
        first = layer * n_seg

        def epilogue(s, zero, piece):
            seg, half = divmod(piece, 2)
            rows = pl.ds(half * PACK, PACK)
            src = jnp.where(s >= 0, first + s, 3 * n_seg) + seg
            x1 = (stream[src, rows, :].astype(F32) + _rb(att[seg, rows, :])).astype(BF16)
            n1 = _layernorm(x1.astype(F32))
            r = _rb(jnp.sum(n1 * w_r, axis=-1, keepdims=True))
            stream[src, rows, :] = x1
            stream[src + n_seg, rows, :] = (x1.astype(F32) + n1).astype(BF16)
            routed[PAD + s + seg, rows, :] = n1

            def finish():
                best, where = paced[BEST, :, col(0)], paced[WHERE, :, col(0)]
                for j in range(PACK // SUB):
                    score = r[j * SUB:(j + 1) * SUB]
                    row = lax.broadcasted_iota(jnp.int32, best.shape, 0) + (s * T + piece * PACK + j * SUB)
                    better = (score > best) & (s >= 0)
                    best, where = jnp.where(better, score, best), jnp.where(better, row.astype(F32), where)
                paced[zero + BEST, :, col(0)] = best
                paced[zero + WHERE, :, col(0)] = where
            return finish

        set_memory([(k, mem0[:, col(k, half_d)].astype(F32)) for k in range(2)])
        paced[BEST, :, col(0)] = jnp.full((SUB, LANES), -jnp.inf, F32)
        paced[WHERE, :, col(0)] = jnp.zeros((SUB, LANES), F32)

        def lead_in(partial):
            for i in range(3):
                for g in range(n_groups):
                    if ((i, g) in ahead) == partial:
                        parts = {}
                        for j in range(4):
                            project(UNROLL - 1, 0, 0, i, g, j, parts, with_memory=False)

        pl.when(changed < 2)(functools.partial(lead_in, False))
        lead_in(True)

        def trip(t, ahead, timing):
            zero = lax.shift_right_logical(t, 16)
            for u in range(0, UNROLL, 2):
                s = t * UNROLL + u
                side = (functools.partial(normalize, first + s + 2, (u + 2) % UNROLL, zero),
                        functools.partial(epilogue, s - 2, zero))
                attend_pair(s, u, zero, ahead, timing, side)

        @pl.when(layer == 0)
        def _():
            @pl.loop(0, n_trip)
            def _(t):
                pl.when(t == 1)(x_cps[1].wait)
                trip(t, ahead, TIMING[0])

            for cp in ffn_cps:
                cp.wait()

        @pl.when(layer == 1)
        def _():
            @pl.loop(0, n_trip)
            def _(t):
                pl.when(t == n_trip - 1)(out_cps[0].start)
                trip(t, (), TIMING[1])

        acc = [None] * 4
        for j in range(4):
            for g in range(n_groups):
                project_out(0, g, j, acc, with_memory=False)
        finish_out(0, acc)
        for finish in [epilogue(n_seg - 2, 0, piece) for piece in (3, 2, 1, 0)][::-1]:
            finish()
        pl.when(layer == 1)(out_cps[1].start)

        best, where = paced[BEST, :, col(0)], paced[WHERE, :, col(0)]
        top = jnp.max(best, axis=0, keepdims=True)
        sel = jnp.min(jnp.where(best == top, where, S - 1), axis=0, keepdims=True)
        sel = sel.astype(jnp.int32)[0, 0]
        seg = jnp.clip(sel // T, 0, n_seg - 1)
        n1 = routed[PAD + seg]
        g = _rb(_mm(n1, wg[...]))
        u = _rb(_mm(n1, wu[...]))
        y = _rb(_mm(_rb(g * jax.nn.sigmoid(g)) * u, wd[...]))
        y = _rb(y * _rb(jax.nn.sigmoid(top[:, :1])))
        hit = lax.broadcasted_iota(jnp.int32, (T, D), 0) + seg * T == sel
        x2 = (stream[first + seg].astype(F32) + _rb(n1 + jnp.where(hit, y, 0.0))).astype(BF16)

        @pl.when(layer == 1)
        def _():
            for cp in out_cps:
                cp.wait()

        stream[first + n_seg + seg] = x2
        pl.when(seg < 2)(functools.partial(normalize_first, first + n_seg))

        @pl.when(layer == 1)
        def _():
            fix_cp = pltpu.make_async_copy(stream.at[first + n_seg + seg], out_hbm.at[seg], osem.at[0])
            fix_cp.start()
            fix_cp.wait()

        return seg

    lax.fori_loop(0, 2, run_layer, 0)


@functools.partial(jax.jit, static_argnames=("A_seg_len",))
def pallas_interleave_layers__memory_aug_recurrent_mem_tr__moe_arch_mod__prompt_kernel(
    A_x, A_mem0, A_Wq, A_Wk, A_Wv, A_Wo, A_seg_len, B_x, B_w_r, B_w_gate, B_w_up, B_w_down,
):
    del B_x
    B, S, D = A_x.shape
    _, H, Dh = A_Wq.shape
    M = A_mem0.shape[1]
    T = int(A_seg_len)
    F = B_w_gate.shape[1]
    assert B == 1 and S % (T * UNROLL) == 0 and T == 2 * PACK and M == SUB
    assert H == 4 * CHUNK and Dh == LANES and D == GROUP * Dh
    n_seg = S // T
    per_w = H // CHUNK
    n_groups = H // GROUP

    hbm = pl.BlockSpec(memory_space=pl.ANY)
    out = pl.pallas_call(
        functools.partial(_kernel, S=S, D=D, H=H, Dh=Dh, M=M, T=T),
        out_shape=jax.ShapeDtypeStruct((n_seg, T, D), BF16),
        in_specs=[hbm] * 10,
        out_specs=hbm,
        scratch_shapes=[
            pltpu.VMEM((4 * n_seg + PAD, T, D), BF16),
            pltpu.VMEM((n_seg + PAD, T, D), F32),
            pltpu.VMEM((n_seg, SUB, D), BF16),
            pltpu.VMEM((n_seg * SUB // 2, D), U32),
            pltpu.VMEM((2 * per_w, CHUNK, n_seg * SUB, Dh), F32),
            pltpu.VMEM((3 * per_w, D, CHUNK, Dh), BF16),
            pltpu.VMEM((per_w, CHUNK * Dh, D), BF16),
            pltpu.VMEM((4 * n_groups, 9, D // 2 // LANES, D // 4, LANES), U32),
            pltpu.VMEM((D, F), BF16),
            pltpu.VMEM((D, F), BF16),
            pltpu.VMEM((F, D), BF16),
            pltpu.VMEM((M, D), BF16),
            pltpu.VMEM((D,), BF16),
            pltpu.VMEM((2, T, D), F32),
            [pltpu.VMEM((2 * T + PACK, D), F32)] * UNROLL,
            [[[pltpu.VMEM((M + T, D), F32)] * n_groups] * 3] * UNROLL,
            [pltpu.VMEM((GROUP, M + T - SUB, M + T), F32)] * n_groups,
            [[pltpu.VMEM((M + T, D), F32)] * n_groups] * UNROLL,
            pltpu.VMEM((6 + UNROLL * n_groups, SUB, D), F32),
            pltpu.SemaphoreType.DMA((8,)),
            pltpu.SemaphoreType.DMA((4 * per_w,)),
            pltpu.SemaphoreType.DMA((2,)),
        ],
        compiler_params=pltpu.CompilerParams(vmem_limit_bytes=112 * 1024 * 1024),
    )(
        A_x.reshape(n_seg, T, D), A_mem0.reshape(M, D), A_Wq, A_Wk, A_Wv,
        A_Wo.reshape(per_w, CHUNK * Dh, D), B_w_r, B_w_gate, B_w_up, B_w_down,
    )
    return out.reshape(B, S, D)
```
